```python
import os as _os
_os.environ.setdefault("JAX_PLATFORMS", "cpu")
import jax
import jax.numpy as jnp

def _softmax(x, axis=-1):
    return jax.nn.softmax(x, axis=axis)
def _gelu(x):
    return jax.nn.gelu(x, approximate=True)
def _silu(x):
    return jax.nn.silu(x)
def _sigmoid(x):
    return jax.nn.sigmoid(x)
def _layernorm(x, axis=-1, eps=1e-5):
    m = jnp.mean(x, axis=axis, keepdims=True)
    v = jnp.var(x, axis=axis, keepdims=True)
    return (x - m) / jnp.sqrt(v + eps)
def _scatter_add(tgt, idx, src, axis=0):
    return tgt.at[idx].add(src)
def _segment_sum(src, seg, n):
    return jax.ops.segment_sum(src, seg, n)
class _Rng:
    def __init__(self, key):
        self._k = key
    def _next(self):
        self._k, sub = jax.random.split(self._k)
        return sub
    def normal(self, shape):
        return jax.random.normal(self._next(), shape, dtype=jnp.bfloat16)
    def randint(self, lo, hi, shape):
        return jax.random.randint(self._next(), shape, lo, hi, dtype=jnp.int32)
    def uniform(self, shape, lo=0.0, hi=1.0):
        return jax.random.uniform(self._next(), shape, jnp.bfloat16, lo, hi)
    def permutation(self, n):
        return jax.random.permutation(self._next(), n)


kernel_name = 'concat_heads__sliding_block__sliding_block__prompt'

def setup_inputs():
    _rng = _Rng(jax.random.key(int.from_bytes(__import__("os").urandom(4), "little")))
    _w = (lambda a: (lambda t: t.astype(jnp.bfloat16) if jnp.issubdtype(t.dtype, jnp.floating) else t)(jnp.asarray(a)))
    def _A_setup():
        B, S, D = 1, 2048, 448
        return {
            "x": _w((lambda *s: _rng.normal(s) * 0.2)(B, S, D)),
            "wqkv": _w((lambda *s: _rng.normal(s) * 0.2)(D, 3 * D)),
            "wo": _w((lambda *s: _rng.normal(s) * 0.05)(D, D)),
        }
    _A_in = _A_setup()

    def _B_setup():
        B, S, D = 1, 2048, 448
        return {
            "x": _w((lambda *s: _rng.normal(s) * 0.2)(B, S, D)),
            "wqkv": _w((lambda *s: _rng.normal(s) * 0.2)(D, 3 * D)),
            "wo": _w((lambda *s: _rng.normal(s) * 0.05)(D, D)),
        }
    _B_in = _B_setup()

    return {
        "A_x": _A_in["x"],
        "A_wqkv": _A_in["wqkv"],
        "A_wo": _A_in["wo"],
        "B_x": _B_in["x"],
        "B_wqkv": _B_in["wqkv"],
        "B_wo": _B_in["wo"],
    }

def reference(A_x, A_wqkv, A_wo, B_x, B_wqkv, B_wo):
    def _A_ref(x, wqkv, wo):
        B, S, D = x.shape
        H = 16; Dh = D // H; W = 256
        qkv = (lambda x, *d: x.transpose(*d))((x @ wqkv).reshape(B, S, 3, H, Dh), 2, 0, 3, 1, 4)
        q, k, v = qkv[0], qkv[1], qkv[2]
        scores = jnp.einsum("bhqd,bhkd->bhqk", q, k) * (Dh ** -0.5)
        idx = jnp.arange(S)
        mask = (idx[:, None] - idx[None, :] >= 0) & (idx[:, None] - idx[None, :] < W)
        scores = jnp.where(mask[None, None], scores, -1e9)
        p = _softmax(scores, axis=-1)
        o = jnp.einsum("bhqk,bhkd->bhqd", p, v)
        return (lambda x, *d: x.transpose(*d))(o, 0, 2, 1, 3).reshape(B, S, D) @ wo

    def _B_ref(x, wqkv, wo):
        B, S, D = x.shape
        H = 16; Dh = D // H; W = 256
        qkv = (lambda x, *d: x.transpose(*d))((x @ wqkv).reshape(B, S, 3, H, Dh), 2, 0, 3, 1, 4)
        q, k, v = qkv[0], qkv[1], qkv[2]
        scores = jnp.einsum("bhqd,bhkd->bhqk", q, k) * (Dh ** -0.5)
        idx = jnp.arange(S)
        mask = (idx[:, None] - idx[None, :] >= 0) & (idx[:, None] - idx[None, :] < W)
        scores = jnp.where(mask[None, None], scores, -1e9)
        p = _softmax(scores, axis=-1)
        o = jnp.einsum("bhqk,bhkd->bhqd", p, v)
        return (lambda x, *d: x.transpose(*d))(o, 0, 2, 1, 3).reshape(B, S, D) @ wo

    a = _A_ref(A_x, A_wqkv, A_wo)
    b = _B_ref(B_x, B_wqkv, B_wo)
    return jnp.concatenate([a, b], axis=-1)
```

```python
import math
import jax, jax.numpy as jnp
from jax import lax
import jax.experimental.pallas as pl
import jax.experimental.pallas.tpu as pltpu

S, D, H, DH, W = 2048, 448, 16, 28, 256
TQ = 256
NQ = TQ // 128
DELAY = 3
PVOFF = (0, 1, 2)
SPLITS = ((5, 5, 4, 4), (4, 4, 5, 5))
NEG = -1e30
QSCALE = (DH ** -0.5) * math.log2(math.e)
f32, bf16, i32, u32 = jnp.float32, jnp.bfloat16, jnp.int32, jnp.uint32
HI = 0xFFFF0000


def _iota(shape, dim):
    return lax.broadcasted_iota(i32, shape, dim)


def _w(x):
    return pltpu.bitcast(x, u32)


def _b(x):
    return pltpu.bitcast(x, bf16)


def _pack(a, b):
    ua = lax.bitcast_convert_type(a, u32)
    ub = lax.bitcast_convert_type(b, u32)
    return (ua >> 16) | (ub & jnp.uint32(HI))


def kernel(xa_ref, xb_ref, wa_ref, woa_ref, wb_ref, wob_ref, o_ref,
           wt_scr, wot_scr, k_scr, ktmp_scr, vt_scr, qt_scr, ot_scr, mq_scr):
    step = pl.program_id(0)

    @pl.when(step == 0)
    def _():
        lane = _iota((W, 512), 1)
        kpad = _w(jnp.where(lane % 128 == 112, NEG, 0.0).astype(bf16))
        for b, (w_ref, wo_ref) in enumerate(((wa_ref, woa_ref), (wb_ref, wob_ref))):
            k_scr[b, 0:W // 2, :] = kpad
            vt_scr[b, :, 0:W] = jnp.zeros((256, W), u32)
            wt_scr[b] = _w(w_ref[...].T)
            wot_scr[b] = _w(wo_ref[...].T)
        r = _iota((56, 128), 0) // 14
        l = _iota((56, 128), 1) // 32
        for c in range(4):
            mq_scr[c] = jnp.where(r == ((c - l) & 3), jnp.uint32(0xFFFFFFFF), jnp.uint32(0))

    base = pl.multiple_of(step * TQ, TQ)
    baseh = pl.multiple_of(step * (TQ // 2), TQ // 2)
    r32 = _iota((32, 128), 0)
    keyidx = jnp.where(r32 < 16, 2 * r32, 2 * r32 - 31)
    tri = keyidx <= (_iota((32, 128), 1) & 31)
    lane16 = _iota((16, 128), 1)
    sel1 = (lane16 & 32) == 0
    sel2 = (lane16 & 64) == 0
    tail = jnp.where(_iota((8, 128), 0) == 0, jnp.uint32(0x3F803F80), jnp.uint32(0))
    row8 = _iota((8, 128), 0)
    lo4 = row8 < 4

    def project(b, x_ref):
        qkvt = jnp.dot(_b(wt_scr[b]), x_ref[...], preferred_element_type=f32)
        for t in range(4):
            kt = jnp.concatenate([qkvt[D + 112*t: D + 112*t + 112], jnp.zeros((16, TQ), f32)], axis=0)
            ktmp_scr[b, t] = _w(kt.astype(bf16).T)
            e = ktmp_scr[b, t, pl.ds(0, TQ // 4, stride=2), :]
            f = ktmp_scr[b, t, pl.ds(1, TQ // 4, stride=2), :]
            ev = (e & jnp.uint32(0xFFFF)) | (f << 16)
            od = (e >> 16) | (f & jnp.uint32(HI))
            kk = jnp.concatenate([z[8*i:8*i + 8] for i in range(TQ // 32) for z in (ev, od)], axis=0)
            k_scr[b, pl.ds(W // 2 + baseh, TQ // 2), 128*t:128*t + 128] = kk
        for qi in range(NQ):
            for t in range(4):
                q = qkvt[112*t:112*t + 112, 128*qi:128*qi + 128] * QSCALE
                r1 = pltpu.roll(q[24:56], 96, 1)
                r2 = pltpu.roll(q[56:88], 64, 1)
                r3 = pltpu.roll(q[80:112], 32, 1)
                qr = jnp.concatenate([
                    q[0:24], jnp.where(lo4, q[24:32], r1[0:8]), r1[8:32],
                    r2[0:24], jnp.where(lo4, r2[24:32], r3[0:8]), r3[8:32]], axis=0)
                qt_scr[b, 56*t:56*t + 56, 128*qi:128*qi + 128] = _w(qr.astype(bf16))
        rowv = _iota((8, TQ), 0)
        for h in range(H):
            o = 2*D + 28*h
            if h % 2 == 0:
                v = jnp.concatenate([qkvt[o:o + 24],
                                     jnp.where(rowv < 4, qkvt[o + 24:o + 32], 1.0)], axis=0)
            else:
                v = jnp.concatenate([jnp.where(rowv < 4, 1.0, qkvt[o - 4:o + 4]),
                                     qkvt[o + 4:o + 28]], axis=0)
            vt_scr[b, 16*h:16*h + 16, pl.ds(W + base, TQ)] = _w(v.astype(bf16))

    def qk(b, qi, t, c):
        k0h = pl.multiple_of(baseh + qi * 64, 64)
        q32 = qt_scr[b, 56*t:56*t + 56, 128*qi:128*qi + 128]
        w = _b(jnp.concatenate([q32 & mq_scr[c], tail], axis=0))
        parts = SPLITS[c % 2]
        off = 0
        ss = []
        for n in parts:
            kw = _b(k_scr[b, pl.ds(k0h + 16*c + 8*off, 8*n), 128*t:128*t + 128])
            ss.append(jnp.dot(kw, w, preferred_element_type=f32))
            off += n
        s = jnp.concatenate(ss, axis=0)
        sm = jnp.where(tri, s[256:288], s[0:32])
        mid = s[32:256]
        m = jnp.max(jnp.maximum(sm, jnp.max(mid.reshape(7, 32, 128), axis=0)), axis=0, keepdims=True)
        pm = jnp.exp2(sm - m)
        pmid = jnp.exp2(mid - m)
        pf = jnp.where(tri, 0.0, pm)
        pla = jnp.where(tri, pm, 0.0)
        return ([_pack(pf[0:16], pf[16:32])]
                + [_pack(pmid[32*i:32*i + 16], pmid[32*i + 16:32*i + 32]) for i in range(7)]
                + [_pack(pla[0:16], pla[16:32])])

    zero = jnp.zeros((16, 128), u32)

    def sel(m, a, bb):
        if a is None and bb is None:
            return None
        return jnp.where(m, zero if a is None else a, zero if bb is None else bb)

    def pv(b, qi, t, X, T, acc):
        k0 = pl.multiple_of(base + qi * 128, 128)
        Y = [[] for _ in range(4)]
        for B in range(4*T, 4*T + 4):
            xs = [X[c][B - c] if 0 <= B - c <= 8 else None for c in range(4)]
            a = [sel(sel1, xs[k], xs[(k + 1) % 4]) for k in range(4)]
            for j in range(4):
                y = sel(sel2, a[j], a[(j + 2) % 4])
                Y[j].append(zero if y is None else y)
        res = []
        for j in range(4):
            h = 4*t + j
            p = _b(jnp.concatenate(Y[j], axis=0))
            vt = _b(vt_scr[b, 16*h:16*h + 16, pl.ds(k0 + 128*T, 128)])
            o = jnp.dot(vt, p, preferred_element_type=f32)
            res.append(o if acc is None else acc[j] + o)
        return res

    def fin(b, qi, t, acc):
        outs = []
        for j in range(4):
            o = acc[j]
            den = o[28:29] if j % 2 == 0 else o[0:1]
            o = o * (1.0 / den)
            if j:
                o = pltpu.roll(o, 32*j, 1)
            outs.append(o)
        oc = jnp.concatenate([
            outs[0][0:24], jnp.where(lo4, outs[0][24:32], outs[1][0:8]), outs[1][8:32],
            outs[2][0:24], jnp.where(lo4, outs[2][24:32], outs[3][0:8]), outs[3][8:32]], axis=0)
        ot_scr[b, 56*t:56*t + 56, 128*qi:128*qi + 128] = _w(oc.astype(bf16))

    def outproj(b):
        return jnp.dot(_b(wot_scr[b]), _b(ot_scr[b]), preferred_element_type=f32)

    project(0, xa_ref)
    project(1, xb_ref)
    groups = [(b, qi, t) for b in range(2) for qi in range(NQ) for t in range(4)]
    outs = [None, None]
    N = len(groups)
    Xs = [[None] * 4 for _ in range(N)]
    accs = [None] * N

    def emit_pv(slot):
        for T in range(3):
            r = slot - 3 - DELAY - PVOFF[T]
            if r >= 0 and r % 4 == 0 and r // 4 < N:
                g = r // 4
                accs[g] = pv(*groups[g], Xs[g], T, accs[g])
                if T == 2:
                    fin(*groups[g], accs[g])
    slot = 0
    for g in range(N):
        for c in range(4):
            Xs[g][c] = qk(*groups[g], c)
            emit_pv(slot)
            slot += 1
    outs[0] = outproj(0)
    for _ in range(DELAY + 4):
        emit_pv(slot)
        slot += 1
    outs[1] = outproj(1)
    o_ref[...] = jnp.concatenate(outs, axis=0).astype(bf16).T


@jax.jit
def pallas_concat_heads__sliding_block__sliding_block__prompt_kernel(A_x, A_wqkv, A_wo, B_x, B_wqkv, B_wo):
    xa = A_x.reshape(S, D).T
    xb = B_x.reshape(S, D).T
    full = lambda shp: pl.BlockSpec(shp, lambda i: (0, 0))
    xspec = pl.BlockSpec((D, TQ), lambda i: (0, i))
    out = pl.pallas_call(
        kernel,
        grid=(S // TQ,),
        in_specs=[xspec, xspec, full((D, 3*D)), full((D, D)), full((D, 3*D)), full((D, D))],
        out_specs=pl.BlockSpec((TQ, 2*D), lambda i: (i, 0)),
        out_shape=jax.ShapeDtypeStruct((S, 2*D), bf16),
        scratch_shapes=[pltpu.VMEM((2, 3*D // 2, D), u32), pltpu.VMEM((2, D // 2, D), u32),
                        pltpu.VMEM((2, (S + W) // 2, 512), u32), pltpu.VMEM((2, 4, TQ // 2, 128), u32),
                        pltpu.VMEM((2, 256, S + W), u32),
                        pltpu.VMEM((2, D // 2, TQ), u32), pltpu.VMEM((2, D // 2, TQ), u32),
                        pltpu.VMEM((4, 56, 128), u32)],
        compiler_params=pltpu.CompilerParams(dimension_semantics=("arbitrary",), vmem_limit_bytes=64*1024*1024),
    )(xa, xb, A_wqkv, A_wo, B_wqkv, B_wo)
    return out.reshape(1, S, 2*D)
```

```python
import math
import jax, jax.numpy as jnp
from jax import lax
import jax.experimental.pallas as pl
import jax.experimental.pallas.tpu as pltpu

S, D, H, DH, W = 2048, 448, 16, 28, 256
NT = S // 128
NEG = -1e30
QSCALE = (DH ** -0.5) * math.log2(math.e)
f32, bf16, i32, u32 = jnp.float32, jnp.bfloat16, jnp.int32, jnp.uint32
HI = 0xFFFF0000
DELAY = 2
PVOFF = (0,1,2)
SSTAGE = 3
WCH = (0,256,640,1344)
TAILF = (1,1,1,1,2)
XC = 1
XA1 = 1
BUD = (4,14)
NVT = 3
NHB = 2
WBSLOT = 28
MFENCE = 0
MPDELAY = 8
LFENCE = 4
LPDELAY = 4
LA = 54
LB = 58
SCOPES = 0


def _iota(shape, dim):
    return lax.broadcasted_iota(i32, shape, dim)


def _w(x):
    return pltpu.bitcast(x, u32)


def _b(x):
    return pltpu.bitcast(x, bf16)


def _pack(a, b):
    ua = lax.bitcast_convert_type(a, u32)
    ub = lax.bitcast_convert_type(b, u32)
    return (ua >> 16) | (ub & jnp.uint32(HI))


def _split(n, flip):
    parts = [n // 4 + (1 if k < n % 4 else 0) for k in range(4)]
    if flip:
        parts = parts[::-1]
    return [p for p in parts if p]


def _wait(name, cps):
    if SCOPES:
        with jax.named_scope(name):
            for cp in cps:
                cp.wait()
    else:
        for cp in cps:
            cp.wait()


def kernel(xa_hbm, xb_hbm, wa_hbm, woa_hbm, wb_hbm, wob_hbm, o_hbm,
           xa_s, xb_s, wa_s, wb_s, woa_s, wob_s, wta_s, wtb_s, wota_s, wotb_s,
           ka_s, kb_s, vta_s, vtb_s, qta_s, qtb_s, ota_s, otb_s, ktmp_s, omid_s, mq_s,
           s0_s, s1_s, o_s, wsem, osem):
    step = pl.program_id(0)
    x_hbm, x_s = (xa_hbm, xb_hbm), (xa_s, xb_s)
    wt_s, wot_s = (wta_s, wtb_s), (wota_s, wotb_s)
    k_s, vt_s, qt_s, ot_s = (ka_s, kb_s), (vta_s, vtb_s), (qta_s, qtb_s), (ota_s, otb_s)

    def xcopy(b, lo, hi, k):
        return pltpu.make_async_copy(x_hbm[b].at[:, lo:hi], x_s[b].at[:, lo:hi], wsem.at[8 + k])

    def ocopy(row, c0=0, c1=2 * D):
        return pltpu.make_async_copy(o_s.at[pl.ds(row, 128), c0:c1], o_hbm.at[pl.ds(row, 128), c0:c1], osem.at[0])

    nwa = len(WCH) - 1
    wa_copies = [pltpu.make_async_copy(wa_hbm.at[:, WCH[i]:WCH[i + 1]], wa_s.at[:, WCH[i]:WCH[i + 1]], wsem.at[i])
                 for i in range(nwa)]
    wb_copy = pltpu.make_async_copy(wb_hbm, wb_s, wsem.at[nwa])
    woa_copy = pltpu.make_async_copy(woa_hbm, woa_s, wsem.at[nwa + 1])
    wob_copy = pltpu.make_async_copy(wob_hbm, wob_s, wsem.at[nwa + 2])
    xa0, xa1, xb0 = xcopy(0, 0, 256, 0), xcopy(0, 256, 512, 1), xcopy(1, 0, 256, 2)
    xr1 = [xcopy(1, 256, 768, 3), xcopy(0, 512, 1024, 4)]
    xr2 = [xcopy(1, 768, S, 5), xcopy(0, 1024, S, 6)]

    def body(kind):
        first, last = kind == "first", kind == "last"
        FENCE, PDELAY = (LFENCE, LPDELAY) if last else (MFENCE, MPDELAY)
        us = {"first": (0, 1), "mid": (2, 3, 4, 5), "last": (14, 15)}[kind]
        r32 = _iota((32, 128), 0)
        keyidx = jnp.where(r32 < 16, 2 * r32, 2 * r32 - 31)
        tri = keyidx <= (_iota((32, 128), 1) & 31)
        lane16 = _iota((16, 128), 1)
        sel1 = (lane16 & 32) == 0
        sel2 = (lane16 & 64) == 0
        lo4 = _iota((8, 128), 0) < 4
        zero = jnp.zeros((16, 128), u32)
        cnt = [0]
        xcache = {}
        scnt = [0]
        ss_s = (s0_s, s1_s)
        zdyn = step // 8

        def gtok(q, dyn=False):
            if kind == "mid":
                return pl.multiple_of((step - 1) * 512 + 128 * q, 128)
            if dyn and FENCE:
                return pl.multiple_of(zdyn * 128 + 128 * q, 128)
            return 128 * q

        cur = [0]
        posts = []

        def later(th):
            posts.append((cur[0] + PDELAY, th))

        def run_posts(upto):
            while posts and posts[0][0] <= upto:
                posts.pop(0)[1]()

        def ring(q):
            return slice(128 * (q % 4), 128 * (q % 4) + 128)

        def proj(b, q, part, t):
            r0 = part * (D // 2) + 56 * t
            if XC and (b, q) in xcache:
                xt = xcache[b, q]
            else:
                xt = x_s[b][:, pl.ds(gtok(q), 128)]
                if XC == 2:
                    xt = _b(_w(xt))
                xcache[b, q] = xt
            y = jnp.dot(_b(wt_s[b][r0:r0 + 56, :]), xt, preferred_element_type=f32)
            if part == 0:
                y = y * QSCALE
                r1 = pltpu.roll(y[24:56], 96, 1)
                r2 = pltpu.roll(y[56:88], 64, 1)
                r3 = pltpu.roll(y[80:112], 32, 1)
                qr = jnp.concatenate([
                    y[0:24], jnp.where(lo4, y[24:32], r1[0:8]), r1[8:32],
                    r2[0:24], jnp.where(lo4, r2[24:32], r3[0:8]), r3[8:32]], axis=0)
                qt_s[b][56*t:56*t + 56, ring(q)] = _w(qr.astype(bf16))
            elif part == 1:
                kt = jnp.concatenate([y, jnp.zeros((16, 128), f32)], axis=0)
                slot = cnt[0] % 4
                cnt[0] += 1
                ktmp_s[slot] = _w(kt.astype(bf16).T)
                e = ktmp_s[slot, pl.ds(0, 32, stride=2), :]
                f = ktmp_s[slot, pl.ds(1, 32, stride=2), :]
                ev = (e & jnp.uint32(0xFFFF)) | (f << 16)
                od = (e >> 16) | (f & jnp.uint32(HI))
                kk = jnp.concatenate([z[8*i:8*i + 8] for i in range(4) for z in (ev, od)], axis=0)
                k_s[b][64*(q % 4):64*(q % 4) + 64, 128*t:128*t + 128] = kk
            else:
                v = jnp.concatenate([
                    y[0:24], jnp.where(lo4, y[24:32], 1.0), jnp.where(lo4, 1.0, y[24:32]), y[32:56],
                    y[56:80], jnp.where(lo4, y[80:88], 1.0), jnp.where(lo4, 1.0, y[80:88]), y[88:112]], axis=0)
                vt_s[b][64*t:64*t + 64, ring(q)] = _w(v.astype(bf16))

        def kload(b, t, off, n):
            lo = off % 256
            if lo + n <= 256:
                return k_s[b][lo:lo + n, 128*t:128*t + 128]
            return jnp.concatenate([k_s[b][lo:256, 128*t:128*t + 128],
                                    k_s[b][0:lo + n - 256, 128*t:128*t + 128]], axis=0)

        def qk(b, q, t, c):
            imin = max(0, 8 - 4 * q - c)
            q32 = qt_s[b][56*t:56*t + 56, ring(q)]
            if FENCE and not first and (cur[0] % FENCE == 0):
                ztail = _w(o_s[pl.ds(pl.multiple_of(S + 16 * zdyn, 16), 16), 0:128])
            else:
                ztail = zero[0:8]
            w = _b(jnp.concatenate([q32 & mq_s[c], ztail], axis=0))
            off = 64 * q + 16 * c - 128 + 16 * imin
            ss = []
            for n in _split(2 * (9 - imin), c % 2):
                ss.append(jnp.dot(_b(kload(b, t, off, 8 * n)), w, preferred_element_type=f32))
                off += 8 * n
            s = jnp.concatenate(ss, axis=0) if len(ss) > 1 else ss[0]
            blk = {i: s[32 * (i - imin):32 * (i - imin) + 32] for i in range(imin, 9)}
            sm = jnp.where(tri, blk[8], blk[0] if imin == 0 else NEG)
            mx = sm
            for i in range(max(imin, 1), 8):
                mx = jnp.maximum(mx, blk[i])
            m = jnp.max(mx, axis=0, keepdims=True)
            if SSTAGE and imin == 0:
                sref = ss_s[scnt[0] % 2]
                scnt[0] += 1
                early = set()
                o = 0
                for z in ss:
                    n = z.shape[0] // 16
                    early.update(range(o, o + min(n, SSTAGE)))
                    o += n
                ch = {}
                for u in range(2, 16):
                    if u in early:
                        sref[0, 16*u:16*u + 16, :] = s[16*u:16*u + 16]
                for u in range(2, 16):
                    ch[u] = sref[zdyn, 16*u:16*u + 16, :] if u in early else s[16*u:16*u + 16]
                for i in range(1, 8):
                    blk[i] = jnp.concatenate([ch[2*i], ch[2*i + 1]], axis=0)
            pm = jnp.exp2(sm - m)
            X = [None] * 9
            for i in range(max(imin, 1), 8):
                p = jnp.exp2(blk[i] - m)
                X[i] = _pack(p[0:16], p[16:32])
            if imin == 0:
                pf = jnp.where(tri, 0.0, pm)
                X[0] = _pack(pf[0:16], pf[16:32])
                pm = jnp.where(tri, pm, 0.0)
            X[8] = _pack(pm[0:16], pm[16:32])
            return X

        def sel(m, a, bb):
            if a is None and bb is None:
                return None
            return jnp.where(m, zero if a is None else a, zero if bb is None else bb)

        def pv(b, q, t, X, T, acc):
            if q + T < 2:
                return acc
            Y = [[] for _ in range(4)]
            for B in range(4*T, 4*T + 4):
                xs = [X[c][B - c] if 0 <= B - c <= 8 else None for c in range(4)]
                a = [sel(sel1, xs[k], xs[(k + 1) % 4]) for k in range(4)]
                for j in range(4):
                    y = sel(sel2, a[j], a[(j + 2) % 4])
                    Y[j].append(zero if y is None else y)
            res = []
            for j in range(4):
                h = 4*t + j
                p = _b(jnp.concatenate(Y[j], axis=0))
                vt = _b(vt_s[b][16*h:16*h + 16, ring(q + T - 2)])
                o = jnp.dot(vt, p, preferred_element_type=f32)
                res.append(o if acc is None else o + acc[j])
            return res

        def fin(b, q, t, acc):
            outs = []
            for j in range(4):
                o = acc[j]
                den = o[28:29] if j % 2 == 0 else o[0:1]
                o = o * (1.0 / den)
                if j:
                    o = pltpu.roll(o, 32*j, 1)
                outs.append(o)
            oc = jnp.concatenate([
                outs[0][0:24], jnp.where(lo4, outs[0][24:32], outs[1][0:8]), outs[1][8:32],
                outs[2][0:24], jnp.where(lo4, outs[2][24:32], outs[3][0:8]), outs[3][8:32]], axis=0)
            ot_s[b][56*t:56*t + 56, ring(q)] = _w(oc.astype(bf16))

        ohold = {}

        opart = {}

        def outp(b, q, n, phase=None):
            r0, r1 = ((0, 128, 256, 384, 448) if b == 0 else (0, 64, 192, 320, 448))[n:n + 2]
            k0, k1 = {None: (0, D), 1: (128, D), 2: (0, 128)}[phase]
            y = jnp.dot(_b(wot_s[b][r0 // 2:r1 // 2, k0:k1]), _b(ot_s[b][k0 // 2:k1 // 2, ring(q)]),
                        preferred_element_type=f32)
            if phase == 1:
                opart[n] = y
                return
            if phase == 2:
                y = y + opart[n]
            pieces = q == NT - 1

            def put(c0, c1, val):
                row = gtok(q, dyn=True)
                o_s[pl.ds(row, 128), c0:c1] = val.astype(bf16).T
                if pieces:
                    ocopy(row, c0, c1).start()
                elif c1 == 2 * D:
                    ocopy(row).start()

            def post():
                if b == 0:
                    if n == 0:
                        ohold[q] = y
                    elif n == 1:
                        put(0, 256, jnp.concatenate([ohold.pop(q), y], axis=0))
                    else:
                        omid_s[q % 4, 128 * (n - 2):r1 - 256] = y
                else:
                    if n == 0:
                        put(256, 512, jnp.concatenate([omid_s[q % 4], y], axis=0))
                    elif n == 1:
                        ohold[q] = y
                    elif n == 2:
                        put(512, 768, jnp.concatenate([ohold.pop(q), y], axis=0))
                    else:
                        put(768, 896, y)
            later(post)

        def wtile(src, dst, i, ncol):
            c0, c1 = 128 * i, min(128 * i + 128, ncol)
            dst[c0 // 2:c1 // 2, :] = _w(src[:, c0:c1].T)

        def projs(u, order=(1, 0, 2)):
            s, b = divmod(u, 2)
            return [(lambda p=p, t=t, q=q: proj(b, q, p, t))
                    for p in order for q in (2*s, 2*s + 1) for t in range(4)]

        def outs(u, qi):
            s, b = divmod(u, 2)
            return [(lambda n=n: outp(b, 2*s + qi, n)) for n in range(4)]

        groups = [(u % 2, 2 * (u // 2) + qi, t) for u in us for qi in range(2) for t in range(4)]
        if last:
            groups = ([(0, 14, t) for t in range(4)] + [(1, 14, t) for t in range(4)]
                      + [(0, 15, t) for t in range(4)] + [(1, 15, t) for t in (3, 2, 1, 0)])
        N = len(groups)
        Xs = [[None] * 4 for _ in range(N)]
        accs = [None] * N

        def emit_pv(slot):
            for T in range(3):
                r = slot - 3 - DELAY - PVOFF[T]
                if r >= 0 and r % 4 == 0 and r // 4 < N:
                    g = r // 4
                    accs[g] = pv(*groups[g], Xs[g], T, accs[g])
                    if T == 2:
                        fin(*groups[g], accs[g])
                        Xs[g] = accs[g] = None

        fill = {}

        def spread(thunks, lo, hi):
            n = len(thunks)
            for k, th in enumerate(thunks):
                fill.setdefault(lo + (k * (hi - lo)) // n, []).append(th)

        NTL = sum(TAILF)
        if first:
            for i in range(nwa):
                wa_copies[i].start()
                if i == 0:
                    xa0.start()
                if i == XA1:
                    xa1.start()
            wb_copy.start()
            xb0.start()
            woa_copy.start()
            wob_copy.start()
            r = _iota((56, 128), 0) // 14
            l = _iota((56, 128), 1) // 32
            o_s[S:S + 16, :] = jnp.zeros((16, 2 * D), bf16)
            for c in range(4):
                mq_s[c] = jnp.where(r == ((c - l) & 3), jnp.uint32(0xFFFFFFFF), jnp.uint32(0))
            todo = [(q, part, t) for q in range(4) for part in range(3) for t in range(4)]
            for i in range(nwa):
                _wait(f"w{i}", [wa_copies[i]] + ([xa0] if i == 0 else []) + ([xa1] if i == XA1 else []))
                if i == nwa - 1:
                    for cp in xr1 + xr2:
                        cp.start()
                for ti in range(WCH[i] // 128, (WCH[i + 1] + 127) // 128):
                    wtile(wa_s, wta_s, ti, 3 * D)
                nq = 4 if i >= XA1 else 2
                avail = [p for p in todo if p[0] < nq and p[1] * D + 112 * p[2] + 112 <= WCH[i + 1]]
                avail.sort(key=lambda p: (p[1] * D + 112 * p[2], p[0]))
                if i < nwa - 1:
                    avail = avail[:BUD[i]]
                    kch = [p for p in avail if p[1] == 1]
                    oth = [p for p in avail if p[1] != 1]
                    avail = oth[:-2] + kch + oth[-2:]
                else:
                    old = [p for p in avail if p[1] * D + 112 * p[2] + 112 <= WCH[i]]
                    extra = [p for p in old if p[0] >= 2][:max(0, 2 - len([p for p in old if p[0] < 2]))]
                    avail = [p for p in avail if p[0] < 2 or p in extra]
                for p in avail:
                    proj(0, p[0], p[1], p[2])
                    todo.remove(p)
            todo.sort(key=lambda p: ((1, 0, 2).index(p[1]), p[0], p[2]))

            def wb_prep():
                _wait("wb", [wb_copy, xb0, woa_copy, wob_copy])
                for ti in range(11):
                    wtile(wb_s, wtb_s, ti, 3 * D)
                for ti in range(4):
                    wtile(woa_s, wota_s, ti, D)
                    wtile(wob_s, wotb_s, ti, D)
            p2 = [(lambda p=p: proj(0, *p)) for p in todo]
            nk = NHB + NVT
            spread(p2[:len(p2) - nk], 0, WBSLOT)
            fill.setdefault(WBSLOT, []).append(wb_prep)
            spread(p2[len(p2) - nk:len(p2) - NVT], WBSLOT, WBSLOT + 1)
            pb = [[(lambda p=p, t=t, q=q: proj(1, q, p, t)) for p in order for t in range(4)]
                  for q, order in ((0, (0, 1, 2)), (1, (1, 0, 2)))]
            spread(pb[0], WBSLOT + 1, 32)
            spread(pb[1], 32, 46)
            rest = outs(0, 0) + outs(0, 1) + p2[len(p2) - NVT:]
            spread(rest[:len(rest) - NTL], 46, 64)
            tail = rest[len(rest) - NTL:]
        elif not last:
            @pl.when(step == 2)
            def _():
                for cp in xr2:
                    cp.wait()
            for k, u in enumerate(us):
                base = 32 * k
                p = projs(u + 1)
                if u == us[-1]:
                    p, tail = p[:24 - NTL], p[24 - NTL:]
                spread(p, base, base + 30)
                spread(outs(u - 1, 0) + outs(u - 1, 1), base + (8 if k else 0), base + 32)
        else:
            pb = [[(lambda p=p, t=t, q=q: proj(1, q, p, t)) for p in (1, 0, 2) for t in range(4)] for q in (14, 15)]
            spread(pb[0], 0, 15)
            spread(outs(13, 0) + outs(13, 1) + pb[1], 15, 46)
            oa = outs(14, 1)
            spread(outs(14, 0) + outs(15, 0), 46, LA)
            spread(oa[:2], LA, LB)
            tail = oa[2:]

        slot = 0
        for g in range(N):
            for c in range(4):
                cur[0] = slot
                run_posts(slot)
                Xs[g][c] = qk(*groups[g], c)
                for th in fill.get(slot, []):
                    th()
                emit_pv(slot)
                slot += 1

        def take(n):
            for _ in range(n):
                th = tail.pop(0)
                if th is not None:
                    th()
        nd = DELAY + max(PVOFF)
        if last:
            run_posts(10**9)
            take(len(tail))
            for k in range(nd):
                emit_pv(slot)
                slot += 1
            for ph in (1, 2):
                for n in range(4):
                    outp(1, 15, n, ph)
            run_posts(10**9)
            _wait("ow", [ocopy(128 * q) for q in range(NT - 1)]
                  + [ocopy(128 * (NT - 1), c0, c1) for c0, c1 in ((0, 256), (256, 512), (512, 768), (768, 896))])
            return
        for k in range(nd):
            if k < len(TAILF) - 1:
                take(TAILF[k])
            emit_pv(slot)
            slot += 1
        take(len(tail))
        run_posts(10**9)
        if first:
            _wait("xr1", xr1)

    def sc(kind):
        def f():
            if SCOPES:
                with jax.named_scope(kind):
                    body(kind)
            else:
                body(kind)
        return f
    pl.when(step == 0)(sc("first"))
    pl.when(jnp.logical_and(step > 0, step < 4))(sc("mid"))
    pl.when(step == 4)(sc("last"))


@jax.jit
def pallas_concat_heads__sliding_block__sliding_block__prompt_kernel(A_x, A_wqkv, A_wo, B_x, B_wqkv, B_wo):
    xa = A_x.reshape(S, D).T
    xb = B_x.reshape(S, D).T
    V = pltpu.VMEM
    two = lambda shp, dt: [V(shp, dt), V(shp, dt)]
    out = pl.pallas_call(
        kernel,
        grid=(5,),
        in_specs=[pl.BlockSpec(memory_space=pl.ANY)] * 6,
        out_specs=pl.BlockSpec(memory_space=pl.ANY),
        out_shape=jax.ShapeDtypeStruct((S, 2*D), bf16),
        scratch_shapes=(two((D, S), bf16) + two((D, 3*D), bf16) + two((D, D), bf16)
                        + two((3*D // 2, D), u32) + two((D // 2, D), u32)
                        + two((256, 512), u32) + two((256, 512), u32)
                        + two((D // 2, 512), u32) + two((D // 2, 512), u32)
                        + [V((4, 64, 128), u32), V((4, 192, 128), f32), V((4, 56, 128), u32)]
                        + two((1, 256, 128), f32) + [V((S + 16, 2*D), bf16),
                           pltpu.SemaphoreType.DMA((16,)),
                           pltpu.SemaphoreType.DMA((1,))]),
        compiler_params=pltpu.CompilerParams(dimension_semantics=("arbitrary",), vmem_limit_bytes=100*1024*1024),
    )(xa, xb, A_wqkv, A_wo, B_wqkv, B_wo)
    return out.reshape(1, S, 2*D)
```

```python
import math
import jax, jax.numpy as jnp
from jax import lax
import jax.experimental.pallas as pl
import jax.experimental.pallas.tpu as pltpu

S, D, H, DH, W = 2048, 448, 16, 28, 256
NT = S // 128
NEG = -1e30
QSCALE = (DH ** -0.5) * math.log2(math.e)
f32, bf16, i32, u32 = jnp.float32, jnp.bfloat16, jnp.int32, jnp.uint32
HI = 0xFFFF0000
WCH = (0,384,640,1344)
XA1 = 1
BUD = (6,10)
NVT = 2
NHB = 2
WBSLOT = 30
LA = 58
LB = 60
TONLY = 1
NDEF = 3
NPRE = 1
FPIECES = ((384,640),(640,896))
NT0 = 2
PARAMS = {
    "first": dict(FENCE=0, PDELAY=0, DELAY=3, PVOFF=(0, 0, 1), SSTAGE=2, SPEC=0, NSB=6, ORDER=0, TAILF=(2, 1, 1, 0, 2)),
    "mid": dict(FENCE=16, PDELAY=12, DELAY=3, PVOFF=(0, 0, 1), SSTAGE=3, SPEC=1, NSB=4, ORDER=1, TAILF=(1, 1, 1, 1, 3)),
    "last": dict(FENCE=4, PDELAY=4, DELAY=2, PVOFF=(0, 1, 2), SSTAGE=3, SPEC=1, NSB=6, ORDER=1, TAILF=(1, 1, 1, 1, 2)),
}
SIMIN = 4
FB1 = 48
L1 = 14
L2 = 48
TFENCE = 1
UNIF = 1
OPOS = 3
PORD = (0,1,2)
SCOPES = 0


def _iota(shape, dim):
    return lax.broadcasted_iota(i32, shape, dim)


def _w(x):
    return pltpu.bitcast(x, u32)


def _b(x):
    return pltpu.bitcast(x, bf16)


def _pack(a, b):
    ua = lax.bitcast_convert_type(a, u32)
    ub = lax.bitcast_convert_type(b, u32)
    return (ua >> 16) | (ub & jnp.uint32(HI))


def _split(n, flip):
    parts = [n // 4 + (1 if k < n % 4 else 0) for k in range(4)]
    if flip:
        parts = parts[::-1]
    return [p for p in parts if p]


def _wait(name, cps):
    if SCOPES:
        with jax.named_scope(name):
            for cp in cps:
                cp.wait()
    else:
        for cp in cps:
            cp.wait()


def kernel(xa_hbm, xb_hbm, wa_hbm, woa_hbm, wb_hbm, wob_hbm, o_hbm,
           xa_s, xb_s, wa_s, wb_s, woa_s, wob_s, wta_s, wtb_s, wota_s, wotb_s,
           ka_s, kb_s, vta_s, vtb_s, qta_s, qtb_s, ota_s, otb_s, ktmp_s, omid_s, mq_s,
           s0_s, s1_s, s2_s, s3_s, s4_s, s5_s, s6_s, s7_s, o_s, wsem, osem):
    step = pl.program_id(0)
    x_hbm, x_s = (xa_hbm, xb_hbm), (xa_s, xb_s)
    wt_s, wot_s = (wta_s, wtb_s), (wota_s, wotb_s)
    k_s, vt_s, qt_s, ot_s = (ka_s, kb_s), (vta_s, vtb_s), (qta_s, qtb_s), (ota_s, otb_s)

    def xcopy(b, lo, hi, k):
        j, o = divmod(lo + 256 * b, 512)
        return pltpu.make_async_copy(x_hbm[b].at[:, lo:hi], x_s[b].at[j, :, o:o + hi - lo], wsem.at[8 + k])

    def ocopy(row, c0=0, c1=2 * D):
        return pltpu.make_async_copy(o_s.at[pl.ds(row, 128), c0:c1], o_hbm.at[pl.ds(row, 128), c0:c1], osem.at[0])

    nwa = len(WCH) - 1
    wa_copies = [pltpu.make_async_copy(wa_hbm.at[:, WCH[i]:WCH[i + 1]], wa_s.at[:, WCH[i]:WCH[i + 1]], wsem.at[i])
                 for i in range(nwa)]
    wb_copy = pltpu.make_async_copy(wb_hbm, wb_s, wsem.at[nwa])
    woa_copy = pltpu.make_async_copy(woa_hbm, woa_s, wsem.at[nwa + 1])
    wob_copy = pltpu.make_async_copy(wob_hbm, wob_s, wsem.at[nwa + 2])
    xa0, xa1, xb0 = xcopy(0, 0, 256, 0), xcopy(0, 256, 512, 1), xcopy(1, 0, 256, 2)
    xr1 = [xcopy(1, 256, 768, 3), xcopy(0, 512, 1024, 4)]
    xr2 = [xcopy(1, 768, 1280, 5), xcopy(0, 1024, 1536, 6), xcopy(1, 1280, 1792, 7), xcopy(0, 1536, 2048, 8),
           xcopy(1, 1792, 2048, 9)]

    def body(kind):
        first, last = kind == "first", kind == "last"
        P = PARAMS[kind]
        FENCE, PDELAY, DELAY, PVOFF, SSTAGE, SPEC, NSB, ORDER, TAILF = (
            P[k] for k in ("FENCE", "PDELAY", "DELAY", "PVOFF", "SSTAGE", "SPEC", "NSB", "ORDER", "TAILF"))
        us = {"first": (0, 1), "mid": (2, 3, 4, 5), "last": (14, 15)}[kind]
        r32 = _iota((32, 128), 0)
        keyidx = jnp.where(r32 < 16, 2 * r32, 2 * r32 - 31)
        tri = keyidx <= (_iota((32, 128), 1) & 31)
        lane16 = _iota((16, 128), 1)
        sel1 = (lane16 & 32) == 0
        sel2 = (lane16 & 64) == 0
        lo4 = _iota((8, 128), 0) < 4
        zero = jnp.zeros((16, 128), u32)
        cnt = [0]
        xcache = {}
        scnt = [0]
        ss_s = (s0_s, s1_s, s2_s, s3_s, s4_s, s5_s, s6_s, s7_s)
        zdyn = step // 8

        def gtok(q, dyn=False):
            if kind == "mid":
                return pl.multiple_of((step - 1) * 512 + 128 * q, 128)
            if dyn and FENCE:
                return pl.multiple_of(zdyn * 128 + 128 * q, 128)
            return 128 * q

        q0 = 2 * (us[0] // 2)
        have = {}
        if not first:
            for b in range(2):
                for t in range(4):
                    for q in range(q0 - 2, q0 + (2 if b == 0 else 0)):
                        for kd in "qkv":
                            have[kd, b, q % 4, t] = q
                    for q in range(q0 - 2, q0):
                        have["o", b, q % 4, t] = q
            for q in range(q0 - 2, q0):
                have["m", 0, q % 4, 2] = have["m", 0, q % 4, 3] = q

        def made(kd, b, q, t):
            have[kd, b, q % 4, t] = q

        def need(kd, b, q, t):
            assert have.get((kd, b, q % 4, t)) == q, (kind, kd, b, q, t, have.get((kd, b, q % 4, t)))

        cur = [0]
        posts = []

        def later(th):
            posts.append((cur[0] + PDELAY, th))

        def run_posts(upto):
            while posts and posts[0][0] <= upto:
                posts.pop(0)[1]()

        def ring(q):
            return slice(128 * (q % 4), 128 * (q % 4) + 128)

        def proj(b, q, part, t, defer=None):
            r0 = part * (D // 2) + 56 * t
            if (b, q) not in xcache:
                j, o = divmod(128 * q + 256 * b, 512)
                xcache[b, q] = x_s[b][j + step - 1 if kind == "mid" else j, :, o:o + 128]
            xt = xcache[b, q]
            y = jnp.dot(_b(wt_s[b][r0:r0 + 56, :]), xt, preferred_element_type=f32)
            if defer is not None:
                defer.append(lambda: ppost(b, q, part, t, y))
            else:
                ppost(b, q, part, t, y)

        def ppost(b, q, part, t, y):
            made("qkv"[part], b, q, t)
            if part == 0:
                y = y * QSCALE
                r1 = pltpu.roll(y[24:56], 96, 1)
                r2 = pltpu.roll(y[56:88], 64, 1)
                r3 = pltpu.roll(y[80:112], 32, 1)
                qr = jnp.concatenate([
                    y[0:24], jnp.where(lo4, y[24:32], r1[0:8]), r1[8:32],
                    r2[0:24], jnp.where(lo4, r2[24:32], r3[0:8]), r3[8:32]], axis=0)
                qt_s[b][56*t:56*t + 56, ring(q)] = _w(qr.astype(bf16))
            elif part == 1:
                kt = jnp.concatenate([y, jnp.zeros((16, 128), f32)], axis=0)
                slot = cnt[0] % 4
                cnt[0] += 1
                ktmp_s[slot] = _w(kt.astype(bf16).T)
                e = ktmp_s[slot, pl.ds(0, 32, stride=2), :]
                f = ktmp_s[slot, pl.ds(1, 32, stride=2), :]
                ev = (e & jnp.uint32(0xFFFF)) | (f << 16)
                od = (e >> 16) | (f & jnp.uint32(HI))
                kk = jnp.concatenate([z[8*i:8*i + 8] for i in range(4) for z in (ev, od)], axis=0)
                k_s[b][64*(q % 4):64*(q % 4) + 64, 128*t:128*t + 128] = kk
            else:
                v = jnp.concatenate([
                    y[0:24], jnp.where(lo4, y[24:32], 1.0), jnp.where(lo4, 1.0, y[24:32]), y[32:56],
                    y[56:80], jnp.where(lo4, y[80:88], 1.0), jnp.where(lo4, 1.0, y[80:88]), y[88:112]], axis=0)
                vt_s[b][64*t:64*t + 64, ring(q)] = _w(v.astype(bf16))

        def kload(b, t, off, n):
            lo = off % 256
            if lo + n <= 256:
                return k_s[b][lo:lo + n, 128*t:128*t + 128]
            return jnp.concatenate([k_s[b][lo:256, 128*t:128*t + 128],
                                    k_s[b][0:lo + n - 256, 128*t:128*t + 128]], axis=0)

        def qk(b, q, t, c):
            imin = max(0, 8 - 4 * q - c)
            need("q", b, q, t)
            for qq in range(max(0, q - 2), q + 1):
                need("k", b, qq, t)
            q32 = qt_s[b][56*t:56*t + 56, ring(q)]
            if FENCE and not first and (cur[0] % FENCE == 0):
                ztail = fence_zero()
            else:
                ztail = zero[0:8]
            w = _b(jnp.concatenate([q32 & mq_s[c], ztail], axis=0))
            off = 64 * q + 16 * c - 128
            if imin == 0 and SPEC:
                sizes = (4, 4, 3, 3) if c % 2 == 0 else (3, 3, 4, 4)
                plan, o = [], 2
                for k, n in enumerate(sizes):
                    mids = list(range(o, o + n))
                    sp = (0, 16, 1, 17)[k]
                    plan.append(mids + [sp] if SPEC == 1 else [sp] + mids)
                    o += n
            else:
                plan, o = [], 2 * imin
                for n in _split(2 * (9 - imin), c % 2):
                    plan.append(list(range(o, o + n)))
                    o += n
            ch = {}
            for us_ in plan:
                runs = []
                for u in us_:
                    if runs and runs[-1][0] + runs[-1][1] == u:
                        runs[-1][1] += 1
                    else:
                        runs.append([u, 1])
                kw = [kload(b, t, off + 8 * u, 8 * n) for u, n in runs]
                kw = kw[0] if len(kw) == 1 else jnp.concatenate(kw, axis=0)
                z = jnp.dot(_b(kw), w, preferred_element_type=f32)
                for k, u in enumerate(us_):
                    ch[u] = z[16*k:16*k + 16]

            def blk(i):
                return jnp.concatenate([ch[2*i], ch[2*i + 1]], axis=0)
            sm = jnp.where(tri, blk(8), blk(0) if imin == 0 else NEG)
            mx = sm
            for i in range(max(imin, 1), 8):
                mx = jnp.maximum(mx, blk(i))
            m = jnp.max(mx, axis=0, keepdims=True)
            if SSTAGE and imin <= SIMIN:
                sref = ss_s[scnt[0] % NSB]
                scnt[0] += 1
                early = [u for us_ in plan for u in us_[:min(SSTAGE, len(us_) - 1)] if 2 <= u < 16]
                for u in early:
                    sref[0, 16*u:16*u + 16, :] = ch[u]
                if SPEC == 2 and imin == 0:
                    sref[0, 0:32, :] = sm
                    sm = sref[zdyn, 0:32, :]
                for u in early:
                    ch[u] = sref[zdyn, 16*u:16*u + 16, :]
            pm = jnp.exp2(sm - m)
            X = [None] * 9
            for i in range(max(imin, 1), 8):
                p = jnp.exp2(blk(i) - m)
                X[i] = _pack(p[0:16], p[16:32])
            if imin == 0:
                pf = jnp.where(tri, 0.0, pm)
                X[0] = _pack(pf[0:16], pf[16:32])
                pm = jnp.where(tri, pm, 0.0)
            X[8] = _pack(pm[0:16], pm[16:32])
            return X

        def fence_zero():
            return _w(o_s[pl.ds(pl.multiple_of(S + 16 * zdyn, 16), 16), 0:128])

        def pv(b, q, t, X, T, acc):
            if q + T < 2:
                return acc
            for j in range(4):
                need("v", b, q + T - 2, t)
            zz = zero
            if last and (b, q, t) == (1, NT - 1, 0) and T == TFENCE - 1:
                fz = fence_zero()
                zz = jnp.concatenate([fz, fz], axis=0)

            def sel(m, a, bb):
                if a is None and bb is None:
                    return None
                return jnp.where(m, zz if a is None else a, zz if bb is None else bb)
            Y = [[] for _ in range(4)]
            for B in range(4*T, 4*T + 4):
                xs = [X[c][B - c] if 0 <= B - c <= 8 else None for c in range(4)]
                a = [sel(sel1, xs[k], xs[(k + 1) % 4]) for k in range(4)]
                for j in range(4):
                    y = sel(sel2, a[j], a[(j + 2) % 4])
                    Y[j].append(zero if y is None else y)
            res = []
            for j in range(4):
                h = 4*t + j
                p = _b(jnp.concatenate(Y[j], axis=0))
                vt = _b(vt_s[b][16*h:16*h + 16, ring(q + T - 2)])
                o = jnp.dot(vt, p, preferred_element_type=f32)
                res.append(o if acc is None else o + acc[j])
            return res

        def fin(b, q, t, acc):
            made("o", b, q, t)
            outs = []
            for j in range(4):
                o = acc[j]
                den = o[28:29] if j % 2 == 0 else o[0:1]
                o = o * (1.0 / den)
                if j:
                    o = pltpu.roll(o, 32*j, 1)
                outs.append(o)
            oc = jnp.concatenate([
                outs[0][0:24], jnp.where(lo4, outs[0][24:32], outs[1][0:8]), outs[1][8:32],
                outs[2][0:24], jnp.where(lo4, outs[2][24:32], outs[3][0:8]), outs[3][8:32]], axis=0)
            ot_s[b][56*t:56*t + 56, ring(q)] = _w(oc.astype(bf16))

        ohold = {}

        def put(q, c0, c1, val):
            row = gtok(q, dyn=True)
            o_s[pl.ds(row, 128), c0:c1] = val.astype(bf16).T
            if q == NT - 1:
                ocopy(row, c0, c1).start()
            elif c1 == 2 * D:
                ocopy(row).start()

        def outp(b, q, n):
            for t in range(4):
                need("o", b, q, t)
            r0, r1 = ((0, 128, 256, 384, 448) if b == 0 else (0, 64, 192, 320, 448))[n:n + 2]
            y = jnp.dot(_b(wot_s[b][r0 // 2:r1 // 2, :]), _b(ot_s[b][:, ring(q)]),
                        preferred_element_type=f32)

            def post():
                if b == 0:
                    if n == 0:
                        ohold[q] = y
                    elif n == 1:
                        put(q, 0, 256, jnp.concatenate([ohold.pop(q), y], axis=0))
                    elif n == 2 and q == NT - 1:
                        put(q, 256, 384, y)
                    else:
                        made("m", 0, q, n)
                        omid_s[q % 4, 128 * (n - 2):r1 - 256] = y
                else:
                    if n == 0:
                        need("m", 0, q, 2)
                        need("m", 0, q, 3)
                        put(q, 256, 512, jnp.concatenate([omid_s[q % 4], y], axis=0))
                    elif n == 1:
                        ohold[q] = y
                    elif n == 2:
                        put(q, 512, 768, jnp.concatenate([ohold.pop(q), y], axis=0))
                    else:
                        put(q, 768, 896, y)
            later(post)

        def final_out():
            q = NT - 1
            for t in range(4):
                need("o", 1, q, t)
            need("m", 0, q, 3)
            parts = []
            for k0, k1 in ((128, D), (0, 128)):
                rhs = _b(ot_s[1][k0 // 2:k1 // 2, ring(q)])
                ys = [jnp.dot(_b(wot_s[1][56*n:56*n + 56, k0:k1]), rhs, preferred_element_type=f32) for n in range(4)]
                parts = [y + p for y, p in zip(ys, parts)] if parts else ys
            y = jnp.concatenate([omid_s[q % 4, 128:192]] + parts, axis=0)
            for c0, c1 in FPIECES:
                put(q, c0, c1, y[c0 - 384:c1 - 384])

        def wtile(src, dst, i, ncol):
            c0, c1 = 128 * i, min(128 * i + 128, ncol)
            dst[c0 // 2:c1 // 2, :] = _w(src[:, c0:c1].T)

        def projs(u, order=(1, 0, 2)):
            s, b = divmod(u, 2)
            return [(lambda p=p, t=t, q=q: proj(b, q, p, t))
                    for p in order for q in (2*s, 2*s + 1) for t in range(4)]

        def outs(u, qi):
            s, b = divmod(u, 2)
            return [(lambda n=n: outp(b, 2*s + qi, n)) for n in range(4)]

        groups = [(u % 2, 2 * (u // 2) + qi, t) for u in us for qi in range(2) for t in range(4)]
        if last:
            groups = ([(0, 14, t) for t in range(4)] + [(1, 14, t) for t in range(4)]
                      + [(0, 15, t) for t in range(4)] + [(1, 15, t) for t in (3, 2, 1, 0)])
        N = len(groups)
        Xs = [[None] * 4 for _ in range(N)]
        accs = [None] * N

        def emit_pv(slot):
            for T in range(3):
                r = slot - 3 - DELAY - PVOFF[T]
                if r >= 0 and r % 4 == 0 and r // 4 < N:
                    g = r // 4
                    accs[g] = pv(*groups[g], Xs[g], T, accs[g])
                    if T == 2:
                        fin(*groups[g], accs[g])
                        Xs[g] = accs[g] = None

        fill = {}

        def spread(thunks, lo, hi):
            n = len(thunks)
            for k, th in enumerate(thunks):
                fill.setdefault(lo + (k * (hi - lo)) // n, []).append(th)

        NTL = sum(TAILF)
        if first:
            for i in range(nwa):
                wa_copies[i].start()
                if i == 0:
                    xa0.start()
                if i == XA1:
                    xa1.start()
            wb_copy.start()
            xb0.start()
            woa_copy.start()
            wob_copy.start()
            r = _iota((56, 128), 0) // 14
            l = _iota((56, 128), 1) // 32
            o_s[S:S + 16, :] = jnp.zeros((16, 2 * D), bf16)
            for c in range(4):
                mq_s[c] = jnp.where(r == ((c - l) & 3), jnp.uint32(0xFFFFFFFF), jnp.uint32(0))
            todo = [(q, part, t) for q in range(4) for part in range(3) for t in range(4)]
            held = []

            def flush():
                while held:
                    held.pop(0)()
            for i in range(nwa):
                tiles = range(WCH[i] // 128, (WCH[i + 1] + 127) // 128)
                if i == 0 and TONLY:
                    _wait("wt", [wa_copies[0]])
                    for ti in tiles[:NT0]:
                        wtile(wa_s, wta_s, ti, 3 * D)
                    _wait("w0", [xa0] + ([xa1] if XA1 == 0 else []))
                    for ti in tiles[NT0:]:
                        wtile(wa_s, wta_s, ti, 3 * D)
                else:
                    _wait(f"w{i}", [wa_copies[i]] + ([xa0] if i == 0 else []) + ([xa1] if i == XA1 else []))
                    for ti in tiles:
                        wtile(wa_s, wta_s, ti, 3 * D)
                flush()
                if i == nwa - 1:
                    for cp in xr1 + xr2:
                        cp.start()
                nq = 4 if i >= XA1 else 2
                avail = [p for p in todo if p[0] < nq and p[1] * D + 112 * p[2] + 112 <= WCH[i + 1]]
                avail.sort(key=lambda p: (p[1] * D + 112 * p[2], p[0]))
                if i < nwa - 1:
                    avail = avail[:BUD[i]]
                else:
                    old = [p for p in avail if p[1] * D + 112 * p[2] + 112 <= WCH[i]]
                    extra = [p for p in old if p[0] >= 2][:max(0, 2 - len([p for p in old if p[0] < 2]))]
                    avail = [p for p in avail if p[0] < 2 or p in extra]
                for k, p in enumerate(avail):
                    proj(0, *p, defer=held if (i < nwa - 1 and k >= len(avail) - NDEF) else None)
                    todo.remove(p)
            todo.sort(key=lambda p: ((1, 0, 2).index(p[1]), p[0], p[2]))

            def wb_prep():
                _wait("wb", [wb_copy, xb0, woa_copy, wob_copy])
                flush()
                for ti in range(11):
                    wtile(wb_s, wtb_s, ti, 3 * D)
                for ti in range(4):
                    wtile(woa_s, wota_s, ti, D)
                    wtile(wob_s, wotb_s, ti, D)
            nk = NPRE + NHB + NVT
            n2 = len(todo)
            p2 = [(lambda p=p, k=k: proj(0, *p, defer=held if n2 - nk <= k < n2 - nk + NPRE else None))
                  for k, p in enumerate(todo)]
            spread(p2[:n2 - nk], 0, WBSLOT)
            spread(p2[n2 - nk:n2 - nk + NPRE], WBSLOT, WBSLOT + 1)
            fill.setdefault(WBSLOT, []).append(wb_prep)
            spread(p2[n2 - NHB - NVT:n2 - NVT], WBSLOT, WBSLOT + 1)
            pb = [[(lambda p=p, t=t, q=q: proj(1, q, p, t)) for p in order for t in range(4)]
                  for q, order in ((0, (0, 1, 2)), (1, (1, 0, 2)))]
            spread(pb[0], WBSLOT + 1, 32)
            spread(pb[1], 32, FB1)
            rest = outs(0, 0) + outs(0, 1) + p2[len(p2) - NVT:]
            spread(rest[:len(rest) - NTL], FB1, 64)
            tail = rest[len(rest) - NTL:]
        elif not last:
            @pl.when(step == 2)
            def _():
                for cp in xr2:
                    cp.wait()
            for k, u in enumerate(us):
                base = 32 * k
                p = projs(u + 1, PORD)
                if u == us[-1]:
                    p, tail = p[:24 - NTL], p[24 - NTL:]
                o = outs(u - 1, 0) + outs(u - 1, 1)
                if UNIF:
                    ps = [s for s in range(32) if s % 4 != OPOS]
                    for i, th in enumerate(p):
                        fill.setdefault(base + ps[(i * 24) // len(p)], []).append(th)
                    for i, th in enumerate(o):
                        fill.setdefault(base + 4 * i + OPOS, []).append(th)
                else:
                    spread(p, base, base + 30)
                    spread(o, base + (8 if k else 0), base + 32)
        else:
            pb = [[(lambda p=p, t=t, q=q: proj(1, q, p, t)) for p in (1, 0, 2) for t in range(4)] for q in (14, 15)]
            spread(pb[0], 0, L1)
            spread(outs(13, 0) + outs(13, 1) + pb[1], L1, L2)
            oa = outs(14, 1)
            spread(outs(14, 0) + outs(15, 0), L2, LA)
            spread(oa[:2], LA, LB)
            tail = oa[2:]

        slot = 0
        for g in range(N):
            for c in range(4):
                cur[0] = slot
                run_posts(slot)
                Xs[g][c] = qk(*groups[g], c)
                if ORDER == 1:
                    emit_pv(slot)
                for th in fill.get(slot, []):
                    th()
                if ORDER == 0:
                    emit_pv(slot)
                slot += 1

        def take(n):
            for _ in range(n):
                th = tail.pop(0)
                if th is not None:
                    th()
        nd = DELAY + max(PVOFF)
        if last:
            run_posts(10**9)
            take(len(tail))
            for k in range(nd):
                emit_pv(slot)
                slot += 1
            run_posts(10**9)
            final_out()
            _wait("ow", [ocopy(128 * q) for q in range(NT - 1)]
                  + [ocopy(128 * (NT - 1), c0, c1) for c0, c1 in ((0, 256), (256, 384)) + FPIECES])
            return
        for k in range(nd):
            if k < len(TAILF) - 1:
                take(TAILF[k])
            emit_pv(slot)
            slot += 1
        take(len(tail))
        run_posts(10**9)
        if first:
            _wait("xr1", xr1)

    def sc(kind):
        def f():
            if SCOPES:
                with jax.named_scope(kind):
                    body(kind)
            else:
                body(kind)
        return f
    pl.when(step == 0)(sc("first"))
    pl.when(jnp.logical_and(step > 0, step < 4))(sc("mid"))
    pl.when(step == 4)(sc("last"))


@jax.jit
def pallas_concat_heads__sliding_block__sliding_block__prompt_kernel(A_x, A_wqkv, A_wo, B_x, B_wqkv, B_wo):
    xa = A_x.reshape(S, D).T
    xb = B_x.reshape(S, D).T
    V = pltpu.VMEM
    two = lambda shp, dt: [V(shp, dt), V(shp, dt)]
    out = pl.pallas_call(
        kernel,
        grid=(5,),
        in_specs=[pl.BlockSpec(memory_space=pl.ANY)] * 6,
        out_specs=pl.BlockSpec(memory_space=pl.ANY),
        out_shape=jax.ShapeDtypeStruct((S, 2*D), bf16),
        scratch_shapes=([V((4, D, 512), bf16), V((5, D, 512), bf16)] + two((D, 3*D), bf16) + two((D, D), bf16)
                        + two((3*D // 2, D), u32) + two((D // 2, D), u32)
                        + two((256, 512), u32) + two((256, 512), u32)
                        + two((D // 2, 512), u32) + two((D // 2, 512), u32)
                        + [V((4, 64, 128), u32), V((4, 192, 128), f32), V((4, 56, 128), u32)]
                        + [V((1, 256, 128), f32)] * 8 + [V((S + 16, 2*D), bf16),
                           pltpu.SemaphoreType.DMA((18,)),
                           pltpu.SemaphoreType.DMA((1,))]),
        compiler_params=pltpu.CompilerParams(dimension_semantics=("arbitrary",), vmem_limit_bytes=100*1024*1024),
    )(xa, xb, A_wqkv, A_wo, B_wqkv, B_wo)
    return out.reshape(1, S, 2*D)
```

```python
import math
import jax, jax.numpy as jnp
from jax import lax
import jax.experimental.pallas as pl
import jax.experimental.pallas.tpu as pltpu

S, D, H, DH, W = 2048, 448, 16, 28, 256
NT = S // 128
NEG = -1e30
QSCALE = (DH ** -0.5) * math.log2(math.e)
f32, bf16, i32, u32 = jnp.float32, jnp.bfloat16, jnp.int32, jnp.uint32
HI = 0xFFFF0000
WCH = (0,384,640,1344)
XA1 = 1
BUD = (6,11)
NVT = 2
NHB = 2
WBSLOT = 29
LA = 60
LB = 62
TONLY = 1
NDEF = 3
NPRE = 1
FPIECES = ((384,512),(512,768),(768,896))
NT0 = 2
PARAMS = {
    "first": dict(FENCE=0, PDELAY=4, DELAY=4, PVOFF=(0, 0, 1), SSTAGE=3, SPEC=0, NSB=4, ORDER=1, TAILF=(1, 1, 1, 1, 2)),
    "mid": dict(FENCE=32, PDELAY=12, DELAY=4, PVOFF=(0, 0, 0), SSTAGE=4, SPEC=1, NSB=8, ORDER=1, TAILF=(2, 1, 0, 0, 2)),
    "last": dict(FENCE=4, PDELAY=8, DELAY=3, PVOFF=(0, 1, 1), SSTAGE=4, SPEC=1, NSB=8, ORDER=1, TAILF=(1, 1, 1, 1, 2)),
}
SIMIN = 2
FB1 = 48
L1 = 18
L2 = 50
TFENCE = 1
NOSEM = 1
NOBND = 1
UNIF = 1
OPOS = 1
PORD = (1,0,2)
SCOPES = 0


def _iota(shape, dim):
    return lax.broadcasted_iota(i32, shape, dim)


def _w(x):
    return pltpu.bitcast(x, u32)


def _b(x):
    return pltpu.bitcast(x, bf16)


def _pack(a, b):
    ua = lax.bitcast_convert_type(a, u32)
    ub = lax.bitcast_convert_type(b, u32)
    return (ua >> 16) | (ub & jnp.uint32(HI))


def _split(n, flip):
    parts = [n // 4 + (1 if k < n % 4 else 0) for k in range(4)]
    if flip:
        parts = parts[::-1]
    return [p for p in parts if p]


def _wait(name, cps):
    if SCOPES:
        with jax.named_scope(name):
            for cp in cps:
                cp.wait()
    else:
        for cp in cps:
            cp.wait()


def kernel(xa_hbm, xb_hbm, wa_hbm, woa_hbm, wb_hbm, wob_hbm, o_hbm,
           xa_s, xb_s, wa_s, wb_s, woa_s, wob_s, wta_s, wtb_s, wota_s, wotb_s,
           ka_s, kb_s, vta_s, vtb_s, qta_s, qtb_s, ota_s, otb_s, omid_s, mq_s,
           s0_s, s1_s, s2_s, s3_s, s4_s, s5_s, s6_s, s7_s, o_s, wsem, osem):
    step = pl.program_id(0)
    x_hbm, x_s = (xa_hbm, xb_hbm), (xa_s, xb_s)
    wt_s, wot_s = (wta_s, wtb_s), (wota_s, wotb_s)
    k_s, vt_s, qt_s, ot_s = (ka_s, kb_s), (vta_s, vtb_s), (qta_s, qtb_s), (ota_s, otb_s)

    def xcopy(b, lo, hi, k):
        j, o = divmod(lo + 256 * b, 512)
        return pltpu.make_async_copy(x_hbm[b].at[:, lo:hi], x_s[b].at[j, :, o:o + hi - lo], wsem.at[8 + k])

    def ocopy(row, c0=0, c1=2 * D):
        return pltpu.make_async_copy(o_s.at[pl.ds(row, 128), c0:c1], o_hbm.at[pl.ds(row, 128), c0:c1], osem.at[0])

    nwa = len(WCH) - 1
    wa_copies = [pltpu.make_async_copy(wa_hbm.at[:, WCH[i]:WCH[i + 1]], wa_s.at[:, WCH[i]:WCH[i + 1]], wsem.at[i])
                 for i in range(nwa)]
    wb_copy = pltpu.make_async_copy(wb_hbm, wb_s, wsem.at[nwa])
    woa_copy = pltpu.make_async_copy(woa_hbm, woa_s, wsem.at[nwa + 1])
    wob_copy = pltpu.make_async_copy(wob_hbm, wob_s, wsem.at[nwa + 2])
    xa0, xa1, xb0 = xcopy(0, 0, 256, 0), xcopy(0, 256, 512, 1), xcopy(1, 0, 256, 2)
    xr1 = [xcopy(1, 256, 768, 3), xcopy(0, 512, 1024, 4)]
    xr2 = [xcopy(1, 768, 1280, 5), xcopy(0, 1024, 1536, 6), xcopy(1, 1280, 1792, 7), xcopy(0, 1536, 2048, 8),
           xcopy(1, 1792, 2048, 9)]

    def body(kind):
        first, last = kind == "first", kind == "last"
        P = PARAMS[kind]
        FENCE, PDELAY, DELAY, PVOFF, SSTAGE, SPEC, NSB, ORDER, TAILF = (
            P[k] for k in ("FENCE", "PDELAY", "DELAY", "PVOFF", "SSTAGE", "SPEC", "NSB", "ORDER", "TAILF"))
        us = {"first": (0, 1), "mid": (2, 3, 4, 5), "last": (14, 15)}[kind]
        r32 = _iota((32, 128), 0)
        keyidx = jnp.where(r32 < 16, 2 * r32, 2 * r32 - 31)
        tri = keyidx <= (_iota((32, 128), 1) & 31)
        lane16 = _iota((16, 128), 1)
        sel1 = (lane16 & 32) == 0
        sel2 = (lane16 & 64) == 0
        lo4 = _iota((8, 128), 0) < 4
        zero = jnp.zeros((16, 128), u32)
        xcache = {}
        scnt = [0]
        ss_s = (s0_s, s1_s, s2_s, s3_s, s4_s, s5_s, s6_s, s7_s)
        zdyn = step // 8

        def gtok(q, dyn=False):
            if kind == "mid":
                return pl.multiple_of((step - 1) * 512 + 128 * q, 128)
            if dyn and FENCE:
                return pl.multiple_of(zdyn * 128 + 128 * q, 128)
            return 128 * q

        q0 = 2 * (us[0] // 2)
        have = {}
        if not first:
            for b in range(2):
                for t in range(4):
                    for q in range(q0 - 2, q0 + (2 if b == 0 else 0)):
                        for kd in "qkv":
                            have[kd, b, q % 4, t] = q
                    for q in range(q0 - 2, q0):
                        have["o", b, q % 4, t] = q
            for q in range(q0 - 2, q0):
                have["m", 0, q % 4, 2] = have["m", 0, q % 4, 3] = q

        def made(kd, b, q, t):
            have[kd, b, q % 4, t] = q

        def need(kd, b, q, t):
            assert have.get((kd, b, q % 4, t)) == q, (kind, kd, b, q, t, have.get((kd, b, q % 4, t)))

        cur = [0]
        posts = []

        def later(th):
            posts.append((cur[0] + PDELAY, th))

        def run_posts(upto):
            while posts and posts[0][0] <= upto:
                posts.pop(0)[1]()

        def ring(q):
            return slice(128 * (q % 4), 128 * (q % 4) + 128)

        def proj(b, q, part, t, defer=None):
            r0 = part * (D // 2) + 56 * t
            if (b, q) not in xcache:
                j, o = divmod(128 * q + 256 * b, 512)
                xcache[b, q] = x_s[b][j + step - 1 if kind == "mid" else j, :, o:o + 128]
            xt = xcache[b, q]
            y = jnp.dot(_b(wt_s[b][r0:r0 + 56, :]), xt, preferred_element_type=f32)
            if defer is not None:
                defer.append(lambda: ppost(b, q, part, t, y))
            else:
                ppost(b, q, part, t, y)

        def ppost(b, q, part, t, y):
            made("qkv"[part], b, q, t)
            if part == 0:
                y = y * QSCALE
                r1 = pltpu.roll(y[24:56], 96, 1)
                r2 = pltpu.roll(y[56:88], 64, 1)
                r3 = pltpu.roll(y[80:112], 32, 1)
                qr = jnp.concatenate([
                    y[0:24], jnp.where(lo4, y[24:32], r1[0:8]), r1[8:32],
                    r2[0:24], jnp.where(lo4, r2[24:32], r3[0:8]), r3[8:32]], axis=0)
                qt_s[b][56*t:56*t + 56, ring(q)] = _w(qr.astype(bf16))
            elif part == 1:
                kt = jnp.concatenate([y, jnp.zeros((16, 128), f32)], axis=0)
                kw = _w(kt.astype(bf16).T)
                ev = _w(lax.bitcast_convert_type(kw << 16, f32).astype(bf16))
                od = _w(lax.bitcast_convert_type(kw & jnp.uint32(HI), f32).astype(bf16))
                kk = jnp.concatenate([z[8*i:8*i + 8] for i in range(4) for z in (ev, od)], axis=0)
                k_s[b][64*(q % 4):64*(q % 4) + 64, 128*t:128*t + 128] = kk
            else:
                v = jnp.concatenate([
                    y[0:24], jnp.where(lo4, y[24:32], 1.0), jnp.where(lo4, 1.0, y[24:32]), y[32:56],
                    y[56:80], jnp.where(lo4, y[80:88], 1.0), jnp.where(lo4, 1.0, y[80:88]), y[88:112]], axis=0)
                vt_s[b][64*t:64*t + 64, ring(q)] = _w(v.astype(bf16))

        def kload(b, t, off, n):
            lo = off % 256
            if lo + n <= 256:
                return k_s[b][lo:lo + n, 128*t:128*t + 128]
            return jnp.concatenate([k_s[b][lo:256, 128*t:128*t + 128],
                                    k_s[b][0:lo + n - 256, 128*t:128*t + 128]], axis=0)

        def qk(b, q, t, c):
            imin = max(0, 8 - 4 * q - c)
            need("q", b, q, t)
            for qq in range(max(0, q - 2), q + 1):
                need("k", b, qq, t)
            q32 = qt_s[b][56*t:56*t + 56, ring(q)]
            if FENCE and not first and (cur[0] % FENCE == 0):
                ztail = fence_zero()
            else:
                ztail = zero[0:8]
            w = _b(jnp.concatenate([q32 & mq_s[c], ztail], axis=0))
            off = 64 * q + 16 * c - 128
            if imin == 0 and SPEC:
                sizes = (4, 4, 3, 3) if c % 2 == 0 else (3, 3, 4, 4)
                plan, o = [], 2
                for k, n in enumerate(sizes):
                    mids = list(range(o, o + n))
                    sp = (0, 16, 1, 17)[k]
                    plan.append(mids + [sp] if SPEC == 1 else [sp] + mids)
                    o += n
            else:
                plan, o = [], 2 * imin
                for n in _split(2 * (9 - imin), c % 2):
                    plan.append(list(range(o, o + n)))
                    o += n
            ch = {}
            for us_ in plan:
                runs = []
                for u in us_:
                    if runs and runs[-1][0] + runs[-1][1] == u:
                        runs[-1][1] += 1
                    else:
                        runs.append([u, 1])
                kw = [kload(b, t, off + 8 * u, 8 * n) for u, n in runs]
                kw = kw[0] if len(kw) == 1 else jnp.concatenate(kw, axis=0)
                z = jnp.dot(_b(kw), w, preferred_element_type=f32)
                for k, u in enumerate(us_):
                    ch[u] = z[16*k:16*k + 16]

            def blk(i):
                return jnp.concatenate([ch[2*i], ch[2*i + 1]], axis=0)
            sm = jnp.where(tri, blk(8), blk(0) if imin == 0 else NEG)
            mx = sm
            for i in range(max(imin, 1), 8):
                mx = jnp.maximum(mx, blk(i))
            m = jnp.max(mx, axis=0, keepdims=True)
            if SSTAGE and imin <= SIMIN:
                sref = ss_s[scnt[0] % NSB]
                scnt[0] += 1
                early = [u for us_ in plan for u in us_[:min(SSTAGE, len(us_) - 1)] if 2 <= u < 16]
                for u in early:
                    sref[0, 16*u:16*u + 16, :] = ch[u]
                if SPEC == 2 and imin == 0:
                    sref[0, 0:32, :] = sm
                    sm = sref[zdyn, 0:32, :]
                for u in early:
                    ch[u] = sref[zdyn, 16*u:16*u + 16, :]
            pm = jnp.exp2(sm - m)
            X = [None] * 9
            for i in range(max(imin, 1), 8):
                p = jnp.exp2(blk(i) - m)
                X[i] = _pack(p[0:16], p[16:32])
            if imin == 0:
                pf = jnp.where(tri, 0.0, pm)
                X[0] = _pack(pf[0:16], pf[16:32])
                pm = jnp.where(tri, pm, 0.0)
            X[8] = _pack(pm[0:16], pm[16:32])
            return X

        def fence_zero():
            return _w(o_s[pl.ds(pl.multiple_of(S + 16 * zdyn, 16), 16), 0:128])

        def pv(b, q, t, X, T, acc):
            if q + T < 2:
                return acc
            for j in range(4):
                need("v", b, q + T - 2, t)
            zz = zero
            if last and (b, q, t) == (1, NT - 1, 0) and T == TFENCE - 1:
                fz = fence_zero()
                zz = jnp.concatenate([fz, fz], axis=0)

            def sel(m, a, bb):
                if a is None and bb is None:
                    return None
                return jnp.where(m, zz if a is None else a, zz if bb is None else bb)
            Y = [[] for _ in range(4)]
            for B in range(4*T, 4*T + 4):
                xs = [X[c][B - c] if 0 <= B - c <= 8 else None for c in range(4)]
                a = [sel(sel1, xs[k], xs[(k + 1) % 4]) for k in range(4)]
                for j in range(4):
                    y = sel(sel2, a[j], a[(j + 2) % 4])
                    Y[j].append(zero if y is None else y)
            res = []
            for j in range(4):
                h = 4*t + j
                p = _b(jnp.concatenate(Y[j], axis=0))
                vt = _b(vt_s[b][16*h:16*h + 16, ring(q + T - 2)])
                o = jnp.dot(vt, p, preferred_element_type=f32)
                res.append(o if acc is None else o + acc[j])
            return res

        def fin(b, q, t, acc):
            made("o", b, q, t)
            outs = []
            for j in range(4):
                o = acc[j]
                den = o[28:29] if j % 2 == 0 else o[0:1]
                o = o * (1.0 / den)
                if j:
                    o = pltpu.roll(o, 32*j, 1)
                outs.append(o)
            oc = jnp.concatenate([
                outs[0][0:24], jnp.where(lo4, outs[0][24:32], outs[1][0:8]), outs[1][8:32],
                outs[2][0:24], jnp.where(lo4, outs[2][24:32], outs[3][0:8]), outs[3][8:32]], axis=0)
            ot_s[b][56*t:56*t + 56, ring(q)] = _w(oc.astype(bf16))

        ohold = {}

        def put(q, c0, c1, val):
            row = gtok(q, dyn=True)
            o_s[pl.ds(row, 128), c0:c1] = val.astype(bf16).T
            if q == NT - 1:
                ocopy(row, c0, c1).start()
            elif c1 == 2 * D:
                ocopy(row).start()

        def outp(b, q, n):
            for t in range(4):
                need("o", b, q, t)
            r0, r1 = ((0, 128, 256, 384, 448) if b == 0 else (0, 64, 192, 320, 448))[n:n + 2]
            y = jnp.dot(_b(wot_s[b][r0 // 2:r1 // 2, :]), _b(ot_s[b][:, ring(q)]),
                        preferred_element_type=f32)

            def post():
                if b == 0:
                    if n == 0:
                        ohold[q] = y
                    elif n == 1:
                        put(q, 0, 256, jnp.concatenate([ohold.pop(q), y], axis=0))
                    elif n == 2 and q == NT - 1:
                        put(q, 256, 384, y)
                    else:
                        made("m", 0, q, n)
                        omid_s[q % 4, 128 * (n - 2):r1 - 256] = y
                else:
                    if n == 0:
                        need("m", 0, q, 2)
                        need("m", 0, q, 3)
                        put(q, 256, 512, jnp.concatenate([omid_s[q % 4], y], axis=0))
                    elif n == 1:
                        ohold[q] = y
                    elif n == 2:
                        put(q, 512, 768, jnp.concatenate([ohold.pop(q), y], axis=0))
                    else:
                        put(q, 768, 896, y)
            later(post)

        def final_out():
            q = NT - 1
            for t in range(4):
                need("o", 1, q, t)
            need("m", 0, q, 3)
            parts = []
            for k0, k1 in ((128, D), (0, 128)):
                rhs = _b(ot_s[1][k0 // 2:k1 // 2, ring(q)])
                ys = [jnp.dot(_b(wot_s[1][56*n:56*n + 56, k0:k1]), rhs, preferred_element_type=f32) for n in range(4)]
                parts = [y + p for y, p in zip(ys, parts)] if parts else ys
            y = jnp.concatenate([omid_s[q % 4, 128:192]] + parts, axis=0)
            for c0, c1 in FPIECES:
                put(q, c0, c1, y[c0 - 384:c1 - 384])

        def wtile(src, dst, i, ncol):
            c0, c1 = 128 * i, min(128 * i + 128, ncol)
            dst[c0 // 2:c1 // 2, :] = _w(src[:, c0:c1].T)

        def projs(u, order=(1, 0, 2)):
            s, b = divmod(u, 2)
            return [(lambda p=p, t=t, q=q: proj(b, q, p, t))
                    for p in order for q in (2*s, 2*s + 1) for t in range(4)]

        def outs(u, qi):
            s, b = divmod(u, 2)
            return [(lambda n=n: outp(b, 2*s + qi, n)) for n in range(4)]

        groups = [(u % 2, 2 * (u // 2) + qi, t) for u in us for qi in range(2) for t in range(4)]
        if last:
            groups = ([(0, 14, t) for t in range(4)] + [(1, 14, t) for t in range(4)]
                      + [(0, 15, t) for t in range(4)] + [(1, 15, t) for t in (3, 2, 1, 0)])
        N = len(groups)
        Xs = [[None] * 4 for _ in range(N)]
        accs = [None] * N

        def emit_pv(slot):
            for T in range(3):
                r = slot - 3 - DELAY - PVOFF[T]
                if r >= 0 and r % 4 == 0 and r // 4 < N:
                    g = r // 4
                    accs[g] = pv(*groups[g], Xs[g], T, accs[g])
                    if T == 2:
                        fin(*groups[g], accs[g])
                        Xs[g] = accs[g] = None

        fill = {}

        def spread(thunks, lo, hi):
            n = len(thunks)
            for k, th in enumerate(thunks):
                fill.setdefault(lo + (k * (hi - lo)) // n, []).append(th)

        NTL = sum(TAILF)
        if first:
            for i in range(nwa):
                wa_copies[i].start()
                if i == 0:
                    xa0.start()
                if i == XA1:
                    xa1.start()
            wb_copy.start()
            xb0.start()
            woa_copy.start()
            wob_copy.start()
            r = _iota((56, 128), 0) // 14
            l = _iota((56, 128), 1) // 32
            o_s[S:S + 16, :] = jnp.zeros((16, 2 * D), bf16)
            for c in range(4):
                mq_s[c] = jnp.where(r == ((c - l) & 3), jnp.uint32(0xFFFFFFFF), jnp.uint32(0))
            todo = [(q, part, t) for q in range(4) for part in range(3) for t in range(4)]
            held = []

            def flush():
                while held:
                    held.pop(0)()
            for i in range(nwa):
                tiles = range(WCH[i] // 128, (WCH[i + 1] + 127) // 128)
                if i == 0 and TONLY:
                    _wait("wt", [wa_copies[0]])
                    for ti in tiles[:NT0]:
                        wtile(wa_s, wta_s, ti, 3 * D)
                    _wait("w0", [xa0] + ([xa1] if XA1 == 0 else []))
                    for ti in tiles[NT0:]:
                        wtile(wa_s, wta_s, ti, 3 * D)
                else:
                    _wait(f"w{i}", [wa_copies[i]] + ([xa0] if i == 0 else []) + ([xa1] if i == XA1 else []))
                    for ti in tiles:
                        wtile(wa_s, wta_s, ti, 3 * D)
                flush()
                if i == nwa - 1:
                    for cp in xr1 + xr2:
                        cp.start()
                nq = 4 if i >= XA1 else 2
                avail = [p for p in todo if p[0] < nq and p[1] * D + 112 * p[2] + 112 <= WCH[i + 1]]
                avail.sort(key=lambda p: (p[1] * D + 112 * p[2], p[0]))
                if i < nwa - 1:
                    avail = avail[:BUD[i]]
                else:
                    old = [p for p in avail if p[1] * D + 112 * p[2] + 112 <= WCH[i]]
                    extra = [p for p in old if p[0] >= 2][:max(0, 2 - len([p for p in old if p[0] < 2]))]
                    avail = [p for p in avail if p[0] < 2 or p in extra]
                for k, p in enumerate(avail):
                    proj(0, *p, defer=held if (i < nwa - 1 and k >= len(avail) - NDEF) else None)
                    todo.remove(p)
            todo.sort(key=lambda p: ((1, 0, 2).index(p[1]), p[0], p[2]))

            def wb_prep():
                _wait("wb", [wb_copy, xb0, woa_copy, wob_copy])
                flush()
                for ti in range(11):
                    wtile(wb_s, wtb_s, ti, 3 * D)
                for ti in range(4):
                    wtile(woa_s, wota_s, ti, D)
                    wtile(wob_s, wotb_s, ti, D)
            nk = NPRE + NHB + NVT
            n2 = len(todo)
            p2 = [(lambda p=p, k=k: proj(0, *p, defer=held if n2 - nk <= k < n2 - nk + NPRE else None))
                  for k, p in enumerate(todo)]
            spread(p2[:n2 - nk], 0, WBSLOT)
            spread(p2[n2 - nk:n2 - nk + NPRE], WBSLOT, WBSLOT + 1)
            fill.setdefault(WBSLOT, []).append(wb_prep)
            spread(p2[n2 - NHB - NVT:n2 - NVT], WBSLOT, WBSLOT + 1)
            pb = [[(lambda p=p, t=t, q=q: proj(1, q, p, t)) for p in order for t in range(4)]
                  for q, order in ((0, (0, 1, 2)), (1, (1, 0, 2)))]
            spread(pb[0], WBSLOT + 1, 32)
            spread(pb[1], 32, FB1)
            rest = outs(0, 0) + outs(0, 1) + p2[len(p2) - NVT:]
            spread(rest[:len(rest) - NTL], FB1, 64)
            tail = rest[len(rest) - NTL:]
        elif not last:
            @pl.when(step == 2)
            def _():
                for cp in xr2:
                    cp.wait()
            for k, u in enumerate(us):
                base = 32 * k
                p = projs(u + 1, PORD)
                if u == us[-1]:
                    p, tail = p[:24 - NTL], p[24 - NTL:]
                o = outs(u - 1, 0) + outs(u - 1, 1)
                if UNIF:
                    ps = [s for s in range(32) if s % 4 != OPOS]
                    for i, th in enumerate(p):
                        fill.setdefault(base + ps[(i * 24) // len(p)], []).append(th)
                    for i, th in enumerate(o):
                        fill.setdefault(base + 4 * i + OPOS, []).append(th)
                else:
                    spread(p, base, base + 30)
                    spread(o, base + (8 if k else 0), base + 32)
        else:
            pb = [[(lambda p=p, t=t, q=q: proj(1, q, p, t)) for p in (1, 0, 2) for t in range(4)] for q in (14, 15)]
            spread(pb[0], 0, L1)
            spread(outs(13, 0) + outs(13, 1) + pb[1], L1, L2)
            oa = outs(14, 1)
            spread(outs(14, 0) + outs(15, 0), L2, LA)
            spread(oa[:2], LA, LB)
            tail = oa[2:]

        slot = 0
        for g in range(N):
            for c in range(4):
                cur[0] = slot
                run_posts(slot)
                Xs[g][c] = qk(*groups[g], c)
                if ORDER == 1:
                    emit_pv(slot)
                for th in fill.get(slot, []):
                    th()
                if ORDER == 0:
                    emit_pv(slot)
                slot += 1

        def take(n):
            for _ in range(n):
                th = tail.pop(0)
                if th is not None:
                    th()
        nd = DELAY + max(PVOFF)
        if last:
            run_posts(10**9)
            take(len(tail))
            for k in range(nd):
                emit_pv(slot)
                slot += 1
            run_posts(10**9)
            final_out()
            _wait("ow", [ocopy(128 * q) for q in range(NT - 1)]
                  + [ocopy(128 * (NT - 1), c0, c1) for c0, c1 in ((0, 256), (256, 384)) + FPIECES])
            return
        for k in range(nd):
            if k < len(TAILF) - 1:
                take(TAILF[k])
            emit_pv(slot)
            slot += 1
        take(len(tail))
        run_posts(10**9)
        if first:
            _wait("xr1", xr1)

    def sc(kind):
        def f():
            if SCOPES:
                with jax.named_scope(kind):
                    body(kind)
            else:
                body(kind)
        return f
    pl.when(step == 0)(sc("first"))
    pl.when(jnp.logical_and(step > 0, step < 4))(sc("mid"))
    pl.when(step == 4)(sc("last"))


@jax.jit
def pallas_concat_heads__sliding_block__sliding_block__prompt_kernel(A_x, A_wqkv, A_wo, B_x, B_wqkv, B_wo):
    xa = A_x.reshape(S, D).T
    xb = B_x.reshape(S, D).T
    V = pltpu.VMEM
    two = lambda shp, dt: [V(shp, dt), V(shp, dt)]
    out = pl.pallas_call(
        kernel,
        grid=(5,),
        in_specs=[pl.BlockSpec(memory_space=pl.ANY)] * 6,
        out_specs=pl.BlockSpec(memory_space=pl.ANY),
        out_shape=jax.ShapeDtypeStruct((S, 2*D), bf16),
        scratch_shapes=([V((4, D, 512), bf16), V((5, D, 512), bf16)] + two((D, 3*D), bf16) + two((D, D), bf16)
                        + two((3*D // 2, D), u32) + two((D // 2, D), u32)
                        + two((256, 512), u32) + two((256, 512), u32)
                        + two((D // 2, 512), u32) + two((D // 2, 512), u32)
                        + [V((4, 192, 128), f32), V((4, 56, 128), u32)]
                        + [V((1, 256, 128), f32)] * 8 + [V((S + 16, 2*D), bf16),
                           pltpu.SemaphoreType.DMA((18,)),
                           pltpu.SemaphoreType.DMA((1,))]),
        compiler_params=pltpu.CompilerParams(dimension_semantics=("arbitrary",), vmem_limit_bytes=100*1024*1024,
                                             disable_semaphore_checks=bool(NOSEM), disable_bounds_checks=bool(NOBND)),
    )(xa, xb, A_wqkv, A_wo, B_wqkv, B_wo)
    return out.reshape(1, S, 2*D)
```

```python
import math

import jax
import jax.numpy as jnp
from jax import lax
import jax.experimental.pallas as pl
import jax.experimental.pallas.tpu as pltpu

S, D, H, DH, W = 2048, 448, 16, 28, 256
NT = S // 128
NEG = -1e30
QSCALE = (DH ** -0.5) * math.log2(math.e)
f32, bf16, i32, u32 = jnp.float32, jnp.bfloat16, jnp.int32, jnp.uint32
HI = 0xFFFF0000

STAGES = ((128, 1, 1), (256, 2, 3), (384, 3, 5), (640, 4, 11), (1344, 4, 2))
WBSLOT, FB1, NDEF = 38, 64, 2
LA, LB = 25, 28
OPOS = 1
SIMIN = 2
NSTAGE_BUFS = 8
FPIECES = ((384, 512), (512, 768), (768, 896))
PARAMS = {
    "first": dict(FENCE=0, PDELAY=8, DELAY=3, PVOFF=(0, 1, 1), SSTAGE=3, NSB=6, TAILF=(2, 1, 0, 0, 3)),
    "mid": dict(FENCE=0, PDELAY=12, DELAY=4, PVOFF=(0, 0, 0), SSTAGE=4, NSB=6, TAILF=(2, 1, 0, 0, 2)),
    "last": dict(FENCE=8, PDELAY=8, DELAY=3, PVOFF=(0, 0, 1), SSTAGE=4, NSB=8, TAILF=()),
}


def _iota(shape, dim):
    return lax.broadcasted_iota(i32, shape, dim)


def _w(x):
    return pltpu.bitcast(x, u32)


def _b(x):
    return pltpu.bitcast(x, bf16)


def _pack(a, b):
    ua = lax.bitcast_convert_type(a, u32)
    ub = lax.bitcast_convert_type(b, u32)
    return (ua >> 16) | (ub & jnp.uint32(HI))


def _split(n, flip):
    parts = [n // 4 + (1 if k < n % 4 else 0) for k in range(4)]
    if flip:
        parts = parts[::-1]
    return [p for p in parts if p]


def _wait(copies):
    for cp in copies:
        cp.wait()


def _kernel(xa_hbm, xb_hbm, wa_hbm, woa_hbm, wb_hbm, wob_hbm, o_hbm,
            xa_s, xb_s, wa_s, wb_s, woa_s, wob_s, wta_s, wtb_s, wota_s, wotb_s,
            ka_s, kb_s, vta_s, vtb_s, qta_s, qtb_s, ota_s, otb_s, omid_s, mq_s,
            s0_s, s1_s, s2_s, s3_s, s4_s, s5_s, s6_s, s7_s, o_s, isem, osem):
    step = pl.program_id(0)
    x_hbm, x_s = (xa_hbm, xb_hbm), (xa_s, xb_s)
    wt_s, wot_s = (wta_s, wtb_s), (wota_s, wotb_s)
    k_s, vt_s, qt_s, ot_s = (ka_s, kb_s), (vta_s, vtb_s), (qta_s, qtb_s), (ota_s, otb_s)
    ss_s = (s0_s, s1_s, s2_s, s3_s, s4_s, s5_s, s6_s, s7_s)

    nsem = [0]

    def icopy(src, dst):
        nsem[0] += 1
        return pltpu.make_async_copy(src, dst, isem.at[nsem[0] - 1])

    def xcopy(b, lo, hi):
        j, o = divmod(lo, 512)
        return icopy(x_hbm[b].at[:, lo:hi], x_s[b].at[j, :, o:o + hi - lo])

    def ocopy(row, c0=0, c1=2 * D):
        return pltpu.make_async_copy(o_s.at[pl.ds(row, 128), c0:c1], o_hbm.at[pl.ds(row, 128), c0:c1], osem.at[0])

    stage_w, stage_x = [], []
    pw = pq = 0
    for cw, cq, _ in STAGES:
        stage_w.append([icopy(wa_hbm.at[:, pw:cw], wa_s.at[:, pw:cw])] if cw > pw else [])
        stage_x.append([xcopy(0, 128 * pq, 128 * cq)] if cq > pq else [])
        pw, pq = cw, cq
    bcopies = [icopy(wb_hbm, wb_s), xcopy(1, 0, 512), icopy(woa_hbm, woa_s), icopy(wob_hbm, wob_s)]
    xr1 = [xcopy(0, 512, 1024), xcopy(1, 512, 1024)]
    xr2 = [xcopy(0, 1024, 1536), xcopy(1, 1024, 1536), xcopy(0, 1536, 2048), xcopy(1, 1536, 2048)]

    def body(kind):
        first, last = kind == "first", kind == "last"
        prm = PARAMS[kind]
        FENCE, PDELAY, DELAY, PVOFF, SSTAGE, NSB, TAILF = (
            prm[k] for k in ("FENCE", "PDELAY", "DELAY", "PVOFF", "SSTAGE", "NSB", "TAILF"))
        us = {"first": (0, 2, 1), "mid": (3, 4, 5, 6), "last": (15,)}[kind]
        r32 = _iota((32, 128), 0)
        keyidx = jnp.where(r32 < 16, 2 * r32, 2 * r32 - 31)
        tri = keyidx <= (_iota((32, 128), 1) & 31)
        lane16 = _iota((16, 128), 1)
        sel1 = (lane16 & 32) == 0
        sel2 = (lane16 & 64) == 0
        lo4 = _iota((8, 128), 0) < 4
        zero = jnp.zeros((16, 128), u32)
        xcache = {}
        scnt = [0]
        zdyn = step // 8

        def orow(q):
            if kind == "mid":
                return pl.multiple_of((step - 1) * 512 + 128 * q, 128)
            if FENCE:
                return pl.multiple_of(zdyn * 128 + 128 * q, 128)
            return 128 * q

        q0 = 2 * (us[0] // 2)
        have = {}
        if not first:
            for t in range(4):
                for q in range(q0 - 2, q0 + 2):
                    for b in range(2):
                        for kd in "qkv":
                            have[kd, b, q % 4, t] = q
                for q in range(q0 - 2, q0):
                    have["o", 1, q % 4, t] = q
                    have["o", 0, (q + 2) % 4, t] = q + 2
            for q in range(q0 - 2, q0):
                have["m", 0, q % 4, 2] = have["m", 0, q % 4, 3] = q

        def made(kd, b, q, t):
            have[kd, b, q % 4, t] = q

        def need(kd, b, q, t):
            assert have.get((kd, b, q % 4, t)) == q, (kind, kd, b, q, t)

        cur = [0]
        posts = []

        def later(th):
            posts.append((cur[0] + PDELAY, th))

        def run_posts(upto):
            while posts and posts[0][0] <= upto:
                posts.pop(0)[1]()

        def ring(q):
            return slice(128 * (q % 4), 128 * (q % 4) + 128)

        def proj(b, q, part, t, defer=None):
            r0 = part * (D // 2) + 56 * t
            if (b, q) not in xcache:
                j, o = divmod(128 * q, 512)
                xcache[b, q] = x_s[b][j + step - 1 if kind == "mid" else j, :, o:o + 128]
            xt = xcache[b, q]
            y = jnp.dot(_b(wt_s[b][r0:r0 + 56, :]), xt, preferred_element_type=f32)
            if defer is not None:
                defer.append(lambda: proj_post(b, q, part, t, y))
            else:
                proj_post(b, q, part, t, y)

        def proj_post(b, q, part, t, y):
            made("qkv"[part], b, q, t)
            if part == 0:
                y = y * QSCALE
                r1 = pltpu.roll(y[24:56], 96, 1)
                r2 = pltpu.roll(y[56:88], 64, 1)
                r3 = pltpu.roll(y[80:112], 32, 1)
                qr = jnp.concatenate([
                    y[0:24], jnp.where(lo4, y[24:32], r1[0:8]), r1[8:32],
                    r2[0:24], jnp.where(lo4, r2[24:32], r3[0:8]), r3[8:32]], axis=0)
                qt_s[b][56*t:56*t + 56, ring(q)] = _w(qr.astype(bf16))
            elif part == 1:
                kt = jnp.concatenate([y, jnp.zeros((16, 128), f32)], axis=0)
                kw = _w(kt.astype(bf16).T)
                ev = _w(lax.bitcast_convert_type(kw << 16, f32).astype(bf16))
                od = _w(lax.bitcast_convert_type(kw & jnp.uint32(HI), f32).astype(bf16))
                kk = jnp.concatenate([z[8*i:8*i + 8] for i in range(4) for z in (ev, od)], axis=0)
                k_s[b][64*(q % 4):64*(q % 4) + 64, 128*t:128*t + 128] = kk
            else:
                v = jnp.concatenate([
                    y[0:24], jnp.where(lo4, y[24:32], 1.0), jnp.where(lo4, 1.0, y[24:32]), y[32:56],
                    y[56:80], jnp.where(lo4, y[80:88], 1.0), jnp.where(lo4, 1.0, y[80:88]), y[88:112]], axis=0)
                vt_s[b][64*t:64*t + 64, ring(q)] = _w(v.astype(bf16))

        def kload(b, t, off, n):
            lo = off % 256
            if lo + n <= 256:
                return k_s[b][lo:lo + n, 128*t:128*t + 128]
            return jnp.concatenate([k_s[b][lo:256, 128*t:128*t + 128],
                                    k_s[b][0:lo + n - 256, 128*t:128*t + 128]], axis=0)

        def fence_zero():
            return _w(o_s[pl.ds(pl.multiple_of(S + 16 * zdyn, 16), 16), 0:128])

        def qk(b, q, t, c):
            imin = max(0, 8 - 4 * q - c)
            need("q", b, q, t)
            for qq in range(max(0, q - 2), q + 1):
                need("k", b, qq, t)
            q32 = qt_s[b][56*t:56*t + 56, ring(q)]
            ztail = fence_zero() if FENCE and cur[0] % FENCE == 0 else zero[0:8]
            w = _b(jnp.concatenate([q32 & mq_s[c], ztail], axis=0))
            off = 64 * q + 16 * c - 128
            if imin == 0:
                plan, o = [], 2
                for k, n in enumerate((4, 4, 3, 3) if c % 2 == 0 else (3, 3, 4, 4)):
                    plan.append(list(range(o, o + n)) + [(0, 16, 1, 17)[k]])
                    o += n
            else:
                plan, o = [], 2 * imin
                for n in _split(2 * (9 - imin), c % 2):
                    plan.append(list(range(o, o + n)))
                    o += n
            ch = {}
            for chunks in plan:
                runs = []
                for u in chunks:
                    if runs and runs[-1][0] + runs[-1][1] == u:
                        runs[-1][1] += 1
                    else:
                        runs.append([u, 1])
                kw = [kload(b, t, off + 8 * u, 8 * n) for u, n in runs]
                kw = kw[0] if len(kw) == 1 else jnp.concatenate(kw, axis=0)
                z = jnp.dot(_b(kw), w, preferred_element_type=f32)
                for k, u in enumerate(chunks):
                    ch[u] = z[16*k:16*k + 16]

            def blk(i):
                return jnp.concatenate([ch[2*i], ch[2*i + 1]], axis=0)
            sm = jnp.where(tri, blk(8), blk(0) if imin == 0 else NEG)
            mx = sm
            for i in range(max(imin, 1), 8):
                mx = jnp.maximum(mx, blk(i))
            m = jnp.max(mx, axis=0, keepdims=True)
            if imin <= SIMIN:
                sref = ss_s[scnt[0] % NSB]
                scnt[0] += 1
                early = [u for chunks in plan for u in chunks[:min(SSTAGE, len(chunks) - 1)] if 2 <= u < 16]
                for u in early:
                    sref[0, 16*u:16*u + 16, :] = ch[u]
                for u in early:
                    ch[u] = sref[zdyn, 16*u:16*u + 16, :]
            pm = jnp.exp2(sm - m)
            X = [None] * 9
            for i in range(max(imin, 1), 8):
                p = jnp.exp2(blk(i) - m)
                X[i] = _pack(p[0:16], p[16:32])
            if imin == 0:
                pf = jnp.where(tri, 0.0, pm)
                X[0] = _pack(pf[0:16], pf[16:32])
                pm = jnp.where(tri, pm, 0.0)
            X[8] = _pack(pm[0:16], pm[16:32])
            return X

        def pv(b, q, t, X, T, acc):
            if q + T < 2:
                return acc
            need("v", b, q + T - 2, t)
            zz = zero
            if last and (b, q, t, T) == (1, NT - 1, 0, 0):
                fz = fence_zero()
                zz = jnp.concatenate([fz, fz], axis=0)

            def sel(m, a, bb):
                if a is None and bb is None:
                    return None
                return jnp.where(m, zz if a is None else a, zz if bb is None else bb)
            Y = [[] for _ in range(4)]
            for B in range(4*T, 4*T + 4):
                xs = [X[c][B - c] if 0 <= B - c <= 8 else None for c in range(4)]
                a = [sel(sel1, xs[k], xs[(k + 1) % 4]) for k in range(4)]
                for j in range(4):
                    y = sel(sel2, a[j], a[(j + 2) % 4])
                    Y[j].append(zero if y is None else y)
            res = []
            for j in range(4):
                h = 4*t + j
                p = _b(jnp.concatenate(Y[j], axis=0))
                vt = _b(vt_s[b][16*h:16*h + 16, ring(q + T - 2)])
                o = jnp.dot(vt, p, preferred_element_type=f32)
                res.append(o if acc is None else o + acc[j])
            return res

        def fin(b, q, t, acc):
            made("o", b, q, t)
            outs = []
            for j in range(4):
                o = acc[j]
                den = o[28:29] if j % 2 == 0 else o[0:1]
                o = o * (1.0 / den)
                if j:
                    o = pltpu.roll(o, 32*j, 1)
                outs.append(o)
            oc = jnp.concatenate([
                outs[0][0:24], jnp.where(lo4, outs[0][24:32], outs[1][0:8]), outs[1][8:32],
                outs[2][0:24], jnp.where(lo4, outs[2][24:32], outs[3][0:8]), outs[3][8:32]], axis=0)
            ot_s[b][56*t:56*t + 56, ring(q)] = _w(oc.astype(bf16))

        ohold = {}

        def put(q, c0, c1, val):
            row = orow(q)
            o_s[pl.ds(row, 128), c0:c1] = val.astype(bf16).T
            if q == NT - 1:
                ocopy(row, c0, c1).start()
            elif c1 == 2 * D:
                ocopy(row).start()

        def outp(b, q, n):
            for t in range(4):
                need("o", b, q, t)
            r0, r1 = ((0, 128, 256, 384, 448) if b == 0 else (0, 64, 192, 320, 448))[n:n + 2]
            y = jnp.dot(_b(wot_s[b][r0 // 2:r1 // 2, :]), _b(ot_s[b][:, ring(q)]),
                        preferred_element_type=f32)

            def post():
                if b == 0:
                    if n == 0:
                        ohold[q] = y
                    elif n == 1:
                        put(q, 0, 256, jnp.concatenate([ohold.pop(q), y], axis=0))
                    elif n == 2 and q == NT - 1:
                        put(q, 256, 384, y)
                    else:
                        made("m", 0, q, n)
                        omid_s[q % 4, 128 * (n - 2):r1 - 256] = y
                else:
                    if n == 0:
                        need("m", 0, q, 2)
                        need("m", 0, q, 3)
                        put(q, 256, 512, jnp.concatenate([omid_s[q % 4], y], axis=0))
                    elif n == 1:
                        ohold[q] = y
                    elif n == 2:
                        put(q, 512, 768, jnp.concatenate([ohold.pop(q), y], axis=0))
                    else:
                        put(q, 768, 896, y)
            later(post)

        def final_out():
            q = NT - 1
            for t in range(4):
                need("o", 1, q, t)
            need("m", 0, q, 3)
            parts = []
            sets = [list(range(n, 28, 4)) for n in range(4)]
            for k0, k1 in ((128, D), (0, 128)):
                rhs = _b(ot_s[1][k0 // 2:k1 // 2, ring(q)])
                ys = [jnp.dot(_b(jnp.concatenate([wot_s[1][8*u:8*u + 8, k0:k1] for u in st], axis=0)), rhs,
                              preferred_element_type=f32) for st in sets]
                parts = [y + p for y, p in zip(ys, parts)] if parts else ys
            ch = {u: p[16*i:16*i + 16] for st, p in zip(sets, parts) for i, u in enumerate(st)}
            y = jnp.concatenate([omid_s[q % 4, 128:192]] + [ch[u] for u in range(28)], axis=0)
            for c0, c1 in FPIECES:
                put(q, c0, c1, y[c0 - 384:c1 - 384])

        def wtile(src, dst, i, ncol):
            c0, c1 = 128 * i, min(128 * i + 128, ncol)
            dst[c0 // 2:c1 // 2, :] = _w(src[:, c0:c1].T)

        def projs(u):
            s, b = divmod(u, 2)
            return [(lambda p=p, t=t, q=q: proj(b, q, p, t))
                    for p in (1, 0, 2) for q in (2*s, 2*s + 1) for t in range(4)]

        def outs(u, qi):
            s, b = divmod(u, 2)
            return [(lambda n=n: outp(b, 2*s + qi, n)) for n in range(4)]

        groups = [(u % 2, 2 * (u // 2) + qi, t) for u in us for qi in range(2) for t in range(4)]
        if last:
            groups = [(1, NT - 2, t) for t in range(4)] + [(1, NT - 1, t) for t in (3, 2, 1, 0)]
        N = len(groups)
        Xs = [[None] * 4 for _ in range(N)]
        accs = [None] * N

        def emit_pv(slot):
            for T in range(3):
                r = slot - 3 - DELAY - PVOFF[T]
                if r >= 0 and r % 4 == 0 and r // 4 < N:
                    g = r // 4
                    accs[g] = pv(*groups[g], Xs[g], T, accs[g])
                    if T == 2:
                        fin(*groups[g], accs[g])
                        Xs[g] = accs[g] = None

        fill = {}

        def spread(thunks, lo, hi):
            n = len(thunks)
            for k, th in enumerate(thunks):
                fill.setdefault(lo + (k * (hi - lo)) // n, []).append(th)

        ntail = sum(TAILF)
        if first:
            for cw, cx in zip(stage_w, stage_x):
                for cp in cw + cx:
                    cp.start()
            for cp in bcopies:
                cp.start()
            r = _iota((56, 128), 0) // 14
            l = _iota((56, 128), 1) // 32
            o_s[S:S + 16, :] = jnp.zeros((16, 2 * D), bf16)
            for c in range(4):
                mq_s[c] = jnp.where(r == ((c - l) & 3), jnp.uint32(0xFFFFFFFF), jnp.uint32(0))
            todo = [(q, part, t) for q in range(4) for part in range(3) for t in range(4)]
            held = []

            def flush():
                while held:
                    held.pop(0)()

            def rowend(p):
                return p[1] * D + 112 * p[2] + 112
            pw = 0
            ns = len(STAGES)
            for i, (cw, cq, bud) in enumerate(STAGES):
                tiles = range(pw // 128, (cw + 127) // 128)
                if i == 0:
                    _wait(stage_w[0])
                    for ti in tiles:
                        wtile(wa_s, wta_s, ti, 3 * D)
                    _wait(stage_x[0])
                else:
                    _wait(stage_w[i] + stage_x[i])
                    for ti in tiles:
                        wtile(wa_s, wta_s, ti, 3 * D)
                flush()
                if i == ns - 1:
                    for cp in xr1 + xr2:
                        cp.start()
                avail = [p for p in todo if p[0] < cq and rowend(p) <= cw]
                avail.sort(key=lambda p: (rowend(p), p[0]))
                if i < ns - 1:
                    avail = avail[:bud]
                else:
                    old = [p for p in avail if rowend(p) <= pw]
                    extra = [p for p in old if p[0] >= bud][:max(0, 2 - len([p for p in old if p[0] < bud]))]
                    avail = [p for p in avail if p[0] < bud or p in extra]
                for k, p in enumerate(avail):
                    proj(0, *p, defer=held if (i < ns - 1 and k >= len(avail) - NDEF) else None)
                    todo.remove(p)
                pw = cw
            todo.sort(key=lambda p: (p[0], (1, 0, 2).index(p[1]), p[2]))

            def b_prep():
                _wait(bcopies)
                flush()
                for ti in range(11):
                    wtile(wb_s, wtb_s, ti, 3 * D)
                for ti in range(4):
                    wtile(woa_s, wota_s, ti, D)
                    wtile(wob_s, wotb_s, ti, D)
            spread([(lambda p=p: proj(0, *p)) for p in todo[:-1]], 0, WBSLOT)
            fill.setdefault(WBSLOT, []).extend([lambda: proj(0, *todo[-1], defer=held), b_prep])
            spread([(lambda p=p, t=t, q=q: proj(1, q, p, t))
                    for q, order in ((0, (0, 1, 2)), (1, (1, 0, 2))) for p in order for t in range(4)],
                   WBSLOT + 2, FB1)
            rest = outs(0, 0) + outs(0, 1) + projs(3)
            spread(rest[:len(rest) - ntail], FB1, 96)
            tail = rest[len(rest) - ntail:]
        elif not last:
            @pl.when(step == 2)
            def _():
                _wait(xr2)
            pslots = [s for s in range(32) if s % 4 != OPOS]
            for k, u in enumerate(us):
                p = projs(u + 1)
                if u == us[-1]:
                    p, tail = p[:24 - ntail], p[24 - ntail:]
                for i, th in enumerate(p):
                    fill.setdefault(32 * k + pslots[(i * 24) // len(p)], []).append(th)
                for i, th in enumerate(outs(u - 2, 0) + outs(u - 2, 1)):
                    fill.setdefault(32 * k + 4 * i + OPOS, []).append(th)
        else:
            oa = outs(14, 1)
            spread(outs(13, 0) + outs(13, 1) + outs(14, 0) + oa[:2], 0, LA)
            spread(outs(15, 0), LA, LB)
            tail = oa[2:]

        slot = 0
        for g in range(N):
            for c in range(4):
                cur[0] = slot
                run_posts(slot)
                Xs[g][c] = qk(*groups[g], c)
                emit_pv(slot)
                for th in fill.get(slot, []):
                    th()
                slot += 1

        def take(n):
            for _ in range(n):
                tail.pop(0)()
        nd = DELAY + max(PVOFF)
        if last:
            run_posts(10**9)
            take(len(tail))
            for k in range(nd):
                emit_pv(slot)
                slot += 1
            run_posts(10**9)
            final_out()
            _wait([ocopy(128 * q) for q in range(NT - 1)]
                  + [ocopy(128 * (NT - 1), c0, c1) for c0, c1 in ((0, 256), (256, 384)) + FPIECES])
            return
        for k in range(nd):
            if k < len(TAILF) - 1:
                take(TAILF[k])
            emit_pv(slot)
            slot += 1
        take(len(tail))
        run_posts(10**9)
        if first:
            _wait(xr1)

    pl.when(step == 0)(lambda: body("first"))
    pl.when(jnp.logical_and(step > 0, step < 4))(lambda: body("mid"))
    pl.when(step == 4)(lambda: body("last"))


@jax.jit
def pallas_concat_heads__sliding_block__sliding_block__prompt_kernel(
    A_x: jax.Array,
    A_wqkv: jax.Array,
    A_wo: jax.Array,
    B_x: jax.Array,
    B_wqkv: jax.Array,
    B_wo: jax.Array,
):
    xa = A_x.reshape(S, D).T
    xb = B_x.reshape(S, D).T
    V = pltpu.VMEM

    def two(shape, dtype):
        return [V(shape, dtype), V(shape, dtype)]

    scratch = (
        two((4, D, 512), bf16)
        + two((D, 3 * D), bf16) + two((D, D), bf16)
        + two((3 * D // 2, D), u32) + two((D // 2, D), u32)
        + two((256, 512), u32) + two((256, 512), u32)
        + two((D // 2, 512), u32) + two((D // 2, 512), u32)
        + [V((4, 192, 128), f32), V((4, 56, 128), u32)]
        + [V((1, 256, 128), f32)] * NSTAGE_BUFS
        + [V((S + 16, 2 * D), bf16),
           pltpu.SemaphoreType.DMA((2 * len(STAGES) + 10,)),
           pltpu.SemaphoreType.DMA((1,))])
    out = pl.pallas_call(
        _kernel,
        grid=(5,),
        in_specs=[pl.BlockSpec(memory_space=pl.ANY)] * 6,
        out_specs=pl.BlockSpec(memory_space=pl.ANY),
        out_shape=jax.ShapeDtypeStruct((S, 2 * D), bf16),
        scratch_shapes=scratch,
        compiler_params=pltpu.CompilerParams(
            dimension_semantics=("arbitrary",), vmem_limit_bytes=100 * 1024 * 1024,
            disable_semaphore_checks=True, disable_bounds_checks=True),
    )(xa, xb, A_wqkv, A_wo, B_wqkv, B_wo)
    return out.reshape(1, S, 2 * D)
```

```python
import math
import jax, jax.numpy as jnp
from jax import lax
import jax.experimental.pallas as pl
import jax.experimental.pallas.tpu as pltpu

S, D, H, DH, W = 2048, 448, 16, 28, 256
NT = S // 128
NEG = -1e30
QSCALE = (DH ** -0.5) * math.log2(math.e)
f32, bf16, i32, u32 = jnp.float32, jnp.bfloat16, jnp.int32, jnp.uint32
HI = 0xFFFF0000
STAGES = ((128,1,1),(256,2,3),(384,3,5),(640,4,10),(1344,4,2))
NHB = 0
WBSLOT = 35
LA = 26
LB = 32
NDEF = 3
NPRE = 1
FPIECES = ((384,512),(512,768),(768,896))
NT0 = 1
PARAMS = {
    "first": dict(FENCE=0, PDELAY=8, DELAY=4, PVOFF=(0, 0, 1), SSTAGE=4, SPEC=1, NSB=10, ORDER=1, QSPL=4, PAT="a0f2fb1f3f", TAILF=(2, 1, 0, 0, 3)),
    "mid": dict(FENCE=0, PDELAY=8, DELAY=5, PVOFF=(0, 1, 1), SSTAGE=3, SPEC=1, NSB=10, ORDER=1, QSPL=4, PAT="a0f2fb1f3f", TAILF=(1, 1, 1, 1, 3)),
    "last": dict(FENCE=16, PDELAY=8, DELAY=4, PVOFF=(0, 0, 0), SSTAGE=3, SPEC=1, NSB=12, ORDER=1, QSPL=4, PAT="a0f2fb1f3f", TAILF=(1, 1, 1, 1, 2)),
}
SIMIN = 4
FB1 = 68
TFENCE = 1
NOSEM = 1
NOBND = 1
FINT = 1
SPOS = 0
PSTAGE = 1
MSTAGE = 0
KEEP = 0
UNIF = 1
OPOS = 2
PORD = (1,0,2)
SCOPES = 0


def _iota(shape, dim):
    return lax.broadcasted_iota(i32, shape, dim)


def _w(x):
    return pltpu.bitcast(x, u32)


def _b(x):
    return pltpu.bitcast(x, bf16)


def _pack(a, b):
    ua = lax.bitcast_convert_type(a, u32)
    ub = lax.bitcast_convert_type(b, u32)
    return (ua >> 16) | (ub & jnp.uint32(HI))


def _split(n, flip):
    parts = [n // 4 + (1 if k < n % 4 else 0) for k in range(4)]
    if flip:
        parts = parts[::-1]
    return [p for p in parts if p]


def _wait(name, cps):
    if SCOPES:
        with jax.named_scope(name):
            for cp in cps:
                cp.wait()
    else:
        for cp in cps:
            cp.wait()


def kernel(xa_hbm, xb_hbm, wa_hbm, woa_hbm, wb_hbm, wob_hbm, o_hbm,
           xa_s, xb_s, wa_s, wb_s, woa_s, wob_s, wta_s, wtb_s, wota_s, wotb_s,
           ka_s, kb_s, kwa_s, kwb_s, vta_s, vtb_s, qta_s, qtb_s, ota_s, otb_s, omid_s, mq_s,
           s0_s, s1_s, s2_s, s3_s, s4_s, s5_s, s6_s, s7_s, s8_s, s9_s, s10_s, s11_s, o_s, wsem, osem):
    step = pl.program_id(0)
    x_hbm, x_s = (xa_hbm, xb_hbm), (xa_s, xb_s)
    wt_s, wot_s = (wta_s, wtb_s), (wota_s, wotb_s)
    ksw_s = (kwa_s, kwb_s)
    k_s, vt_s, qt_s, ot_s = (ka_s, kb_s), (vta_s, vtb_s), (qta_s, qtb_s), (ota_s, otb_s)

    nsem = [0]

    def icopy(s, d):
        nsem[0] += 1
        return pltpu.make_async_copy(s, d, wsem.at[nsem[0] - 1])

    def xcopy(b, lo, hi):
        j, o = divmod(lo, 512)
        return icopy(x_hbm[b].at[:, lo:hi], x_s[b].at[j, :, o:o + hi - lo])

    def ocopy(row, c0=0, c1=2 * D):
        return pltpu.make_async_copy(o_s.at[pl.ds(row, 128), c0:c1], o_hbm.at[pl.ds(row, 128), c0:c1], osem.at[0])

    stage_w, stage_x = [], []
    pw = pq = 0
    for cw, cq, _ in STAGES:
        stage_w.append([icopy(wa_hbm.at[:, pw:cw], wa_s.at[:, pw:cw])] if cw > pw else [])
        stage_x.append([xcopy(0, 128 * pq, 128 * cq)] if cq > pq else [])
        pw, pq = cw, cq
    bcopies = [icopy(wb_hbm, wb_s), xcopy(1, 0, 512), icopy(woa_hbm, woa_s), icopy(wob_hbm, wob_s)]
    xr1 = [xcopy(0, 512, 1024), xcopy(1, 512, 1024)]
    xr2 = [xcopy(0, 1024, 1536), xcopy(1, 1024, 1536), xcopy(0, 1536, 2048), xcopy(1, 1536, 2048)]

    def body(kind):
        first, last = kind == "first", kind == "last"
        P = PARAMS[kind]
        FENCE, PDELAY, DELAY, PVOFF, SSTAGE, SPEC, NSB, ORDER, TAILF = (
            P[k] for k in ("FENCE", "PDELAY", "DELAY", "PVOFF", "SSTAGE", "SPEC", "NSB", "ORDER", "TAILF"))
        us = {"first": (0, 2, 1), "mid": (3, 4, 5, 6), "last": (15,)}[kind]
        r16 = _iota((16, 128), 0)
        lane16 = _iota((16, 128), 1)
        keyidx = jnp.where(r16 < 8, 2 * r16, 2 * r16 - 15)
        tri_lo = keyidx <= (lane16 & 31)
        tri_hi = keyidx + 16 <= (lane16 & 31)
        g03 = (((lane16 + 32) & 64) == 0)
        sel1 = (lane16 & 32) == 0
        sel2 = (lane16 & 64) == 0
        lo4 = _iota((8, 128), 0) < 4
        left8 = (_iota((8, 128), 1) & 64) == 0
        zero = jnp.zeros((16, 128), u32)
        xcache = {}
        scnt = [0]
        qcnt = [0]
        QSPL, PAT = P['QSPL'], P['PAT']
        ss_s = (s0_s, s1_s, s2_s, s3_s, s4_s, s5_s, s6_s, s7_s, s8_s, s9_s, s10_s, s11_s)
        zdyn = step // 8

        def gtok(q, dyn=False):
            if kind == "mid":
                return pl.multiple_of((step - 1) * 512 + 128 * q, 128)
            if dyn and FENCE:
                return pl.multiple_of(zdyn * 128 + 128 * q, 128)
            return 128 * q

        q0 = 2 * (us[0] // 2)
        have = {}
        if not first:
            for t in range(4):
                for q in range(q0 - 2, q0 + 2):
                    for b in range(2):
                        for kd in "qkv":
                            have[kd, b, q % 4, t] = q
                for q in range(q0 - 2, q0):
                    have["o", 1, q % 4, t] = q
                    have["o", 0, (q + 2) % 4, t] = q + 2
            for q in range(q0 - 2, q0):
                have["m", 0, q % 4, 2] = have["m", 0, q % 4, 3] = q

        def made(kd, b, q, t):
            have[kd, b, q % 4, t] = q

        def need(kd, b, q, t):
            assert have.get((kd, b, q % 4, t)) == q, (kind, kd, b, q, t, have.get((kd, b, q % 4, t)))

        cur = [0]
        posts = []

        def later(th):
            posts.append((cur[0] + PDELAY, th))

        def run_posts(upto):
            while posts and posts[0][0] <= upto:
                posts.pop(0)[1]()

        def ring(q):
            return slice(128 * (q % 4), 128 * (q % 4) + 128)

        def proj(b, q, part, t, defer=None):
            r0 = part * (D // 2) + 56 * t
            if (b, q) not in xcache:
                j, o = divmod(128 * q, 512)
                xcache[b, q] = x_s[b][j + step - 1 if kind == "mid" else j, :, o:o + 128]
            xt = xcache[b, q]
            y = jnp.dot(_b(wt_s[b][r0:r0 + 56, :]), xt, preferred_element_type=f32)
            if defer is not None:
                defer.append(lambda: ppost(b, q, part, t, y))
            else:
                ppost(b, q, part, t, y)

        def ppost(b, q, part, t, y):
            made("qkv"[part], b, q, t)
            if part == 0:
                y = y * QSCALE
                r1 = pltpu.roll(y[24:56], 96, 1)
                r2 = pltpu.roll(y[56:88], 64, 1)
                r3 = pltpu.roll(y[80:112], 32, 1)
                z8 = jnp.zeros((8, 128), f32)
                qr = jnp.concatenate([
                    y[0:24], jnp.where(lo4, y[24:32], r1[0:8]), r1[8:32], z8,
                    r2[0:24], jnp.where(lo4, r2[24:32], r3[0:8]), r3[8:32], z8], axis=0)
                qt_s[b][64*t:64*t + 64, ring(q)] = _w(qr.astype(bf16))
            elif part == 1:
                z8 = jnp.zeros((8, 128), f32)
                kt = jnp.concatenate([y[0:56], z8, y[56:112], z8], axis=0)
                kw = _w(kt.astype(bf16).T)
                ev = lax.bitcast_convert_type(kw << 16, f32)
                od = lax.bitcast_convert_type(kw & jnp.uint32(HI), f32)
                kk = _w(jnp.concatenate([z[8*i:8*i + 8] for i in range(8) for z in (ev, od)], axis=0).astype(bf16))
                if q >= 2:
                    hi = jnp.concatenate([kk[8*u:8*u + 8] for u in (1, 3, 5, 7)], axis=0)
                    ksw_s[b][32*(q % 4):32*(q % 4) + 32, 128*t:128*t + 128] = pltpu.roll(hi, 64, 1)
                k_s[b][64*(q % 4):64*(q % 4) + 64, 128*t:128*t + 128] = kk
            else:
                v = jnp.concatenate([
                    y[0:24], jnp.where(lo4, y[24:32], 1.0), jnp.where(lo4, 1.0, y[24:32]), y[32:56],
                    y[56:80], jnp.where(lo4, y[80:88], 1.0), jnp.where(lo4, 1.0, y[80:88]), y[88:112]], axis=0)
                vt_s[b][64*t:64*t + 64, ring(q)] = _w(v.astype(bf16))

        def kload(b, t, off, n):
            lo = off % 256
            if lo + n <= 256:
                return k_s[b][lo:lo + n, 128*t:128*t + 128]
            return jnp.concatenate([k_s[b][lo:256, 128*t:128*t + 128],
                                    k_s[b][0:lo + n - 256, 128*t:128*t + 128]], axis=0)

        xch = {}

        def special(b, q, t, c):
            q32 = qt_s[b][64*t:64*t + 64, ring(q)]
            f_lo = kload(b, t, 64 * q + 16 * c - 128, 8)
            l_hi = ksw_s[b][32*(q % 4) + 8*c:32*(q % 4) + 8*c + 8, 128*t:128*t + 128]
            za = jnp.dot(_b(jnp.where(left8, f_lo, l_hi)),
                         _b(jnp.concatenate([q32[0:32], q32[0:32]], axis=0) & mq_s[4 + c]), preferred_element_type=f32)
            zb = jnp.dot(_b(jnp.where(left8, l_hi, f_lo)),
                         _b(jnp.concatenate([q32[32:64], q32[32:64]], axis=0) & mq_s[8 + c]), preferred_element_type=f32)
            g = g03 if c % 2 == 0 else sel2
            if c >= 2:
                za, zb = zb, za
            xch[c, "m"] = jnp.where(g, za, zb)
            xch[(c + 2) % 4, "p"] = jnp.where(g, zb, za)

        def qk(b, q, t, c):
            imin = max(0, 8 - 4 * q - c)
            need("q", b, q, t)
            for qq in range(max(0, q - 2), q + 1):
                need("k", b, qq, t)
            q32 = qt_s[b][64*t:64*t + 64, ring(q)]
            w = q32 & mq_s[c]
            if FENCE and not first and (cur[0] % FENCE == 0):
                w = jnp.concatenate([w[0:56], w[56:64] | fence_zero()], axis=0)
            w = _b(w)
            off = 64 * q + 16 * c - 128
            if imin == 0:
                pu = 4 if c < 2 else 13
                mids = [u for u in range(2, 16) if u != pu]
                if QSPL == 4:
                    plan = [mids[0:3] + [1], mids[3:6] + [16], mids[6:10], mids[10:13]]
                    rot = qcnt[0] % 4
                    plan = plan[rot:] + plan[:rot]
                elif QSPL == 3:
                    plan = [mids[0:4] + [1], mids[4:8] + [16], mids[8:13]]
                elif QSPL == 2:
                    plan = [mids[0:7] + [1], mids[7:13] + [16]]
                    if (qcnt[0] // 2) % 2:
                        plan = plan[::-1]
                else:
                    plan = [mids + [1, 16]]
                qcnt[0] += 1
            else:
                plan, o = [], 2 * imin
                for n in _split(2 * (9 - imin), c % 2):
                    plan.append(list(range(o, o + n)))
                    o += n
            ch = {}
            for us_ in plan:
                runs = []
                for u in us_:
                    if runs and runs[-1][0] + runs[-1][1] == u:
                        runs[-1][1] += 1
                    else:
                        runs.append([u, 1])
                kw = [kload(b, t, off + 8 * u, 8 * n) for u, n in runs]
                kw = kw[0] if len(kw) == 1 else jnp.concatenate(kw, axis=0)
                z = jnp.dot(_b(kw), w, preferred_element_type=f32)
                for k, u in enumerate(us_):
                    ch[u] = z[16*k:16*k + 16]
            if imin == 0:
                mm = xch.pop((c, "m"))
                ch[pu] = xch.pop((c, "p"))
                s_lo = jnp.where(tri_lo, ch[16], mm)
                s_hi = jnp.where(tri_hi, mm, ch[1])
            else:
                s_lo = jnp.where(tri_lo, ch[16], NEG)
                s_hi = jnp.where(tri_hi, ch[17], NEG)
            inner = range(2 * max(imin, 1), 16)
            mx = [s_lo, s_hi]
            for u in inner:
                mx[u % 2] = jnp.maximum(mx[u % 2], ch[u])
            m = jnp.max(jnp.maximum(mx[0], mx[1]), axis=0, keepdims=True)
            if SSTAGE and imin <= SIMIN:
                sref = ss_s[scnt[0] % NSB]
                scnt[0] += 1
                early = [u for us_ in plan for u in (us_[:len(us_) - KEEP] if imin == 0 and QSPL < 4 else us_[:SSTAGE if imin == 0 else min(SSTAGE, len(us_) - 1)]) if 2 <= u < 16]
                if imin == 0 and PSTAGE:
                    early = [pu] + early
                for u in early:
                    sref[0, 16*u:16*u + 16, :] = ch[u]
                if MSTAGE:
                    sref[0, 0:16, :] = s_lo
                    sref[0, 16:32, :] = s_hi
                    s_lo, s_hi = sref[zdyn, 0:16, :], sref[zdyn, 16:32, :]
                for u in early:
                    ch[u] = sref[zdyn, 16*u:16*u + 16, :]

            def pk(p):
                return _pack(p[0:8], p[8:16])
            p_lo = jnp.exp2(s_lo - m)
            p_hi = jnp.exp2(s_hi - m)
            X = [None] * 9
            for i in range(max(imin, 1), 8):
                X[i] = jnp.concatenate([pk(jnp.exp2(ch[2*i] - m)), pk(jnp.exp2(ch[2*i + 1] - m))], axis=0)
            if imin == 0:
                X[0] = jnp.concatenate([pk(jnp.where(tri_lo, 0.0, p_lo)), pk(jnp.where(tri_hi, 0.0, p_hi))], axis=0)
                p_lo = jnp.where(tri_lo, p_lo, 0.0)
                p_hi = jnp.where(tri_hi, p_hi, 0.0)
            X[8] = jnp.concatenate([pk(p_lo), pk(p_hi)], axis=0)
            return X

        def fence_zero():
            return _w(o_s[pl.ds(pl.multiple_of(S + 16 * zdyn, 16), 16), 0:128])

        def pv(b, q, t, X, T, acc):
            if q + T < 2:
                return acc
            for j in range(4):
                need("v", b, q + T - 2, t)
            zz = zero
            if last and (b, q, t) == (1, NT - 1, 0) and T == TFENCE - 1:
                fz = fence_zero()
                zz = jnp.concatenate([fz, fz], axis=0)

            def sel(m, a, bb):
                if a is None and bb is None:
                    return None
                return jnp.where(m, zz if a is None else a, zz if bb is None else bb)
            Y = [[] for _ in range(4)]
            for B in range(4*T, 4*T + 4):
                xs = [X[c][B - c] if 0 <= B - c <= 8 else None for c in range(4)]
                a = [sel(sel1, xs[k], xs[(k + 1) % 4]) for k in range(4)]
                for j in range(4):
                    y = sel(sel2, a[j], a[(j + 2) % 4])
                    Y[j].append(zero if y is None else y)
            res = []
            for j in range(4):
                h = 4*t + j
                p = _b(jnp.concatenate(Y[j], axis=0))
                vt = _b(vt_s[b][16*h:16*h + 16, ring(q + T - 2)])
                o = jnp.dot(vt, p, preferred_element_type=f32)
                res.append(o if acc is None else o + acc[j])
            return res

        def fin(b, q, t, acc):
            made("o", b, q, t)
            outs = []
            for j in range(4):
                o = acc[j]
                den = o[28:29] if j % 2 == 0 else o[0:1]
                o = o * (1.0 / den)
                if j:
                    o = pltpu.roll(o, 32*j, 1)
                outs.append(o)
            oc = jnp.concatenate([
                outs[0][0:24], jnp.where(lo4, outs[0][24:32], outs[1][0:8]), outs[1][8:32],
                outs[2][0:24], jnp.where(lo4, outs[2][24:32], outs[3][0:8]), outs[3][8:32]], axis=0)
            ot_s[b][56*t:56*t + 56, ring(q)] = _w(oc.astype(bf16))

        ohold = {}

        def put(q, c0, c1, val):
            row = gtok(q, dyn=True)
            o_s[pl.ds(row, 128), c0:c1] = val.astype(bf16).T
            if q == NT - 1:
                ocopy(row, c0, c1).start()
            elif c1 == 2 * D:
                ocopy(row).start()

        def outp(b, q, n):
            for t in range(4):
                need("o", b, q, t)
            r0, r1 = ((0, 128, 256, 384, 448) if b == 0 else (0, 64, 192, 320, 448))[n:n + 2]
            y = jnp.dot(_b(wot_s[b][r0 // 2:r1 // 2, :]), _b(ot_s[b][:, ring(q)]),
                        preferred_element_type=f32)

            def post():
                if b == 0:
                    if n == 0:
                        ohold[q] = y
                    elif n == 1:
                        put(q, 0, 256, jnp.concatenate([ohold.pop(q), y], axis=0))
                    elif n == 2 and q == NT - 1:
                        put(q, 256, 384, y)
                    else:
                        made("m", 0, q, n)
                        omid_s[q % 4, 128 * (n - 2):r1 - 256] = y
                else:
                    if n == 0:
                        need("m", 0, q, 2)
                        need("m", 0, q, 3)
                        put(q, 256, 512, jnp.concatenate([omid_s[q % 4], y], axis=0))
                    elif n == 1:
                        ohold[q] = y
                    elif n == 2:
                        put(q, 512, 768, jnp.concatenate([ohold.pop(q), y], axis=0))
                    else:
                        put(q, 768, 896, y)
            later(post)

        def final_out():
            q = NT - 1
            for t in range(4):
                need("o", 1, q, t)
            need("m", 0, q, 3)
            parts = []
            sets = [list(range(n, 28, 4)) if FINT else list(range(7 * n, 7 * n + 7)) for n in range(4)]
            for k0, k1 in ((128, D), (0, 128)):
                rhs = _b(ot_s[1][k0 // 2:k1 // 2, ring(q)])
                ys = [jnp.dot(_b(jnp.concatenate([wot_s[1][8*u:8*u + 8, k0:k1] for u in st], axis=0)), rhs,
                              preferred_element_type=f32) for st in sets]
                parts = [y + p for y, p in zip(ys, parts)] if parts else ys
            ch = {u: p[16*i:16*i + 16] for st, p in zip(sets, parts) for i, u in enumerate(st)}
            y = jnp.concatenate([omid_s[q % 4, 128:192]] + [ch[u] for u in range(28)], axis=0)
            for c0, c1 in FPIECES:
                put(q, c0, c1, y[c0 - 384:c1 - 384])

        def wtile(src, dst, i, ncol):
            c0, c1 = 128 * i, min(128 * i + 128, ncol)
            dst[c0 // 2:c1 // 2, :] = _w(src[:, c0:c1].T)

        def projs(u, order=(1, 0, 2)):
            s, b = divmod(u, 2)
            return [(lambda p=p, t=t, q=q: proj(b, q, p, t))
                    for p in order for q in (2*s, 2*s + 1) for t in range(4)]

        def outs(u, qi):
            s, b = divmod(u, 2)
            return [(lambda n=n: outp(b, 2*s + qi, n)) for n in range(4)]

        groups = [(u % 2, 2 * (u // 2) + qi, t) for u in us for qi in range(2) for t in range(4)]
        if last:
            groups = [(1, 14, t) for t in range(4)] + [(1, 15, t) for t in (3, 2, 1, 0)]
        N = len(groups)
        Xs = [[None] * 4 for _ in range(N)]
        accs = [None] * N

        def emit_pv(slot):
            for T in range(3):
                r = slot - 3 - DELAY - PVOFF[T]
                if r >= 0 and r % 4 == 0 and r // 4 < N:
                    g = r // 4
                    accs[g] = pv(*groups[g], Xs[g], T, accs[g])
                    if T == 2:
                        fin(*groups[g], accs[g])
                        Xs[g] = accs[g] = None

        fill = {}

        def spread(thunks, lo, hi):
            n = len(thunks)
            for k, th in enumerate(thunks):
                fill.setdefault(lo + (k * (hi - lo)) // n, []).append(th)

        NTL = sum(TAILF)
        if first:
            for cw, cx in zip(stage_w, stage_x):
                for cp in cw + cx:
                    cp.start()
            for cp in bcopies:
                cp.start()
            row = _iota((64, 128), 0)
            lane = _iota((64, 128), 1)
            half, hh, l, jlo = row // 32, (row % 32) // 14, lane // 32, (lane & 16) == 0
            ok = hh < 2
            o_s[S:S + 16, :] = jnp.zeros((16, 2 * D), bf16)

            def bits(m):
                return jnp.where(m & ok, jnp.uint32(0xFFFFFFFF), jnp.uint32(0))
            for c in range(4):
                mq_s[c] = bits(((2 * half + hh + l) & 3) == c)
                for k in range(2):
                    sb = (2 * k + hh + l) & 3
                    isf = half == k
                    own = (sb == c) & (isf == jlo)
                    other = (sb == (c + 2) % 4) & (isf if c >= 2 else ~isf)
                    mq_s[4 + 4 * k + c] = bits(own | other)
            todo = [(q, part, t) for q in range(4) for part in range(3) for t in range(4)]
            held = []

            def flush():
                while held:
                    held.pop(0)()
            pw = 0
            ns = len(STAGES)
            rowend = lambda p: p[1] * D + 112 * p[2] + 112
            for i, (cw, cq, bud) in enumerate(STAGES):
                tiles = range(pw // 128, (cw + 127) // 128)
                if i == 0:
                    _wait("wt", stage_w[0])
                    for ti in tiles[:NT0]:
                        wtile(wa_s, wta_s, ti, 3 * D)
                    _wait("w0", stage_x[0])
                    tiles = tiles[NT0:]
                else:
                    _wait(f"w{i}", stage_w[i] + stage_x[i])
                for ti in tiles:
                    wtile(wa_s, wta_s, ti, 3 * D)
                flush()
                if i == ns - 1:
                    for cp in xr1 + xr2:
                        cp.start()
                avail = [p for p in todo if p[0] < cq and rowend(p) <= cw]
                avail.sort(key=lambda p: (rowend(p), p[0]))
                if i < ns - 1:
                    avail = avail[:bud]
                else:
                    old = [p for p in avail if rowend(p) <= pw]
                    extra = [p for p in old if p[0] >= bud][:max(0, 2 - len([p for p in old if p[0] < bud]))]
                    avail = [p for p in avail if p[0] < bud or p in extra]
                for k, p in enumerate(avail):
                    proj(0, *p, defer=held if (i < ns - 1 and k >= len(avail) - NDEF) else None)
                    todo.remove(p)
                pw = cw
            todo.sort(key=lambda p: (p[0], (1, 0, 2).index(p[1]), p[2]))

            def wb_prep():
                _wait("wb", bcopies)
                flush()
                for ti in range(11):
                    wtile(wb_s, wtb_s, ti, 3 * D)
                for ti in range(4):
                    wtile(woa_s, wota_s, ti, D)
                    wtile(wob_s, wotb_s, ti, D)
            nk = NPRE + NHB
            n2 = len(todo)
            p2 = [(lambda p=p, k=k: proj(0, *p, defer=held if n2 - nk <= k < n2 - nk + NPRE else None))
                  for k, p in enumerate(todo)]
            n1 = len([p for p in todo if p[0] == 1])
            spread(p2[:n1], 0, 14)
            spread(p2[n1:n2 - nk], 14 if n1 else 0, WBSLOT)
            spread(p2[n2 - nk:n2 - NHB], WBSLOT, WBSLOT + 1)
            fill.setdefault(WBSLOT, []).append(wb_prep)
            spread(p2[n2 - NHB:], WBSLOT, WBSLOT + 2)
            pb = [(lambda p=p, t=t, q=q: proj(1, q, p, t))
                  for q, order in ((0, (0, 1, 2)), (1, (1, 0, 2))) for p in order for t in range(4)]
            spread(pb, WBSLOT + 2, FB1)
            p3 = projs(3, PORD)
            rest = outs(0, 0) + outs(0, 1) + p3
            spread(rest[:len(rest) - NTL], FB1, 96)
            tail = rest[len(rest) - NTL:]
        elif not last:
            @pl.when(step == 2)
            def _():
                for cp in xr2:
                    cp.wait()
            for k, u in enumerate(us):
                base = 32 * k
                p = projs(u + 1, PORD)
                if u == us[-1]:
                    p, tail = p[:24 - NTL], p[24 - NTL:]
                o = outs(u - 2, 0) + outs(u - 2, 1)
                if UNIF:
                    ps = [s for s in range(32) if s % 4 != OPOS]
                    for i, th in enumerate(p):
                        fill.setdefault(base + ps[(i * 24) // len(p)], []).append(th)
                    for i, th in enumerate(o):
                        fill.setdefault(base + 4 * i + OPOS, []).append(th)
                else:
                    spread(p, base, base + 30)
                    spread(o, base + (8 if k else 0), base + 32)
        else:
            oa = outs(14, 1)
            spread(outs(13, 0) + outs(13, 1) + outs(14, 0) + oa[:2], 0, LA)
            spread(outs(15, 0), LA, LB)
            tail = oa[2:]

        slot = 0
        for g in range(N):
            pat = PAT if groups[g][1] >= 2 else "0f2f1f3f"
            for tok in pat:
                cur[0] = slot
                if tok in "ab":
                    c = "ab".index(tok)
                    for t_ in ("q", "k"):
                        need(t_, *groups[g])
                    special(*groups[g], c)
                    special(*groups[g], c + 2)
                elif tok in "ABCD":
                    special(*groups[g], "ABCD".index(tok))
                elif tok == "f":
                    emit_pv(slot)
                    for th in fill.get(slot, []):
                        th()
                    slot += 1
                    run_posts(slot)
                else:
                    Xs[g][int(tok)] = qk(*groups[g], int(tok))

        def take(n):
            for _ in range(n):
                th = tail.pop(0)
                if th is not None:
                    th()
        nd = DELAY + max(PVOFF)
        if last:
            run_posts(10**9)
            take(len(tail))
            for k in range(nd):
                emit_pv(slot)
                slot += 1
            run_posts(10**9)
            final_out()
            _wait("ow", [ocopy(128 * q) for q in range(NT - 1)]
                  + [ocopy(128 * (NT - 1), c0, c1) for c0, c1 in ((0, 256), (256, 384)) + FPIECES])
            return
        for k in range(nd):
            if k < len(TAILF) - 1:
                take(TAILF[k])
            emit_pv(slot)
            slot += 1
        take(len(tail))
        run_posts(10**9)
        if first:
            _wait("xr1", xr1)

    def sc(kind):
        def f():
            if SCOPES:
                with jax.named_scope(kind):
                    body(kind)
            else:
                body(kind)
        return f
    pl.when(step == 0)(sc("first"))
    pl.when(jnp.logical_and(step > 0, step < 4))(sc("mid"))
    pl.when(step == 4)(sc("last"))


@jax.jit
def pallas_concat_heads__sliding_block__sliding_block__prompt_kernel(A_x, A_wqkv, A_wo, B_x, B_wqkv, B_wo):
    xa = A_x.reshape(S, D).T
    xb = B_x.reshape(S, D).T
    V = pltpu.VMEM
    two = lambda shp, dt: [V(shp, dt), V(shp, dt)]
    out = pl.pallas_call(
        kernel,
        grid=(5,),
        in_specs=[pl.BlockSpec(memory_space=pl.ANY)] * 6,
        out_specs=pl.BlockSpec(memory_space=pl.ANY),
        out_shape=jax.ShapeDtypeStruct((S, 2*D), bf16),
        scratch_shapes=(two((4, D, 512), bf16) + two((D, 3*D), bf16) + two((D, D), bf16)
                        + two((3*D // 2, D), u32) + two((D // 2, D), u32)
                        + two((256, 512), u32) + two((128, 512), u32) + two((256, 512), u32)
                        + two((256, 512), u32) + two((D // 2, 512), u32)
                        + [V((4, 192, 128), f32), V((12, 64, 128), u32)]
                        + [V((1, 256, 128), f32)] * 12 + [V((S + 16, 2*D), bf16),
                           pltpu.SemaphoreType.DMA((2 * len(STAGES) + 10,)),
                           pltpu.SemaphoreType.DMA((1,))]),
        compiler_params=pltpu.CompilerParams(dimension_semantics=("arbitrary",), vmem_limit_bytes=100*1024*1024,
                                             disable_semaphore_checks=bool(NOSEM), disable_bounds_checks=bool(NOBND)),
    )(xa, xb, A_wqkv, A_wo, B_wqkv, B_wo)
    return out.reshape(1, S, 2*D)
```

```python
import math

import jax
import jax.numpy as jnp
from jax import lax
import jax.experimental.pallas as pl
import jax.experimental.pallas.tpu as pltpu

S, D, H, DH, W = 2048, 448, 16, 28, 256
NT = S // 128
NEG = -1e30
QSCALE = (DH ** -0.5) * math.log2(math.e)
f32, bf16, i32, u32 = jnp.float32, jnp.bfloat16, jnp.int32, jnp.uint32
HI = 0xFFFF0000

STAGES = ((128, 1, 1), (256, 2, 3), (384, 3, 5), (640, 4, 10), (1344, 4, 2))
WBSLOT, FB1, NDEF = 35, 68, 3
LA, LB = 26, 32
OPOS = 2
SIMIN = 4
NSTAGE_BUFS = 12
FPIECES = ((384, 512), (512, 768), (768, 896))
PARAMS = {
    "first": dict(FENCE=0, PDELAY=8, DELAY=4, PVOFF=(0, 0, 1), SSTAGE=4, NSB=10, TAILF=(2, 1, 0, 0, 3)),
    "mid": dict(FENCE=0, PDELAY=8, DELAY=5, PVOFF=(0, 1, 1), SSTAGE=3, NSB=10, TAILF=(1, 1, 1, 1, 3)),
    "last": dict(FENCE=16, PDELAY=8, DELAY=4, PVOFF=(0, 0, 0), SSTAGE=3, NSB=12, TAILF=()),
}


def _iota(shape, dim):
    return lax.broadcasted_iota(i32, shape, dim)


def _w(x):
    return pltpu.bitcast(x, u32)


def _b(x):
    return pltpu.bitcast(x, bf16)


def _pack(a, b):
    ua = lax.bitcast_convert_type(a, u32)
    ub = lax.bitcast_convert_type(b, u32)
    return (ua >> 16) | (ub & jnp.uint32(HI))


def _split(n, flip):
    parts = [n // 4 + (1 if k < n % 4 else 0) for k in range(4)]
    if flip:
        parts = parts[::-1]
    return [p for p in parts if p]


def _wait(copies):
    for cp in copies:
        cp.wait()


def _kernel(xa_hbm, xb_hbm, wa_hbm, woa_hbm, wb_hbm, wob_hbm, o_hbm,
            xa_s, xb_s, wa_s, wb_s, woa_s, wob_s, wta_s, wtb_s, wota_s, wotb_s,
            ka_s, kb_s, kwa_s, kwb_s, vta_s, vtb_s, qta_s, qtb_s, ota_s, otb_s, omid_s, mq_s,
            *rest):
    ss_s, (o_s, isem, osem) = rest[:NSTAGE_BUFS], rest[NSTAGE_BUFS:]
    step = pl.program_id(0)
    x_hbm, x_s = (xa_hbm, xb_hbm), (xa_s, xb_s)
    wt_s, wot_s = (wta_s, wtb_s), (wota_s, wotb_s)
    k_s, vt_s, qt_s, ot_s = (ka_s, kb_s), (vta_s, vtb_s), (qta_s, qtb_s), (ota_s, otb_s)
    ksw_s = (kwa_s, kwb_s)

    nsem = [0]

    def icopy(src, dst):
        nsem[0] += 1
        return pltpu.make_async_copy(src, dst, isem.at[nsem[0] - 1])

    def xcopy(b, lo, hi):
        j, o = divmod(lo, 512)
        return icopy(x_hbm[b].at[:, lo:hi], x_s[b].at[j, :, o:o + hi - lo])

    def ocopy(row, c0=0, c1=2 * D):
        return pltpu.make_async_copy(o_s.at[pl.ds(row, 128), c0:c1], o_hbm.at[pl.ds(row, 128), c0:c1], osem.at[0])

    stage_w, stage_x = [], []
    pw = pq = 0
    for cw, cq, _ in STAGES:
        stage_w.append([icopy(wa_hbm.at[:, pw:cw], wa_s.at[:, pw:cw])] if cw > pw else [])
        stage_x.append([xcopy(0, 128 * pq, 128 * cq)] if cq > pq else [])
        pw, pq = cw, cq
    bcopies = [icopy(wb_hbm, wb_s), xcopy(1, 0, 512), icopy(woa_hbm, woa_s), icopy(wob_hbm, wob_s)]
    xrest = [xcopy(b, lo, lo + 512) for lo in (512, 1024, 1536) for b in range(2)]

    def body(kind):
        first, last = kind == "first", kind == "last"
        prm = PARAMS[kind]
        FENCE, PDELAY, DELAY, PVOFF, SSTAGE, NSB, TAILF = (
            prm[k] for k in ("FENCE", "PDELAY", "DELAY", "PVOFF", "SSTAGE", "NSB", "TAILF"))
        us = {"first": (0, 2, 1), "mid": (3, 4, 5, 6), "last": (15,)}[kind]
        r16 = _iota((16, 128), 0)
        lane16 = _iota((16, 128), 1)
        keyidx = jnp.where(r16 < 8, 2 * r16, 2 * r16 - 15)
        tri_lo = keyidx <= (lane16 & 31)
        tri_hi = keyidx + 16 <= (lane16 & 31)
        g03 = (((lane16 + 32) & 64) == 0)
        sel1 = (lane16 & 32) == 0
        sel2 = (lane16 & 64) == 0
        lo4 = _iota((8, 128), 0) < 4
        left8 = (_iota((8, 128), 1) & 64) == 0
        zero = jnp.zeros((16, 128), u32)
        xcache = {}
        scnt = [0]
        qcnt = [0]
        zdyn = step // 8

        def orow(q):
            if kind == "mid":
                return pl.multiple_of((step - 1) * 512 + 128 * q, 128)
            if FENCE:
                return pl.multiple_of(zdyn * 128 + 128 * q, 128)
            return 128 * q

        q0 = 2 * (us[0] // 2)
        have = {}
        if not first:
            for t in range(4):
                for q in range(q0 - 2, q0 + 2):
                    for b in range(2):
                        for kd in "qkv":
                            have[kd, b, q % 4, t] = q
                for q in range(q0 - 2, q0):
                    have["o", 1, q % 4, t] = q
                    have["o", 0, (q + 2) % 4, t] = q + 2
            for q in range(q0 - 2, q0):
                have["m", 0, q % 4, 2] = have["m", 0, q % 4, 3] = q

        def made(kd, b, q, t):
            have[kd, b, q % 4, t] = q

        def need(kd, b, q, t):
            assert have.get((kd, b, q % 4, t)) == q, (kind, kd, b, q, t)

        cur = [0]
        posts = []

        def later(th):
            posts.append((cur[0] + PDELAY, th))

        def run_posts(upto):
            while posts and posts[0][0] <= upto:
                posts.pop(0)[1]()

        def ring(q):
            return slice(128 * (q % 4), 128 * (q % 4) + 128)

        def proj(b, q, part, t, defer=None):
            r0 = part * (D // 2) + 56 * t
            if (b, q) not in xcache:
                j, o = divmod(128 * q, 512)
                xcache[b, q] = x_s[b][j + step - 1 if kind == "mid" else j, :, o:o + 128]
            xt = xcache[b, q]
            y = jnp.dot(_b(wt_s[b][r0:r0 + 56, :]), xt, preferred_element_type=f32)
            if defer is not None:
                defer.append(lambda: proj_post(b, q, part, t, y))
            else:
                proj_post(b, q, part, t, y)

        def proj_post(b, q, part, t, y):
            made("qkv"[part], b, q, t)
            if part == 0:
                y = y * QSCALE
                r1 = pltpu.roll(y[24:56], 96, 1)
                r2 = pltpu.roll(y[56:88], 64, 1)
                r3 = pltpu.roll(y[80:112], 32, 1)
                z8 = jnp.zeros((8, 128), f32)
                qr = jnp.concatenate([
                    y[0:24], jnp.where(lo4, y[24:32], r1[0:8]), r1[8:32], z8,
                    r2[0:24], jnp.where(lo4, r2[24:32], r3[0:8]), r3[8:32], z8], axis=0)
                qt_s[b][64*t:64*t + 64, ring(q)] = _w(qr.astype(bf16))
            elif part == 1:
                z8 = jnp.zeros((8, 128), f32)
                kt = jnp.concatenate([y[0:56], z8, y[56:112], z8], axis=0)
                kw = _w(kt.astype(bf16).T)
                ev = lax.bitcast_convert_type(kw << 16, f32)
                od = lax.bitcast_convert_type(kw & jnp.uint32(HI), f32)
                kk = _w(jnp.concatenate([z[8*i:8*i + 8] for i in range(8) for z in (ev, od)], axis=0).astype(bf16))
                if q >= 2:
                    hi = jnp.concatenate([kk[8*u:8*u + 8] for u in (1, 3, 5, 7)], axis=0)
                    ksw_s[b][32*(q % 4):32*(q % 4) + 32, 128*t:128*t + 128] = pltpu.roll(hi, 64, 1)
                k_s[b][64*(q % 4):64*(q % 4) + 64, 128*t:128*t + 128] = kk
            else:
                v = jnp.concatenate([
                    y[0:24], jnp.where(lo4, y[24:32], 1.0), jnp.where(lo4, 1.0, y[24:32]), y[32:56],
                    y[56:80], jnp.where(lo4, y[80:88], 1.0), jnp.where(lo4, 1.0, y[80:88]), y[88:112]], axis=0)
                vt_s[b][64*t:64*t + 64, ring(q)] = _w(v.astype(bf16))

        def kload(b, t, off, n):
            lo = off % 256
            if lo + n <= 256:
                return k_s[b][lo:lo + n, 128*t:128*t + 128]
            return jnp.concatenate([k_s[b][lo:256, 128*t:128*t + 128],
                                    k_s[b][0:lo + n - 256, 128*t:128*t + 128]], axis=0)

        def fence_zero():
            return _w(o_s[pl.ds(pl.multiple_of(S + 16 * zdyn, 16), 16), 0:128])

        xch = {}

        def edge(b, q, t, c):
            q32 = qt_s[b][64*t:64*t + 64, ring(q)]
            f_lo = kload(b, t, 64 * q + 16 * c - 128, 8)
            l_hi = ksw_s[b][32*(q % 4) + 8*c:32*(q % 4) + 8*c + 8, 128*t:128*t + 128]
            za = jnp.dot(_b(jnp.where(left8, f_lo, l_hi)),
                         _b(jnp.concatenate([q32[0:32], q32[0:32]], axis=0) & mq_s[4 + c]),
                         preferred_element_type=f32)
            zb = jnp.dot(_b(jnp.where(left8, l_hi, f_lo)),
                         _b(jnp.concatenate([q32[32:64], q32[32:64]], axis=0) & mq_s[8 + c]),
                         preferred_element_type=f32)
            g = g03 if c % 2 == 0 else sel2
            if c >= 2:
                za, zb = zb, za
            xch[c, "m"] = jnp.where(g, za, zb)
            xch[(c + 2) % 4, "p"] = jnp.where(g, zb, za)

        def qk(b, q, t, c):
            imin = max(0, 8 - 4 * q - c)
            need("q", b, q, t)
            for qq in range(max(0, q - 2), q + 1):
                need("k", b, qq, t)
            q32 = qt_s[b][64*t:64*t + 64, ring(q)]
            w = q32 & mq_s[c]
            if FENCE and cur[0] % FENCE == 0:
                w = jnp.concatenate([w[0:56], w[56:64] | fence_zero()], axis=0)
            w = _b(w)
            off = 64 * q + 16 * c - 128
            if imin == 0:
                pu = 4 if c < 2 else 13
                mids = [u for u in range(2, 16) if u != pu]
                plan = [mids[0:3] + [1], mids[3:6] + [16], mids[6:10], mids[10:13]]
                rot = qcnt[0] % 4
                plan = plan[rot:] + plan[:rot]
                qcnt[0] += 1
            else:
                plan, o = [], 2 * imin
                for n in _split(2 * (9 - imin), c % 2):
                    plan.append(list(range(o, o + n)))
                    o += n
            ch = {}
            for chunks in plan:
                runs = []
                for u in chunks:
                    if runs and runs[-1][0] + runs[-1][1] == u:
                        runs[-1][1] += 1
                    else:
                        runs.append([u, 1])
                kw = [kload(b, t, off + 8 * u, 8 * n) for u, n in runs]
                kw = kw[0] if len(kw) == 1 else jnp.concatenate(kw, axis=0)
                z = jnp.dot(_b(kw), w, preferred_element_type=f32)
                for k, u in enumerate(chunks):
                    ch[u] = z[16*k:16*k + 16]
            if imin == 0:
                mm = xch.pop((c, "m"))
                ch[pu] = xch.pop((c, "p"))
                s_lo = jnp.where(tri_lo, ch[16], mm)
                s_hi = jnp.where(tri_hi, mm, ch[1])
            else:
                s_lo = jnp.where(tri_lo, ch[16], NEG)
                s_hi = jnp.where(tri_hi, ch[17], NEG)
            mx = [s_lo, s_hi]
            for u in range(2 * max(imin, 1), 16):
                mx[u % 2] = jnp.maximum(mx[u % 2], ch[u])
            m = jnp.max(jnp.maximum(mx[0], mx[1]), axis=0, keepdims=True)
            if imin <= SIMIN:
                sref = ss_s[scnt[0] % NSB]
                scnt[0] += 1
                early = [u for chunks in plan
                         for u in chunks[:SSTAGE if imin == 0 else min(SSTAGE, len(chunks) - 1)] if 2 <= u < 16]
                if imin == 0:
                    early = [pu] + early
                for u in early:
                    sref[0, 16*u:16*u + 16, :] = ch[u]
                for u in early:
                    ch[u] = sref[zdyn, 16*u:16*u + 16, :]

            def pk(p):
                return _pack(p[0:8], p[8:16])
            p_lo = jnp.exp2(s_lo - m)
            p_hi = jnp.exp2(s_hi - m)
            X = [None] * 9
            for i in range(max(imin, 1), 8):
                X[i] = jnp.concatenate([pk(jnp.exp2(ch[2*i] - m)), pk(jnp.exp2(ch[2*i + 1] - m))], axis=0)
            if imin == 0:
                X[0] = jnp.concatenate([pk(jnp.where(tri_lo, 0.0, p_lo)), pk(jnp.where(tri_hi, 0.0, p_hi))], axis=0)
                p_lo = jnp.where(tri_lo, p_lo, 0.0)
                p_hi = jnp.where(tri_hi, p_hi, 0.0)
            X[8] = jnp.concatenate([pk(p_lo), pk(p_hi)], axis=0)
            return X

        def pv(b, q, t, X, T, acc):
            if q + T < 2:
                return acc
            need("v", b, q + T - 2, t)
            zz = zero
            if last and (b, q, t, T) == (1, NT - 1, 0, 0):
                fz = fence_zero()
                zz = jnp.concatenate([fz, fz], axis=0)

            def sel(m, a, bb):
                if a is None and bb is None:
                    return None
                return jnp.where(m, zz if a is None else a, zz if bb is None else bb)
            Y = [[] for _ in range(4)]
            for B in range(4*T, 4*T + 4):
                xs = [X[c][B - c] if 0 <= B - c <= 8 else None for c in range(4)]
                a = [sel(sel1, xs[k], xs[(k + 1) % 4]) for k in range(4)]
                for j in range(4):
                    y = sel(sel2, a[j], a[(j + 2) % 4])
                    Y[j].append(zero if y is None else y)
            res = []
            for j in range(4):
                h = 4*t + j
                p = _b(jnp.concatenate(Y[j], axis=0))
                vt = _b(vt_s[b][16*h:16*h + 16, ring(q + T - 2)])
                o = jnp.dot(vt, p, preferred_element_type=f32)
                res.append(o if acc is None else o + acc[j])
            return res

        def fin(b, q, t, acc):
            made("o", b, q, t)
            outs = []
            for j in range(4):
                o = acc[j]
                den = o[28:29] if j % 2 == 0 else o[0:1]
                o = o * (1.0 / den)
                if j:
                    o = pltpu.roll(o, 32*j, 1)
                outs.append(o)
            oc = jnp.concatenate([
                outs[0][0:24], jnp.where(lo4, outs[0][24:32], outs[1][0:8]), outs[1][8:32],
                outs[2][0:24], jnp.where(lo4, outs[2][24:32], outs[3][0:8]), outs[3][8:32]], axis=0)
            ot_s[b][56*t:56*t + 56, ring(q)] = _w(oc.astype(bf16))

        ohold = {}

        def put(q, c0, c1, val):
            row = orow(q)
            o_s[pl.ds(row, 128), c0:c1] = val.astype(bf16).T
            if q == NT - 1:
                ocopy(row, c0, c1).start()
            elif c1 == 2 * D:
                ocopy(row).start()

        def outp(b, q, n):
            for t in range(4):
                need("o", b, q, t)
            r0, r1 = ((0, 128, 256, 384, 448) if b == 0 else (0, 64, 192, 320, 448))[n:n + 2]
            y = jnp.dot(_b(wot_s[b][r0 // 2:r1 // 2, :]), _b(ot_s[b][:, ring(q)]),
                        preferred_element_type=f32)

            def post():
                if b == 0:
                    if n == 0:
                        ohold[q] = y
                    elif n == 1:
                        put(q, 0, 256, jnp.concatenate([ohold.pop(q), y], axis=0))
                    elif n == 2 and q == NT - 1:
                        put(q, 256, 384, y)
                    else:
                        made("m", 0, q, n)
                        omid_s[q % 4, 128 * (n - 2):r1 - 256] = y
                else:
                    if n == 0:
                        need("m", 0, q, 2)
                        need("m", 0, q, 3)
                        put(q, 256, 512, jnp.concatenate([omid_s[q % 4], y], axis=0))
                    elif n == 1:
                        ohold[q] = y
                    elif n == 2:
                        put(q, 512, 768, jnp.concatenate([ohold.pop(q), y], axis=0))
                    else:
                        put(q, 768, 896, y)
            later(post)

        def final_out():
            q = NT - 1
            for t in range(4):
                need("o", 1, q, t)
            need("m", 0, q, 3)
            parts = []
            sets = [list(range(n, 28, 4)) for n in range(4)]
            for k0, k1 in ((128, D), (0, 128)):
                rhs = _b(ot_s[1][k0 // 2:k1 // 2, ring(q)])
                ys = [jnp.dot(_b(jnp.concatenate([wot_s[1][8*u:8*u + 8, k0:k1] for u in st], axis=0)), rhs,
                              preferred_element_type=f32) for st in sets]
                parts = [y + p for y, p in zip(ys, parts)] if parts else ys
            ch = {u: p[16*i:16*i + 16] for st, p in zip(sets, parts) for i, u in enumerate(st)}
            y = jnp.concatenate([omid_s[q % 4, 128:192]] + [ch[u] for u in range(28)], axis=0)
            for c0, c1 in FPIECES:
                put(q, c0, c1, y[c0 - 384:c1 - 384])

        def wtile(src, dst, i, ncol):
            c0, c1 = 128 * i, min(128 * i + 128, ncol)
            dst[c0 // 2:c1 // 2, :] = _w(src[:, c0:c1].T)

        def projs(u):
            s, b = divmod(u, 2)
            return [(lambda p=p, t=t, q=q: proj(b, q, p, t))
                    for p in (1, 0, 2) for q in (2*s, 2*s + 1) for t in range(4)]

        def outs(u, qi):
            s, b = divmod(u, 2)
            return [(lambda n=n: outp(b, 2*s + qi, n)) for n in range(4)]

        groups = [(u % 2, 2 * (u // 2) + qi, t) for u in us for qi in range(2) for t in range(4)]
        if last:
            groups = [(1, NT - 2, t) for t in range(4)] + [(1, NT - 1, t) for t in (3, 2, 1, 0)]
        N = len(groups)
        Xs = [[None] * 4 for _ in range(N)]
        accs = [None] * N

        def emit_pv(slot):
            for T in range(3):
                r = slot - 3 - DELAY - PVOFF[T]
                if r >= 0 and r % 4 == 0 and r // 4 < N:
                    g = r // 4
                    accs[g] = pv(*groups[g], Xs[g], T, accs[g])
                    if T == 2:
                        fin(*groups[g], accs[g])
                        Xs[g] = accs[g] = None

        fill = {}

        def spread(thunks, lo, hi):
            n = len(thunks)
            for k, th in enumerate(thunks):
                fill.setdefault(lo + (k * (hi - lo)) // n, []).append(th)

        ntail = sum(TAILF)
        if first:
            for cw, cx in zip(stage_w, stage_x):
                for cp in cw + cx:
                    cp.start()
            for cp in bcopies:
                cp.start()
            row = _iota((64, 128), 0)
            lane = _iota((64, 128), 1)
            half, hh, l, jlo = row // 32, (row % 32) // 14, lane // 32, (lane & 16) == 0
            ok = hh < 2
            o_s[S:S + 16, :] = jnp.zeros((16, 2 * D), bf16)

            def bits(m):
                return jnp.where(m & ok, jnp.uint32(0xFFFFFFFF), jnp.uint32(0))
            for c in range(4):
                mq_s[c] = bits(((2 * half + hh + l) & 3) == c)
                for k in range(2):
                    sb = (2 * k + hh + l) & 3
                    isf = half == k
                    own = (sb == c) & (isf == jlo)
                    other = (sb == (c + 2) % 4) & (isf if c >= 2 else ~isf)
                    mq_s[4 + 4 * k + c] = bits(own | other)
            todo = [(q, part, t) for q in range(4) for part in range(3) for t in range(4)]
            held = []

            def flush():
                while held:
                    held.pop(0)()

            def rowend(p):
                return p[1] * D + 112 * p[2] + 112
            pw = 0
            ns = len(STAGES)
            for i, (cw, cq, bud) in enumerate(STAGES):
                tiles = range(pw // 128, (cw + 127) // 128)
                if i == 0:
                    _wait(stage_w[0])
                    for ti in tiles:
                        wtile(wa_s, wta_s, ti, 3 * D)
                    _wait(stage_x[0])
                else:
                    _wait(stage_w[i] + stage_x[i])
                    for ti in tiles:
                        wtile(wa_s, wta_s, ti, 3 * D)
                flush()
                if i == ns - 1:
                    for cp in xrest:
                        cp.start()
                avail = [p for p in todo if p[0] < cq and rowend(p) <= cw]
                avail.sort(key=lambda p: (rowend(p), p[0]))
                if i < ns - 1:
                    avail = avail[:bud]
                else:
                    old = [p for p in avail if rowend(p) <= pw]
                    extra = [p for p in old if p[0] >= bud][:max(0, 2 - len([p for p in old if p[0] < bud]))]
                    avail = [p for p in avail if p[0] < bud or p in extra]
                for k, p in enumerate(avail):
                    proj(0, *p, defer=held if (i < ns - 1 and k >= len(avail) - NDEF) else None)
                    todo.remove(p)
                pw = cw
            todo.sort(key=lambda p: (p[0], (1, 0, 2).index(p[1]), p[2]))

            def b_prep():
                _wait(bcopies)
                flush()
                for ti in range(11):
                    wtile(wb_s, wtb_s, ti, 3 * D)
                for ti in range(4):
                    wtile(woa_s, wota_s, ti, D)
                    wtile(wob_s, wotb_s, ti, D)
            spread([(lambda p=p: proj(0, *p)) for p in todo[:-1]], 0, WBSLOT)
            fill.setdefault(WBSLOT, []).extend([lambda: proj(0, *todo[-1], defer=held), b_prep])
            spread([(lambda p=p, t=t, q=q: proj(1, q, p, t))
                    for q, order in ((0, (0, 1, 2)), (1, (1, 0, 2))) for p in order for t in range(4)],
                   WBSLOT + 2, FB1)
            rest = outs(0, 0) + outs(0, 1) + projs(3)
            spread(rest[:len(rest) - ntail], FB1, 96)
            tail = rest[len(rest) - ntail:]
        elif not last:
            pslots = [s for s in range(32) if s % 4 != OPOS]
            for k, u in enumerate(us):
                p = projs(u + 1)
                if u == us[-1]:
                    p, tail = p[:24 - ntail], p[24 - ntail:]
                for i, th in enumerate(p):
                    fill.setdefault(32 * k + pslots[(i * 24) // len(p)], []).append(th)
                for i, th in enumerate(outs(u - 2, 0) + outs(u - 2, 1)):
                    fill.setdefault(32 * k + 4 * i + OPOS, []).append(th)
        else:
            oa = outs(14, 1)
            spread(outs(13, 0) + outs(13, 1) + outs(14, 0) + oa[:2], 0, LA)
            spread(outs(15, 0), LA, LB)
            tail = oa[2:]

        slot = 0
        for g in range(N):
            pat = "a0f2fb1f3f" if groups[g][1] >= 2 else "0f2f1f3f"
            if g == 0 and kind == "mid":
                pat = "fa02fb1f3f"
            for tok in pat:
                cur[0] = slot
                if tok in "ab":
                    need("q", *groups[g])
                    need("k", *groups[g])
                    edge(*groups[g], "ab".index(tok))
                    edge(*groups[g], "ab".index(tok) + 2)
                elif tok == "f":
                    emit_pv(slot)
                    for th in fill.get(slot, []):
                        th()
                    slot += 1
                    run_posts(slot)
                else:
                    Xs[g][int(tok)] = qk(*groups[g], int(tok))

        def take(n):
            for _ in range(n):
                tail.pop(0)()
        nd = DELAY + max(PVOFF)
        if last:
            run_posts(10**9)
            take(len(tail))
            for k in range(nd):
                emit_pv(slot)
                slot += 1
            run_posts(10**9)
            final_out()
            _wait([ocopy(128 * q) for q in range(NT - 1)]
                  + [ocopy(128 * (NT - 1), c0, c1) for c0, c1 in ((0, 256), (256, 384)) + FPIECES])
            return
        for k in range(nd):
            if k < len(TAILF) - 1:
                take(TAILF[k])
            emit_pv(slot)
            slot += 1
        take(len(tail))
        run_posts(10**9)
        if first:
            _wait(xrest)

    pl.when(step == 0)(lambda: body("first"))
    pl.when(jnp.logical_and(step > 0, step < 4))(lambda: body("mid"))
    pl.when(step == 4)(lambda: body("last"))


@jax.jit
def pallas_concat_heads__sliding_block__sliding_block__prompt_kernel(
    A_x: jax.Array,
    A_wqkv: jax.Array,
    A_wo: jax.Array,
    B_x: jax.Array,
    B_wqkv: jax.Array,
    B_wo: jax.Array,
):
    xa = A_x.reshape(S, D).T
    xb = B_x.reshape(S, D).T
    V = pltpu.VMEM

    def two(shape, dtype):
        return [V(shape, dtype), V(shape, dtype)]

    scratch = (
        two((4, D, 512), bf16)
        + two((D, 3 * D), bf16) + two((D, D), bf16)
        + two((3 * D // 2, D), u32) + two((D // 2, D), u32)
        + two((256, 512), u32) + two((128, 512), u32)
        + two((256, 512), u32)
        + two((256, 512), u32) + two((D // 2, 512), u32)
        + [V((4, 192, 128), f32), V((12, 64, 128), u32)]
        + [V((1, 256, 128), f32)] * NSTAGE_BUFS
        + [V((S + 16, 2 * D), bf16),
           pltpu.SemaphoreType.DMA((2 * len(STAGES) + 10,)),
           pltpu.SemaphoreType.DMA((1,))])
    out = pl.pallas_call(
        _kernel,
        grid=(5,),
        in_specs=[pl.BlockSpec(memory_space=pl.ANY)] * 6,
        out_specs=pl.BlockSpec(memory_space=pl.ANY),
        out_shape=jax.ShapeDtypeStruct((S, 2 * D), bf16),
        scratch_shapes=scratch,
        compiler_params=pltpu.CompilerParams(
            dimension_semantics=("arbitrary",), vmem_limit_bytes=100 * 1024 * 1024,
            disable_semaphore_checks=True, disable_bounds_checks=True),
    )(xa, xb, A_wqkv, A_wo, B_wqkv, B_wo)
    return out.reshape(1, S, 2 * D)
```

```python
import math

import jax
import jax.numpy as jnp
from jax import lax
import jax.experimental.pallas as pl
import jax.experimental.pallas.tpu as pltpu

S, D, H, DH, W = 2048, 448, 16, 28, 256
NT = S // 128
NEG = -1e30
QSCALE = (DH ** -0.5) * math.log2(math.e)
f32, bf16, i32, u32 = jnp.float32, jnp.bfloat16, jnp.int32, jnp.uint32
HI = 0xFFFF0000

STAGES = (
    (((0, 128, 0, 640),), ((0, 128),), ((0, 4, 0, 128),)),
    (((0, 128, 640, 1344),), ((128, 256),), ((4, 5, 0, 128), (5, 8, 0, 128), (8, 11, 0, 128))),
    (((128, 256, 0, 1344),), (), ((11, 12, 0, 128), (0, 4, 128, 256), (4, 8, 128, 256), (8, 10, 128, 256))),
    (((256, 448, 0, 1344),), ((256, 448),), ((10, 12, 128, 256),)),
)
WBSLOT, FA1, FB1, LAZY = 38, 30, 66, 8
LA, LB = 26, 32
OPOS = 2
SIMIN = 6
NSTAGE_BUFS = 12
FPIECES = ((384, 512), (512, 768), (768, 896))
PARAMS = {
    "first": dict(FENCE=0, PDELAY=8, DELAY=5, PVOFF=(0, 1, 1), SSTAGE=3, NSB=12, TAILF=(1, 1, 1, 1, 3)),
    "mid": dict(FENCE=0, PDELAY=8, DELAY=5, PVOFF=(0, 1, 1), SSTAGE=3, NSB=10, TAILF=(1, 1, 1, 1, 3)),
    "last": dict(FENCE=16, PDELAY=8, DELAY=4, PVOFF=(0, 0, 0), SSTAGE=3, NSB=12, TAILF=()),
}


def _iota(shape, dim):
    return lax.broadcasted_iota(i32, shape, dim)


def _w(x):
    return pltpu.bitcast(x, u32)


def _b(x):
    return pltpu.bitcast(x, bf16)


def _pack(a, b):
    ua = lax.bitcast_convert_type(a, u32)
    ub = lax.bitcast_convert_type(b, u32)
    return (ua >> 16) | (ub & jnp.uint32(HI))


def _split(n, flip):
    parts = [n // 4 + (1 if k < n % 4 else 0) for k in range(4)]
    if flip:
        parts = parts[::-1]
    return [p for p in parts if p]


def _wait(copies):
    for cp in copies:
        cp.wait()


def _kernel(xa_hbm, xb_hbm, wa_hbm, woa_hbm, wb_hbm, wob_hbm, o_hbm,
            xa_s, xb_s, wa_s, wb_s, woa_s, wob_s, wta_s, wtb_s, wota_s, wotb_s,
            ka_s, kb_s, kwa_s, kwb_s, vta_s, vtb_s, qta_s, qtb_s, ota_s, otb_s, omid_s, mq_s,
            *rest):
    ss_s, (o_s, isem, osem) = rest[:NSTAGE_BUFS], rest[NSTAGE_BUFS:]
    step = pl.program_id(0)
    x_hbm, x_s = (xa_hbm, xb_hbm), (xa_s, xb_s)
    wt_s, wot_s = (wta_s, wtb_s), (wota_s, wotb_s)
    k_s, vt_s, qt_s, ot_s = (ka_s, kb_s), (vta_s, vtb_s), (qta_s, qtb_s), (ota_s, otb_s)
    ksw_s = (kwa_s, kwb_s)

    nsem = [0]

    def icopy(src, dst):
        nsem[0] += 1
        return pltpu.make_async_copy(src, dst, isem.at[nsem[0] - 1])

    def xcopy(b, lo, hi):
        j, o = divmod(lo, 512)
        return icopy(x_hbm[b].at[:, lo:hi], x_s[b].at[j, :, o:o + hi - lo])

    def ocopy(row, c0=0, c1=2 * D):
        return pltpu.make_async_copy(o_s.at[pl.ds(row, 128), c0:c1], o_hbm.at[pl.ds(row, 128), c0:c1], osem.at[0])

    stage_w = [[icopy(wa_hbm.at[k0:k1, c0:c1], wa_s.at[k0:k1, c0:c1]) for k0, k1, c0, c1 in ws]
               for ws, _, _ in STAGES]
    stage_x = [[icopy(xa_hbm.at[k0:k1, 0:512], xa_s.at[0, k0:k1, :]) for k0, k1 in xs] for _, xs, _ in STAGES]
    bcopies = [icopy(wb_hbm, wb_s), xcopy(1, 0, 512), icopy(woa_hbm, woa_s), icopy(wob_hbm, wob_s)]
    xrest = [xcopy(b, lo, lo + 512) for lo in (512, 1024, 1536) for b in range(2)]

    def body(kind):
        first, last = kind == "first", kind == "last"
        prm = PARAMS[kind]
        FENCE, PDELAY, DELAY, PVOFF, SSTAGE, NSB, TAILF = (
            prm[k] for k in ("FENCE", "PDELAY", "DELAY", "PVOFF", "SSTAGE", "NSB", "TAILF"))
        us = {"first": (0, 2, 1), "mid": (3, 4, 5, 6), "last": (15,)}[kind]
        r16 = _iota((16, 128), 0)
        lane16 = _iota((16, 128), 1)
        keyidx = jnp.where(r16 < 8, 2 * r16, 2 * r16 - 15)
        tri_lo = keyidx <= (lane16 & 31)
        tri_hi = keyidx + 16 <= (lane16 & 31)
        g03 = (((lane16 + 32) & 64) == 0)
        sel1 = (lane16 & 32) == 0
        sel2 = (lane16 & 64) == 0
        lo4 = _iota((8, 128), 0) < 4
        left8 = (_iota((8, 128), 1) & 64) == 0
        zero = jnp.zeros((16, 128), u32)
        xcache = {}
        scnt = [0]
        qcnt = [0]
        zdyn = step // 8

        def orow(q):
            if kind == "mid":
                return pl.multiple_of((step - 1) * 512 + 128 * q, 128)
            if FENCE:
                return pl.multiple_of(zdyn * 128 + 128 * q, 128)
            return 128 * q

        q0 = 2 * (us[0] // 2)
        have = {}
        if not first:
            for t in range(4):
                for q in range(q0 - 2, q0 + 2):
                    for b in range(2):
                        for kd in "qkv":
                            have[kd, b, q % 4, t] = q
                for q in range(q0 - 2, q0):
                    have["o", 1, q % 4, t] = q
                    have["o", 0, (q + 2) % 4, t] = q + 2
            for q in range(q0 - 2, q0):
                have["m", 0, q % 4, 2] = have["m", 0, q % 4, 3] = q

        def made(kd, b, q, t):
            have[kd, b, q % 4, t] = q

        def need(kd, b, q, t):
            assert have.get((kd, b, q % 4, t)) == q, (kind, kd, b, q, t)

        cur = [0]
        posts = []

        def later(th):
            posts.append((cur[0] + PDELAY, th))

        def run_posts(upto):
            while posts and posts[0][0] <= upto:
                posts.pop(0)[1]()

        def ring(q):
            return slice(128 * (q % 4), 128 * (q % 4) + 128)

        def proj(b, q, part, t):
            r0 = part * (D // 2) + 56 * t
            if (b, q) not in xcache:
                j, o = divmod(128 * q, 512)
                xcache[b, q] = x_s[b][j + step - 1 if kind == "mid" else j, :, o:o + 128]
            y = jnp.dot(_b(wt_s[b][r0:r0 + 56, :]), xcache[b, q], preferred_element_type=f32)
            proj_post(b, q, part, t, y)

        def proj_post(b, q, part, t, y):
            made("qkv"[part], b, q, t)
            if part == 0:
                y = y * QSCALE
                r1 = pltpu.roll(y[24:56], 96, 1)
                r2 = pltpu.roll(y[56:88], 64, 1)
                r3 = pltpu.roll(y[80:112], 32, 1)
                z8 = jnp.zeros((8, 128), f32)
                qr = jnp.concatenate([
                    y[0:24], jnp.where(lo4, y[24:32], r1[0:8]), r1[8:32], z8,
                    r2[0:24], jnp.where(lo4, r2[24:32], r3[0:8]), r3[8:32], z8], axis=0)
                qt_s[b][64*t:64*t + 64, ring(q)] = _w(qr.astype(bf16))
            elif part == 1:
                z8 = jnp.zeros((8, 128), f32)
                kt = jnp.concatenate([y[0:56], z8, y[56:112], z8], axis=0)
                kw = _w(kt.astype(bf16).T)
                ev = lax.bitcast_convert_type(kw << 16, f32)
                od = lax.bitcast_convert_type(kw & jnp.uint32(HI), f32)
                kk = _w(jnp.concatenate([z[8*i:8*i + 8] for i in range(8) for z in (ev, od)], axis=0).astype(bf16))
                if q >= 2:
                    hi = jnp.concatenate([kk[8*u:8*u + 8] for u in (1, 3, 5, 7)], axis=0)
                    ksw_s[b][32*(q % 4):32*(q % 4) + 32, 128*t:128*t + 128] = pltpu.roll(hi, 64, 1)
                k_s[b][64*(q % 4):64*(q % 4) + 64, 128*t:128*t + 128] = kk
            else:
                v = jnp.concatenate([
                    y[0:24], jnp.where(lo4, y[24:32], 1.0), jnp.where(lo4, 1.0, y[24:32]), y[32:56],
                    y[56:80], jnp.where(lo4, y[80:88], 1.0), jnp.where(lo4, 1.0, y[80:88]), y[88:112]], axis=0)
                vt_s[b][64*t:64*t + 64, ring(q)] = _w(v.astype(bf16))

        def kload(b, t, off, n):
            lo = off % 256
            if lo + n <= 256:
                return k_s[b][lo:lo + n, 128*t:128*t + 128]
            return jnp.concatenate([k_s[b][lo:256, 128*t:128*t + 128],
                                    k_s[b][0:lo + n - 256, 128*t:128*t + 128]], axis=0)

        def fence_zero():
            return _w(o_s[pl.ds(pl.multiple_of(S + 16 * zdyn, 16), 16), 0:128])

        xch = {}

        def edge(b, q, t, c):
            q32 = qt_s[b][64*t:64*t + 64, ring(q)]
            f_lo = kload(b, t, 64 * q + 16 * c - 128, 8)
            l_hi = ksw_s[b][32*(q % 4) + 8*c:32*(q % 4) + 8*c + 8, 128*t:128*t + 128]
            za = jnp.dot(_b(jnp.where(left8, f_lo, l_hi)),
                         _b(jnp.concatenate([q32[0:32], q32[0:32]], axis=0) & mq_s[4 + c]),
                         preferred_element_type=f32)
            zb = jnp.dot(_b(jnp.where(left8, l_hi, f_lo)),
                         _b(jnp.concatenate([q32[32:64], q32[32:64]], axis=0) & mq_s[8 + c]),
                         preferred_element_type=f32)
            g = g03 if c % 2 == 0 else sel2
            if c >= 2:
                za, zb = zb, za
            xch[c, "m"] = jnp.where(g, za, zb)
            xch[(c + 2) % 4, "p"] = jnp.where(g, zb, za)

        def qk(b, q, t, c):
            imin = max(0, 8 - 4 * q - c)
            need("q", b, q, t)
            for qq in range(max(0, q - 2), q + 1):
                need("k", b, qq, t)
            q32 = qt_s[b][64*t:64*t + 64, ring(q)]
            w = q32 & mq_s[c]
            if FENCE and cur[0] % FENCE == 0:
                w = jnp.concatenate([w[0:56], w[56:64] | fence_zero()], axis=0)
            w = _b(w)
            off = 64 * q + 16 * c - 128
            if imin == 0:
                pu = 4 if c < 2 else 13
                mids = [u for u in range(2, 16) if u != pu]
                plan = [mids[0:3] + [1], mids[3:6] + [16], mids[6:10], mids[10:13]]
                rot = qcnt[0] % 4
                plan = plan[rot:] + plan[:rot]
                qcnt[0] += 1
            else:
                plan, o = [], 2 * imin
                for n in _split(2 * (9 - imin), c % 2):
                    plan.append(list(range(o, o + n)))
                    o += n
            ch = {}
            for chunks in plan:
                runs = []
                for u in chunks:
                    if runs and runs[-1][0] + runs[-1][1] == u:
                        runs[-1][1] += 1
                    else:
                        runs.append([u, 1])
                kw = [kload(b, t, off + 8 * u, 8 * n) for u, n in runs]
                kw = kw[0] if len(kw) == 1 else jnp.concatenate(kw, axis=0)
                z = jnp.dot(_b(kw), w, preferred_element_type=f32)
                for k, u in enumerate(chunks):
                    ch[u] = z[16*k:16*k + 16]
            if imin == 0:
                mm = xch.pop((c, "m"))
                ch[pu] = xch.pop((c, "p"))
                s_lo = jnp.where(tri_lo, ch[16], mm)
                s_hi = jnp.where(tri_hi, mm, ch[1])
            else:
                s_lo = jnp.where(tri_lo, ch[16], NEG)
                s_hi = jnp.where(tri_hi, ch[17], NEG)
            mx = [s_lo, s_hi]
            for u in range(2 * max(imin, 1), 16):
                mx[u % 2] = jnp.maximum(mx[u % 2], ch[u])
            m = jnp.max(jnp.maximum(mx[0], mx[1]), axis=0, keepdims=True)
            if imin <= SIMIN:
                sref = ss_s[scnt[0] % NSB]
                scnt[0] += 1
                early = [u for chunks in plan
                         for u in chunks[:SSTAGE if imin == 0 else min(SSTAGE, len(chunks) - 1)] if 2 <= u < 16]
                if imin == 0:
                    early = [pu] + early
                for u in early:
                    sref[0, 16*u:16*u + 16, :] = ch[u]
            else:
                early, sref = [], None
            born = scnt[0]

            def pk(p):
                return _pack(p[0:8], p[8:16])

            def finish():
                assert scnt[0] - born < NSB
                for u in early:
                    ch[u] = sref[zdyn, 16*u:16*u + 16, :]
                p_lo = jnp.exp2(s_lo - m)
                p_hi = jnp.exp2(s_hi - m)
                X = [None] * 9
                for i in range(max(imin, 1), 8):
                    X[i] = jnp.concatenate([pk(jnp.exp2(ch[2*i] - m)), pk(jnp.exp2(ch[2*i + 1] - m))], axis=0)
                if imin == 0:
                    X[0] = jnp.concatenate([pk(jnp.where(tri_lo, 0.0, p_lo)),
                                            pk(jnp.where(tri_hi, 0.0, p_hi))], axis=0)
                    p_lo = jnp.where(tri_lo, p_lo, 0.0)
                    p_hi = jnp.where(tri_hi, p_hi, 0.0)
                X[8] = jnp.concatenate([pk(p_lo), pk(p_hi)], axis=0)
                return X
            return finish if first and WBSLOT - LAZY < cur[0] <= WBSLOT else finish()

        def pv(b, q, t, X, T, acc):
            if q + T < 2:
                return acc
            need("v", b, q + T - 2, t)
            zz = zero
            if last and (b, q, t, T) == (1, NT - 1, 0, 0):
                fz = fence_zero()
                zz = jnp.concatenate([fz, fz], axis=0)

            def sel(m, a, bb):
                if a is None and bb is None:
                    return None
                return jnp.where(m, zz if a is None else a, zz if bb is None else bb)
            Y = [[] for _ in range(4)]
            for B in range(4*T, 4*T + 4):
                xs = [X[c][B - c] if 0 <= B - c <= 8 else None for c in range(4)]
                a = [sel(sel1, xs[k], xs[(k + 1) % 4]) for k in range(4)]
                for j in range(4):
                    y = sel(sel2, a[j], a[(j + 2) % 4])
                    Y[j].append(zero if y is None else y)
            res = []
            for j in range(4):
                h = 4*t + j
                p = _b(jnp.concatenate(Y[j], axis=0))
                vt = _b(vt_s[b][16*h:16*h + 16, ring(q + T - 2)])
                o = jnp.dot(vt, p, preferred_element_type=f32)
                res.append(o if acc is None else o + acc[j])
            return res

        def fin(b, q, t, acc):
            made("o", b, q, t)
            outs = []
            for j in range(4):
                o = acc[j]
                den = o[28:29] if j % 2 == 0 else o[0:1]
                o = o * (1.0 / den)
                if j:
                    o = pltpu.roll(o, 32*j, 1)
                outs.append(o)
            oc = jnp.concatenate([
                outs[0][0:24], jnp.where(lo4, outs[0][24:32], outs[1][0:8]), outs[1][8:32],
                outs[2][0:24], jnp.where(lo4, outs[2][24:32], outs[3][0:8]), outs[3][8:32]], axis=0)
            ot_s[b][56*t:56*t + 56, ring(q)] = _w(oc.astype(bf16))

        ohold = {}

        def put(q, c0, c1, val):
            row = orow(q)
            o_s[pl.ds(row, 128), c0:c1] = val.astype(bf16).T
            if q == NT - 1:
                ocopy(row, c0, c1).start()
            elif c1 == 2 * D:
                ocopy(row).start()

        def outp(b, q, n):
            for t in range(4):
                need("o", b, q, t)
            r0, r1 = ((0, 128, 256, 384, 448) if b == 0 else (0, 64, 192, 320, 448))[n:n + 2]
            y = jnp.dot(_b(wot_s[b][r0 // 2:r1 // 2, :]), _b(ot_s[b][:, ring(q)]),
                        preferred_element_type=f32)

            def post():
                if b == 0:
                    if n == 0:
                        ohold[q] = y
                    elif n == 1:
                        put(q, 0, 256, jnp.concatenate([ohold.pop(q), y], axis=0))
                    elif n == 2 and q == NT - 1:
                        put(q, 256, 384, y)
                    else:
                        made("m", 0, q, n)
                        omid_s[q % 4, 128 * (n - 2):r1 - 256] = y
                else:
                    if n == 0:
                        need("m", 0, q, 2)
                        need("m", 0, q, 3)
                        put(q, 256, 512, jnp.concatenate([omid_s[q % 4], y], axis=0))
                    elif n == 1:
                        ohold[q] = y
                    elif n == 2:
                        put(q, 512, 768, jnp.concatenate([ohold.pop(q), y], axis=0))
                    else:
                        put(q, 768, 896, y)
            later(post)

        def final_out():
            q = NT - 1
            for t in range(4):
                need("o", 1, q, t)
            need("m", 0, q, 3)
            parts = []
            sets = [list(range(n, 28, 4)) for n in range(4)]
            for k0, k1 in ((128, D), (0, 128)):
                rhs = _b(ot_s[1][k0 // 2:k1 // 2, ring(q)])
                ys = [jnp.dot(_b(jnp.concatenate([wot_s[1][8*u:8*u + 8, k0:k1] for u in st], axis=0)), rhs,
                              preferred_element_type=f32) for st in sets]
                parts = [y + p for y, p in zip(ys, parts)] if parts else ys
            ch = {u: p[16*i:16*i + 16] for st, p in zip(sets, parts) for i, u in enumerate(st)}
            y = jnp.concatenate([omid_s[q % 4, 128:192]] + [ch[u] for u in range(28)], axis=0)
            for c0, c1 in FPIECES:
                put(q, c0, c1, y[c0 - 384:c1 - 384])

        def wtile(src, dst, i, ncol):
            c0, c1 = 128 * i, min(128 * i + 128, ncol)
            dst[c0 // 2:c1 // 2, :] = _w(src[:, c0:c1].T)

        def projs(u):
            s, b = divmod(u, 2)
            return [(lambda p=p, t=t, q=q: proj(b, q, p, t))
                    for p in (1, 0, 2) for q in (2*s, 2*s + 1) for t in range(4)]

        def outs(u, qi):
            s, b = divmod(u, 2)
            return [(lambda n=n: outp(b, 2*s + qi, n)) for n in range(4)]

        groups = [(u % 2, 2 * (u // 2) + qi, t) for u in us for qi in range(2) for t in range(4)]
        if last:
            groups = [(1, NT - 2, t) for t in range(4)] + [(1, NT - 1, t) for t in (3, 2, 1, 0)]
        N = len(groups)
        Xs = [[None] * 4 for _ in range(N)]
        accs = [None] * N

        def emit_pv(slot):
            for T in range(3):
                r = slot - 3 - DELAY - PVOFF[T]
                if r >= 0 and r % 4 == 0 and r // 4 < N:
                    g = r // 4
                    Xs[g] = [x() if callable(x) else x for x in Xs[g]]
                    accs[g] = pv(*groups[g], Xs[g], T, accs[g])
                    if T == 2:
                        fin(*groups[g], accs[g])
                        Xs[g] = accs[g] = None

        fill = {}

        def spread(thunks, lo, hi):
            n = len(thunks)
            for k, th in enumerate(thunks):
                fill.setdefault(lo + (k * (hi - lo)) // n, []).append(th)

        ntail = sum(TAILF)
        if first:
            for cw, cx in zip(stage_w, stage_x):
                for cp in cw + cx:
                    cp.start()
            for cp in bcopies:
                cp.start()
            row = _iota((64, 128), 0)
            lane = _iota((64, 128), 1)
            half, hh, l, jlo = row // 32, (row % 32) // 14, lane // 32, (lane & 16) == 0
            ok = hh < 2
            o_s[S:S + 16, :] = jnp.zeros((16, 2 * D), bf16)

            def bits(m):
                return jnp.where(m & ok, jnp.uint32(0xFFFFFFFF), jnp.uint32(0))
            for c in range(4):
                mq_s[c] = bits(((2 * half + hh + l) & 3) == c)
                for k in range(2):
                    sb = (2 * k + hh + l) & 3
                    isf = half == k
                    own = (sb == c) & (isf == jlo)
                    other = (sb == (c + 2) % 4) & (isf if c >= 2 else ~isf)
                    mq_s[4 + 4 * k + c] = bits(own | other)

            def wsub(k0, k1, c0, c1):
                for c in range(c0, c1, 128):
                    ce = min(c + 128, c1)
                    wta_s[c // 2:ce // 2, k0:k1] = _w(wa_s[k0:k1, c:ce].T)
            part_sum = {}
            for i, (ws, xs, work) in enumerate(STAGES):
                _wait(stage_w[i] + (stage_x[i] if i else []))
                for blk in ws:
                    wsub(*blk)
                if i == 0:
                    _wait(stage_x[0])
                if i == len(STAGES) - 1:
                    for cp in xrest:
                        cp.start()
                for n0, n1, k0, k1 in work:
                    y = jnp.dot(_b(wta_s[56 * n0:56 * n1, k0:k1]), xa_s[0, k0:k1, :], preferred_element_type=f32)
                    for n in range(n0, n1):
                        z = y[112 * (n - n0):112 * (n - n0) + 112]
                        assert part_sum.get(n, (None, 0))[1] == k0
                        part_sum[n] = (z if k0 == 0 else z + part_sum[n][0], k1)
            xfin = {}
            held = []

            def proj_fin(qp, n, defer=False):
                z, k0 = part_sum[n]
                if (qp, k0) not in xfin:
                    xfin[qp, k0] = xa_s[0, k0:D, 256 * qp:256 * qp + 256]
                y = jnp.dot(_b(wta_s[56 * n:56 * n + 56, k0:D]), xfin[qp, k0], preferred_element_type=f32)
                y = y + z[:, 256 * qp:256 * qp + 256]

                def post():
                    for i in range(2):
                        proj_post(0, 2 * qp + i, n // 4, n % 4, y[:, 128 * i:128 * i + 128])
                if defer:
                    held.append(post)
                else:
                    post()
            for n in range(12):
                proj_fin(0, n)

            def b_prep():
                _wait(bcopies)
                held.pop()()
                for ti in range(11):
                    wtile(wb_s, wtb_s, ti, 3 * D)
                for ti in range(4):
                    wtile(woa_s, wota_s, ti, D)
                    wtile(wob_s, wotb_s, ti, D)
            spread([(lambda n=n: proj_fin(1, n)) for n in (4, 5, 6, 7, 0, 1, 2, 3)], 0, FA1)
            spread([(lambda n=n: proj_fin(1, n)) for n in (8, 9, 10)], FA1, WBSLOT)
            fill.setdefault(WBSLOT, []).extend([lambda: proj_fin(1, 11, defer=True), b_prep])
            spread([(lambda p=p, t=t, q=q: proj(1, q, p, t))
                    for q, order in ((0, (0, 1, 2)), (1, (1, 0, 2))) for p in order for t in range(4)],
                   WBSLOT + 2, FB1)
            more = outs(0, 0) + outs(0, 1) + projs(3)
            spread(more[:len(more) - ntail], FB1, 96)
            tail = more[len(more) - ntail:]
        elif not last:
            pslots = [s for s in range(32) if s % 4 != OPOS]
            for k, u in enumerate(us):
                p = projs(u + 1)
                if u == us[-1]:
                    p, tail = p[:24 - ntail], p[24 - ntail:]
                for i, th in enumerate(p):
                    fill.setdefault(32 * k + pslots[(i * 24) // len(p)], []).append(th)
                for i, th in enumerate(outs(u - 2, 0) + outs(u - 2, 1)):
                    fill.setdefault(32 * k + 4 * i + OPOS, []).append(th)
        else:
            oa = outs(14, 1)
            spread(outs(13, 0) + outs(13, 1) + outs(14, 0) + oa[:2], 0, LA)
            spread(outs(15, 0), LA, LB)
            tail = oa[2:]

        slot = 0
        for g in range(N):
            pat = "a0f2fb1f3f" if groups[g][1] >= 2 else "0f2f1f3f"
            if g == 0 and kind == "mid":
                pat = "fa02fb1f3f"
            for tok in pat:
                cur[0] = slot
                if tok in "ab":
                    need("q", *groups[g])
                    need("k", *groups[g])
                    edge(*groups[g], "ab".index(tok))
                    edge(*groups[g], "ab".index(tok) + 2)
                elif tok == "f":
                    emit_pv(slot)
                    for th in fill.get(slot, []):
                        th()
                    slot += 1
                    run_posts(slot)
                else:
                    Xs[g][int(tok)] = qk(*groups[g], int(tok))

        def take(n):
            for _ in range(n):
                tail.pop(0)()
        nd = DELAY + max(PVOFF)
        if last:
            run_posts(10**9)
            take(len(tail))
            for k in range(nd):
                emit_pv(slot)
                slot += 1
            run_posts(10**9)
            final_out()
            _wait([ocopy(128 * q) for q in range(NT - 1)]
                  + [ocopy(128 * (NT - 1), c0, c1) for c0, c1 in ((0, 256), (256, 384)) + FPIECES])
            return
        for k in range(nd):
            if k < len(TAILF) - 1:
                take(TAILF[k])
            emit_pv(slot)
            slot += 1
        take(len(tail))
        run_posts(10**9)
        if first:
            _wait(xrest)

    pl.when(step == 0)(lambda: body("first"))
    pl.when(jnp.logical_and(step > 0, step < 4))(lambda: body("mid"))
    pl.when(step == 4)(lambda: body("last"))


@jax.jit
def pallas_concat_heads__sliding_block__sliding_block__prompt_kernel(
    A_x: jax.Array,
    A_wqkv: jax.Array,
    A_wo: jax.Array,
    B_x: jax.Array,
    B_wqkv: jax.Array,
    B_wo: jax.Array,
):
    xa = A_x.reshape(S, D).T
    xb = B_x.reshape(S, D).T
    V = pltpu.VMEM

    def two(shape, dtype):
        return [V(shape, dtype), V(shape, dtype)]

    scratch = (
        two((4, D, 512), bf16)
        + two((D, 3 * D), bf16) + two((D, D), bf16)
        + two((3 * D // 2, D), u32) + two((D // 2, D), u32)
        + two((256, 512), u32) + two((128, 512), u32)
        + two((256, 512), u32)
        + two((256, 512), u32) + two((D // 2, 512), u32)
        + [V((4, 192, 128), f32), V((12, 64, 128), u32)]
        + [V((1, 256, 128), f32)] * NSTAGE_BUFS
        + [V((S + 16, 2 * D), bf16),
           pltpu.SemaphoreType.DMA((24,)),
           pltpu.SemaphoreType.DMA((1,))])
    out = pl.pallas_call(
        _kernel,
        grid=(5,),
        in_specs=[pl.BlockSpec(memory_space=pl.ANY)] * 6,
        out_specs=pl.BlockSpec(memory_space=pl.ANY),
        out_shape=jax.ShapeDtypeStruct((S, 2 * D), bf16),
        scratch_shapes=scratch,
        compiler_params=pltpu.CompilerParams(
            dimension_semantics=("arbitrary",), vmem_limit_bytes=100 * 1024 * 1024,
            disable_semaphore_checks=True, disable_bounds_checks=True),
    )(xa, xb, A_wqkv, A_wo, B_wqkv, B_wo)
    return out.reshape(1, S, 2 * D)
```

```python
import math

import jax
import jax.numpy as jnp
from jax import lax
import jax.experimental.pallas as pl
import jax.experimental.pallas.tpu as pltpu

S, D, H, DH, W = 2048, 448, 16, 28, 256
NT = S // 128
NEG = -1e30
QSCALE = (DH ** -0.5) * math.log2(math.e)
f32, bf16, i32, u32 = jnp.float32, jnp.bfloat16, jnp.int32, jnp.uint32
HI = 0xFFFF0000

STAGES = (
    (((0, 128, 0, 640),), ((0, 128),), ((0, 4, 0, 128),)),
    (((0, 128, 640, 1344),), ((128, 256),), ((4, 5, 0, 128), (5, 8, 0, 128), (8, 11, 0, 128))),
    (((128, 256, 0, 1344),), (), ((11, 12, 0, 128), (0, 4, 128, 256), (4, 8, 128, 256), (8, 10, 128, 256))),
    (((256, 448, 0, 1344),), ((256, 448),), ((10, 12, 128, 256),)),
)
WBSLOT, FA1, FB1, LAZY = 38, 28, 64, 8
LA, LB = 26, 32
OPOS = 2
SIMIN = 6
NSTAGE_BUFS = 12
FPIECES = ((384, 512), (512, 768), (768, 896))
PARAMS = {
    "first": dict(FENCE=0, PDELAY=4, DELAY=4, PVOFF=(0, 1, 2), SSTAGE=4, NSB=12, ROT=(0, 2, 0, 2), TAILF=(2, 1, 0, 0, 3)),
    "mid": dict(FENCE=0, PDELAY=4, DELAY=5, PVOFF=(0, 1, 1), SSTAGE=3, NSB=10, ROT=(3, 2, 1, 0), TAILF=(1, 1, 1, 1, 2)),
    "last": dict(FENCE=8, PDELAY=8, DELAY=4, PVOFF=(0, 0, 0), SSTAGE=3, NSB=10, ROT=(3, 2, 1, 0), TAILF=()),
}


def _iota(shape, dim):
    return lax.broadcasted_iota(i32, shape, dim)


def _w(x):
    return pltpu.bitcast(x, u32)


def _b(x):
    return pltpu.bitcast(x, bf16)


def _pack(a, b):
    ua = lax.bitcast_convert_type(a, u32)
    ub = lax.bitcast_convert_type(b, u32)
    return (ua >> 16) | (ub & jnp.uint32(HI))


def _split(n, flip):
    parts = [n // 4 + (1 if k < n % 4 else 0) for k in range(4)]
    if flip:
        parts = parts[::-1]
    return [p for p in parts if p]


def _wait(copies):
    for cp in copies:
        cp.wait()


def _kernel(xa_hbm, xb_hbm, wa_hbm, woa_hbm, wb_hbm, wob_hbm, o_hbm,
            xa_s, xb_s, wa_s, wb_s, woa_s, wob_s, wta_s, wtb_s, wota_s, wotb_s,
            ka_s, kb_s, kwa_s, kwb_s, vta_s, vtb_s, qta_s, qtb_s, ota_s, otb_s, omid_s, mq_s,
            *rest):
    ss_s, (o_s, isem, osem) = rest[:NSTAGE_BUFS], rest[NSTAGE_BUFS:]
    step = pl.program_id(0)
    x_hbm, x_s = (xa_hbm, xb_hbm), (xa_s, xb_s)
    wt_s, wot_s = (wta_s, wtb_s), (wota_s, wotb_s)
    k_s, vt_s, qt_s, ot_s = (ka_s, kb_s), (vta_s, vtb_s), (qta_s, qtb_s), (ota_s, otb_s)
    ksw_s = (kwa_s, kwb_s)

    nsem = [0]

    def icopy(src, dst):
        nsem[0] += 1
        return pltpu.make_async_copy(src, dst, isem.at[nsem[0] - 1])

    def xcopy(b, lo, hi):
        j, o = divmod(lo, 512)
        return icopy(x_hbm[b].at[:, lo:hi], x_s[b].at[j, :, o:o + hi - lo])

    def ocopy(row, c0=0, c1=2 * D):
        return pltpu.make_async_copy(o_s.at[pl.ds(row, 128), c0:c1], o_hbm.at[pl.ds(row, 128), c0:c1], osem.at[0])

    stage_w = [[icopy(wa_hbm.at[k0:k1, c0:c1], wa_s.at[k0:k1, c0:c1]) for k0, k1, c0, c1 in ws]
               for ws, _, _ in STAGES]
    stage_x = [[icopy(xa_hbm.at[k0:k1, 0:512], xa_s.at[0, k0:k1, :]) for k0, k1 in xs] for _, xs, _ in STAGES]
    bcopies = [icopy(wb_hbm, wb_s), xcopy(1, 0, 512), icopy(woa_hbm, woa_s), icopy(wob_hbm, wob_s)]
    xrest = [xcopy(b, lo, lo + 512) for lo in (512, 1024, 1536) for b in range(2)]

    def body(kind):
        first, last = kind == "first", kind == "last"
        prm = PARAMS[kind]
        FENCE, PDELAY, DELAY, PVOFF, SSTAGE, NSB, ROT, TAILF = (
            prm[k] for k in ("FENCE", "PDELAY", "DELAY", "PVOFF", "SSTAGE", "NSB", "ROT", "TAILF"))
        us = {"first": (0, 2, 1), "mid": (3, 4, 5, 6), "last": (15,)}[kind]
        r16 = _iota((16, 128), 0)
        lane16 = _iota((16, 128), 1)
        keyidx = jnp.where(r16 < 8, 2 * r16, 2 * r16 - 15)
        tri_lo = keyidx <= (lane16 & 31)
        tri_hi = keyidx + 16 <= (lane16 & 31)
        g03 = (((lane16 + 32) & 64) == 0)
        sel1 = (lane16 & 32) == 0
        sel2 = (lane16 & 64) == 0
        lo4 = _iota((8, 128), 0) < 4
        left8 = (_iota((8, 128), 1) & 64) == 0
        zero = jnp.zeros((16, 128), u32)
        xcache = {}
        scnt = [0]
        qcnt = [0]
        zdyn = step // 8

        def orow(q):
            if kind == "mid":
                return pl.multiple_of((step - 1) * 512 + 128 * q, 128)
            if FENCE:
                return pl.multiple_of(zdyn * 128 + 128 * q, 128)
            return 128 * q

        q0 = 2 * (us[0] // 2)
        have = {}
        if not first:
            for t in range(4):
                for q in range(q0 - 2, q0 + 2):
                    for b in range(2):
                        for kd in "qkv":
                            have[kd, b, q % 4, t] = q
                for q in range(q0 - 2, q0):
                    have["o", 1, q % 4, t] = q
                    have["o", 0, (q + 2) % 4, t] = q + 2
            for q in range(q0 - 2, q0):
                have["m", 0, q % 4, 2] = have["m", 0, q % 4, 3] = q

        def made(kd, b, q, t):
            have[kd, b, q % 4, t] = q

        def need(kd, b, q, t):
            assert have.get((kd, b, q % 4, t)) == q, (kind, kd, b, q, t)

        cur = [0]
        posts = []

        def later(th):
            posts.append((cur[0] + PDELAY, th))

        def run_posts(upto):
            while posts and posts[0][0] <= upto:
                posts.pop(0)[1]()

        def ring(q):
            return slice(128 * (q % 4), 128 * (q % 4) + 128)

        def proj(b, q, part, t):
            r0 = part * (D // 2) + 56 * t
            if (b, q) not in xcache:
                j, o = divmod(128 * q, 512)
                xcache[b, q] = x_s[b][j + step - 1 if kind == "mid" else j, :, o:o + 128]
            y = jnp.dot(_b(wt_s[b][r0:r0 + 56, :]), xcache[b, q], preferred_element_type=f32)
            proj_post(b, q, part, t, y)

        def proj_post(b, q, part, t, y):
            made("qkv"[part], b, q, t)
            if part == 0:
                y = y * QSCALE
                r1 = pltpu.roll(y[24:56], 96, 1)
                r2 = pltpu.roll(y[56:88], 64, 1)
                r3 = pltpu.roll(y[80:112], 32, 1)
                z8 = jnp.zeros((8, 128), f32)
                qr = jnp.concatenate([
                    y[0:24], jnp.where(lo4, y[24:32], r1[0:8]), r1[8:32], z8,
                    r2[0:24], jnp.where(lo4, r2[24:32], r3[0:8]), r3[8:32], z8], axis=0)
                qt_s[b][64*t:64*t + 64, ring(q)] = _w(qr.astype(bf16))
            elif part == 1:
                z8 = jnp.zeros((8, 128), f32)
                kt = jnp.concatenate([y[0:56], z8, y[56:112], z8], axis=0)
                kw = _w(kt.astype(bf16).T)
                ev = lax.bitcast_convert_type(kw << 16, f32)
                od = lax.bitcast_convert_type(kw & jnp.uint32(HI), f32)
                kk = _w(jnp.concatenate([z[8*i:8*i + 8] for i in range(8) for z in (ev, od)], axis=0).astype(bf16))
                if q >= 2:
                    hi = jnp.concatenate([kk[8*u:8*u + 8] for u in (1, 3, 5, 7)], axis=0)
                    ksw_s[b][32*(q % 4):32*(q % 4) + 32, 128*t:128*t + 128] = pltpu.roll(hi, 64, 1)
                k_s[b][64*(q % 4):64*(q % 4) + 64, 128*t:128*t + 128] = kk
            else:
                v = jnp.concatenate([
                    y[0:24], jnp.where(lo4, y[24:32], 1.0), jnp.where(lo4, 1.0, y[24:32]), y[32:56],
                    y[56:80], jnp.where(lo4, y[80:88], 1.0), jnp.where(lo4, 1.0, y[80:88]), y[88:112]], axis=0)
                vt_s[b][64*t:64*t + 64, ring(q)] = _w(v.astype(bf16))

        def kload(b, t, off, n):
            lo = off % 256
            if lo + n <= 256:
                return k_s[b][lo:lo + n, 128*t:128*t + 128]
            return jnp.concatenate([k_s[b][lo:256, 128*t:128*t + 128],
                                    k_s[b][0:lo + n - 256, 128*t:128*t + 128]], axis=0)

        def fence_zero():
            return _w(o_s[pl.ds(pl.multiple_of(S + 16 * zdyn, 16), 16), 0:128])

        xch = {}

        def edge(b, q, t, c):
            q32 = qt_s[b][64*t:64*t + 64, ring(q)]
            f_lo = kload(b, t, 64 * q + 16 * c - 128, 8)
            l_hi = ksw_s[b][32*(q % 4) + 8*c:32*(q % 4) + 8*c + 8, 128*t:128*t + 128]
            za = jnp.dot(_b(jnp.where(left8, f_lo, l_hi)),
                         _b(jnp.concatenate([q32[0:32], q32[0:32]], axis=0) & mq_s[4 + c]),
                         preferred_element_type=f32)
            zb = jnp.dot(_b(jnp.where(left8, l_hi, f_lo)),
                         _b(jnp.concatenate([q32[32:64], q32[32:64]], axis=0) & mq_s[8 + c]),
                         preferred_element_type=f32)
            g = g03 if c % 2 == 0 else sel2
            if c >= 2:
                za, zb = zb, za
            xch[c, "m"] = jnp.where(g, za, zb)
            xch[(c + 2) % 4, "p"] = jnp.where(g, zb, za)

        def qk(b, q, t, c):
            imin = max(0, 8 - 4 * q - c)
            need("q", b, q, t)
            for qq in range(max(0, q - 2), q + 1):
                need("k", b, qq, t)
            q32 = qt_s[b][64*t:64*t + 64, ring(q)]
            w = q32 & mq_s[c]
            if FENCE and cur[0] % FENCE == 0:
                w = jnp.concatenate([w[0:56], w[56:64] | fence_zero()], axis=0)
            w = _b(w)
            off = 64 * q + 16 * c - 128
            if imin == 0:
                pu = 4 if c < 2 else 13
                mids = [u for u in range(2, 16) if u != pu]
                plan = [mids[0:2] + [1, 16], mids[2:6], mids[6:10], mids[10:13]]
                rot = ROT[qcnt[0] % 4]
                plan = plan[rot:] + plan[:rot]
                qcnt[0] += 1
            else:
                plan, o = [], 2 * imin
                for n in _split(2 * (9 - imin), c % 2):
                    plan.append(list(range(o, o + n)))
                    o += n
            ch = {}
            for chunks in plan:
                runs = []
                for u in chunks:
                    if runs and runs[-1][0] + runs[-1][1] == u:
                        runs[-1][1] += 1
                    else:
                        runs.append([u, 1])
                kw = [kload(b, t, off + 8 * u, 8 * n) for u, n in runs]
                kw = kw[0] if len(kw) == 1 else jnp.concatenate(kw, axis=0)
                z = jnp.dot(_b(kw), w, preferred_element_type=f32)
                for k, u in enumerate(chunks):
                    ch[u] = z[16*k:16*k + 16]
            if imin == 0:
                mm = xch.pop((c, "m"))
                ch[pu] = xch.pop((c, "p"))
                s_lo = jnp.where(tri_lo, ch[16], mm)
                s_hi = jnp.where(tri_hi, mm, ch[1])
            else:
                s_lo = jnp.where(tri_lo, ch[16], NEG)
                s_hi = jnp.where(tri_hi, ch[17], NEG)
            mx = [s_lo, s_hi]
            for u in range(2 * max(imin, 1), 16):
                mx[u % 2] = jnp.maximum(mx[u % 2], ch[u])
            m = jnp.max(jnp.maximum(mx[0], mx[1]), axis=0, keepdims=True)
            if imin <= SIMIN:
                sref = ss_s[scnt[0] % NSB]
                scnt[0] += 1
                early = [u for chunks in plan
                         for u in chunks[:SSTAGE if imin == 0 else min(SSTAGE, len(chunks) - 1)] if 2 <= u < 16]
                if imin == 0:
                    early = [pu] + early
                for u in early:
                    sref[0, 16*u:16*u + 16, :] = ch[u]
            else:
                early, sref = [], None
            born = scnt[0]

            def pk(p):
                return _pack(p[0:8], p[8:16])

            def finish():
                assert scnt[0] - born < NSB
                for u in early:
                    ch[u] = sref[zdyn, 16*u:16*u + 16, :]
                p_lo = jnp.exp2(s_lo - m)
                p_hi = jnp.exp2(s_hi - m)
                X = [None] * 9
                for i in range(max(imin, 1), 8):
                    X[i] = jnp.concatenate([pk(jnp.exp2(ch[2*i] - m)), pk(jnp.exp2(ch[2*i + 1] - m))], axis=0)
                if imin == 0:
                    X[0] = jnp.concatenate([pk(jnp.where(tri_lo, 0.0, p_lo)),
                                            pk(jnp.where(tri_hi, 0.0, p_hi))], axis=0)
                    p_lo = jnp.where(tri_lo, p_lo, 0.0)
                    p_hi = jnp.where(tri_hi, p_hi, 0.0)
                X[8] = jnp.concatenate([pk(p_lo), pk(p_hi)], axis=0)
                return X
            return finish if first and WBSLOT - LAZY < cur[0] <= WBSLOT else finish()

        def pv(b, q, t, X, T, acc):
            if q + T < 2:
                return acc
            need("v", b, q + T - 2, t)
            zz = zero
            if last and (b, q, t, T) == (1, NT - 1, 0, 0):
                fz = fence_zero()
                zz = jnp.concatenate([fz, fz], axis=0)

            def sel(m, a, bb):
                if a is None and bb is None:
                    return None
                return jnp.where(m, zz if a is None else a, zz if bb is None else bb)
            Y = [[] for _ in range(4)]
            for B in range(4*T, 4*T + 4):
                xs = [X[c][B - c] if 0 <= B - c <= 8 else None for c in range(4)]
                a = [sel(sel1, xs[k], xs[(k + 1) % 4]) for k in range(4)]
                for j in range(4):
                    y = sel(sel2, a[j], a[(j + 2) % 4])
                    Y[j].append(zero if y is None else y)
            res = []
            for j in range(4):
                h = 4*t + j
                p = _b(jnp.concatenate(Y[j], axis=0))
                vt = _b(vt_s[b][16*h:16*h + 16, ring(q + T - 2)])
                o = jnp.dot(vt, p, preferred_element_type=f32)
                res.append(o if acc is None else o + acc[j])
            return res

        def fin(b, q, t, acc):
            made("o", b, q, t)
            outs = []
            for j in range(4):
                o = acc[j]
                den = o[28:29] if j % 2 == 0 else o[0:1]
                o = o * (1.0 / den)
                if j:
                    o = pltpu.roll(o, 32*j, 1)
                outs.append(o)
            oc = jnp.concatenate([
                outs[0][0:24], jnp.where(lo4, outs[0][24:32], outs[1][0:8]), outs[1][8:32],
                outs[2][0:24], jnp.where(lo4, outs[2][24:32], outs[3][0:8]), outs[3][8:32]], axis=0)
            ot_s[b][56*t:56*t + 56, ring(q)] = _w(oc.astype(bf16))

        ohold = {}

        def put(q, c0, c1, val):
            row = orow(q)
            o_s[pl.ds(row, 128), c0:c1] = val.astype(bf16).T
            if q == NT - 1:
                ocopy(row, c0, c1).start()
            elif c1 == 2 * D:
                ocopy(row).start()

        def outp(b, q, n):
            for t in range(4):
                need("o", b, q, t)
            r0, r1 = ((0, 128, 256, 384, 448) if b == 0 else (0, 64, 192, 320, 448))[n:n + 2]
            y = jnp.dot(_b(wot_s[b][r0 // 2:r1 // 2, :]), _b(ot_s[b][:, ring(q)]),
                        preferred_element_type=f32)

            def post():
                if b == 0:
                    if n == 0:
                        ohold[q] = y
                    elif n == 1:
                        put(q, 0, 256, jnp.concatenate([ohold.pop(q), y], axis=0))
                    elif n == 2 and q == NT - 1:
                        put(q, 256, 384, y)
                    else:
                        made("m", 0, q, n)
                        omid_s[q % 4, 128 * (n - 2):r1 - 256] = y
                else:
                    if n == 0:
                        need("m", 0, q, 2)
                        need("m", 0, q, 3)
                        put(q, 256, 512, jnp.concatenate([omid_s[q % 4], y], axis=0))
                    elif n == 1:
                        ohold[q] = y
                    elif n == 2:
                        put(q, 512, 768, jnp.concatenate([ohold.pop(q), y], axis=0))
                    else:
                        put(q, 768, 896, y)
            later(post)

        def final_out():
            q = NT - 1
            for t in range(4):
                need("o", 1, q, t)
            need("m", 0, q, 3)
            parts = []
            sets = [list(range(n, 28, 4)) for n in range(4)]
            for k0, k1 in ((128, D), (0, 128)):
                rhs = _b(ot_s[1][k0 // 2:k1 // 2, ring(q)])
                ys = [jnp.dot(_b(jnp.concatenate([wot_s[1][8*u:8*u + 8, k0:k1] for u in st], axis=0)), rhs,
                              preferred_element_type=f32) for st in sets]
                parts = [y + p for y, p in zip(ys, parts)] if parts else ys
            ch = {u: p[16*i:16*i + 16] for st, p in zip(sets, parts) for i, u in enumerate(st)}
            y = jnp.concatenate([omid_s[q % 4, 128:192]] + [ch[u] for u in range(28)], axis=0)
            for c0, c1 in FPIECES:
                put(q, c0, c1, y[c0 - 384:c1 - 384])

        def wtile(src, dst, i, ncol):
            c0, c1 = 128 * i, min(128 * i + 128, ncol)
            dst[c0 // 2:c1 // 2, :] = _w(src[:, c0:c1].T)

        def projs(u):
            s, b = divmod(u, 2)
            return [(lambda p=p, t=t, q=q: proj(b, q, p, t))
                    for p in (1, 0, 2) for q in (2*s, 2*s + 1) for t in range(4)]

        def outs(u, qi):
            s, b = divmod(u, 2)
            return [(lambda n=n: outp(b, 2*s + qi, n)) for n in range(4)]

        groups = [(u % 2, 2 * (u // 2) + qi, t) for u in us for qi in range(2) for t in range(4)]
        if last:
            groups = [(1, NT - 2, t) for t in range(4)] + [(1, NT - 1, t) for t in (3, 2, 1, 0)]
        N = len(groups)
        Xs = [[None] * 4 for _ in range(N)]
        accs = [None] * N

        def emit_pv(slot):
            for T in range(3):
                r = slot - 3 - DELAY - PVOFF[T]
                if r >= 0 and r % 4 == 0 and r // 4 < N:
                    g = r // 4
                    Xs[g] = [x() if callable(x) else x for x in Xs[g]]
                    accs[g] = pv(*groups[g], Xs[g], T, accs[g])
                    if T == 2:
                        fin(*groups[g], accs[g])
                        Xs[g] = accs[g] = None

        fill = {}

        def spread(thunks, lo, hi):
            n = len(thunks)
            for k, th in enumerate(thunks):
                fill.setdefault(lo + (k * (hi - lo)) // n, []).append(th)

        ntail = sum(TAILF)
        if first:
            for cw, cx in zip(stage_w, stage_x):
                for cp in cw + cx:
                    cp.start()
            for cp in bcopies:
                cp.start()
            row = _iota((64, 128), 0)
            lane = _iota((64, 128), 1)
            half, hh, l, jlo = row // 32, (row % 32) // 14, lane // 32, (lane & 16) == 0
            ok = hh < 2
            o_s[S:S + 16, :] = jnp.zeros((16, 2 * D), bf16)

            def bits(m):
                return jnp.where(m & ok, jnp.uint32(0xFFFFFFFF), jnp.uint32(0))
            for c in range(4):
                mq_s[c] = bits(((2 * half + hh + l) & 3) == c)
                for k in range(2):
                    sb = (2 * k + hh + l) & 3
                    isf = half == k
                    own = (sb == c) & (isf == jlo)
                    other = (sb == (c + 2) % 4) & (isf if c >= 2 else ~isf)
                    mq_s[4 + 4 * k + c] = bits(own | other)

            def wsub(k0, k1, c0, c1):
                for c in range(c0, c1, 128):
                    ce = min(c + 128, c1)
                    wta_s[c // 2:ce // 2, k0:k1] = _w(wa_s[k0:k1, c:ce].T)
            part_sum = {}
            for i, (ws, xs, work) in enumerate(STAGES):
                _wait(stage_w[i] + (stage_x[i] if i else []))
                for blk in ws:
                    wsub(*blk)
                if i == 0:
                    _wait(stage_x[0])
                if i == len(STAGES) - 1:
                    for cp in xrest:
                        cp.start()
                for n0, n1, k0, k1 in work:
                    y = jnp.dot(_b(wta_s[56 * n0:56 * n1, k0:k1]), xa_s[0, k0:k1, :], preferred_element_type=f32)
                    for n in range(n0, n1):
                        z = y[112 * (n - n0):112 * (n - n0) + 112]
                        assert part_sum.get(n, (None, 0))[1] == k0
                        part_sum[n] = (z if k0 == 0 else z + part_sum[n][0], k1)
            xfin = {}
            held = []

            def proj_fin(qp, n, defer=False):
                z, k0 = part_sum[n]
                if (qp, k0) not in xfin:
                    xfin[qp, k0] = xa_s[0, k0:D, 256 * qp:256 * qp + 256]
                y = jnp.dot(_b(wta_s[56 * n:56 * n + 56, k0:D]), xfin[qp, k0], preferred_element_type=f32)
                y = y + z[:, 256 * qp:256 * qp + 256]

                def post():
                    for i in range(2):
                        proj_post(0, 2 * qp + i, n // 4, n % 4, y[:, 128 * i:128 * i + 128])
                if defer:
                    held.append(post)
                else:
                    post()
            for n in range(12):
                proj_fin(0, n)

            def b_prep():
                _wait(bcopies)
                held.pop()()
                for ti in range(11):
                    wtile(wb_s, wtb_s, ti, 3 * D)
                for ti in range(4):
                    wtile(woa_s, wota_s, ti, D)
                    wtile(wob_s, wotb_s, ti, D)
            spread([(lambda n=n: proj_fin(1, n)) for n in (4, 5, 6, 7, 0, 1, 2, 3)], 0, FA1)
            spread([(lambda n=n: proj_fin(1, n)) for n in (8, 9, 10)], FA1, WBSLOT)
            fill.setdefault(WBSLOT, []).extend([lambda: proj_fin(1, 11, defer=True), b_prep])
            spread([(lambda p=p, t=t, q=q: proj(1, q, p, t))
                    for q, order in ((0, (0, 1, 2)), (1, (1, 0, 2))) for p in order for t in range(4)],
                   WBSLOT + 2, FB1)
            more = outs(0, 0) + outs(0, 1) + projs(3)
            spread(more[:len(more) - ntail], FB1, 96)
            tail = more[len(more) - ntail:]
        elif not last:
            pslots = [s for s in range(32) if s % 4 != OPOS]
            for k, u in enumerate(us):
                p = projs(u + 1)
                if u == us[-1]:
                    p, tail = p[:24 - ntail], p[24 - ntail:]
                for i, th in enumerate(p):
                    fill.setdefault(32 * k + pslots[(i * 24) // len(p)], []).append(th)
                for i, th in enumerate(outs(u - 2, 0) + outs(u - 2, 1)):
                    fill.setdefault(32 * k + 4 * i + OPOS, []).append(th)
        else:
            oa = outs(14, 1)
            spread(outs(13, 0) + outs(13, 1) + outs(14, 0) + oa[:2], 0, LA)
            spread(outs(15, 0), LA, LB)
            tail = oa[2:]

        slot = 0
        for g in range(N):
            pat = "a0f2fb1f3f" if groups[g][1] >= 2 else "0f2f1f3f"
            if g == 0 and kind == "mid":
                pat = "fa02fb1f3f"
            for tok in pat:
                cur[0] = slot
                if tok in "ab":
                    need("q", *groups[g])
                    need("k", *groups[g])
                    edge(*groups[g], "ab".index(tok))
                    edge(*groups[g], "ab".index(tok) + 2)
                elif tok == "f":
                    emit_pv(slot)
                    for th in fill.get(slot, []):
                        th()
                    slot += 1
                    run_posts(slot)
                else:
                    Xs[g][int(tok)] = qk(*groups[g], int(tok))

        def take(n):
            for _ in range(n):
                tail.pop(0)()
        nd = DELAY + max(PVOFF)
        if last:
            run_posts(10**9)
            take(len(tail))
            for k in range(nd):
                emit_pv(slot)
                slot += 1
            run_posts(10**9)
            final_out()
            _wait([ocopy(128 * q) for q in range(NT - 1)]
                  + [ocopy(128 * (NT - 1), c0, c1) for c0, c1 in ((0, 256), (256, 384)) + FPIECES])
            return
        for k in range(nd):
            if k < len(TAILF) - 1:
                take(TAILF[k])
            emit_pv(slot)
            slot += 1
        take(len(tail))
        run_posts(10**9)
        if first:
            _wait(xrest)

    pl.when(step == 0)(lambda: body("first"))
    pl.when(jnp.logical_and(step > 0, step < 4))(lambda: body("mid"))
    pl.when(step == 4)(lambda: body("last"))


@jax.jit
def pallas_concat_heads__sliding_block__sliding_block__prompt_kernel(
    A_x: jax.Array,
    A_wqkv: jax.Array,
    A_wo: jax.Array,
    B_x: jax.Array,
    B_wqkv: jax.Array,
    B_wo: jax.Array,
):
    xa = A_x.reshape(S, D).T
    xb = B_x.reshape(S, D).T
    V = pltpu.VMEM

    def two(shape, dtype):
        return [V(shape, dtype), V(shape, dtype)]

    scratch = (
        two((4, D, 512), bf16)
        + two((D, 3 * D), bf16) + two((D, D), bf16)
        + two((3 * D // 2, D), u32) + two((D // 2, D), u32)
        + two((256, 512), u32) + two((128, 512), u32)
        + two((256, 512), u32)
        + two((256, 512), u32) + two((D // 2, 512), u32)
        + [V((4, 192, 128), f32), V((12, 64, 128), u32)]
        + [V((1, 256, 128), f32)] * NSTAGE_BUFS
        + [V((S + 16, 2 * D), bf16),
           pltpu.SemaphoreType.DMA((24,)),
           pltpu.SemaphoreType.DMA((1,))])
    out = pl.pallas_call(
        _kernel,
        grid=(5,),
        in_specs=[pl.BlockSpec(memory_space=pl.ANY)] * 6,
        out_specs=pl.BlockSpec(memory_space=pl.ANY),
        out_shape=jax.ShapeDtypeStruct((S, 2 * D), bf16),
        scratch_shapes=scratch,
        compiler_params=pltpu.CompilerParams(
            dimension_semantics=("arbitrary",), vmem_limit_bytes=100 * 1024 * 1024,
            disable_semaphore_checks=True, disable_bounds_checks=True),
    )(xa, xb, A_wqkv, A_wo, B_wqkv, B_wo)
    return out.reshape(1, S, 2 * D)
```

```python
import math

import jax
import jax.numpy as jnp
from jax import lax
import jax.experimental.pallas as pl
import jax.experimental.pallas.tpu as pltpu

S, D, H, DH, W = 2048, 448, 16, 28, 256
NT = S // 128
NEG = -1e30
QSCALE = (DH ** -0.5) * math.log2(math.e)
f32, bf16, i32, u32 = jnp.float32, jnp.bfloat16, jnp.int32, jnp.uint32
HI = 0xFFFF0000

STAGES = (
    (((0, 128, 0, 640),), ((0, 128),), ((0, 4, 0, 128),)),
    (((0, 128, 640, 1344),), ((128, 256),), ((4, 5, 0, 128), (5, 8, 0, 128), (8, 11, 0, 128))),
    (((128, 256, 0, 1344),), (), ((11, 12, 0, 128), (0, 4, 128, 256), (4, 8, 128, 256), (8, 10, 128, 256))),
    (((256, 448, 0, 1344),), ((256, 448),), ((10, 12, 128, 256),)),
)
WBSLOT, FA1, FB1, LAZY = 38, 26, 68, 6
LA, LB = 27, 30
OPOS = 2
SIMIN = 4
NSTAGE_BUFS = 12
FPIECES = ((384, 512), (512, 768), (768, 896))
PARAMS = {
    "first": dict(FENCE=0, PDELAY=8, DELAY=4, PVOFF=(0, 1, 2), SSTAGE=4, NSB=12, TAILF=(2, 1, 0, 0, 3)),
    "mid": dict(FENCE=0, PDELAY=8, DELAY=5, PVOFF=(0, 1, 1), SSTAGE=3, NSB=10, TAILF=(1, 1, 1, 1, 3)),
    "last": dict(FENCE=8, PDELAY=4, DELAY=4, PVOFF=(0, 0, 0), SSTAGE=3, NSB=12, TAILF=()),
}


def _iota(shape, dim):
    return lax.broadcasted_iota(i32, shape, dim)


def _w(x):
    return pltpu.bitcast(x, u32)


def _b(x):
    return pltpu.bitcast(x, bf16)


def _pack(a, b):
    ua = lax.bitcast_convert_type(a, u32)
    ub = lax.bitcast_convert_type(b, u32)
    return (ua >> 16) | (ub & jnp.uint32(HI))


def _wait(copies):
    for cp in copies:
        cp.wait()


def _kernel(xa_hbm, xb_hbm, wa_hbm, woa_hbm, wb_hbm, wob_hbm, o_hbm,
            xa_s, xb_s, wa_s, wb_s, woa_s, wob_s, wta_s, wtb_s, wota_s, wotb_s,
            ka_s, kb_s, vta_s, vtb_s, qta_s, qtb_s, ota_s, otb_s, omid_s, mq_s,
            *rest):
    ss_s, (o_s, isem, osem) = rest[:NSTAGE_BUFS], rest[NSTAGE_BUFS:]
    step = pl.program_id(0)
    x_hbm, x_s = (xa_hbm, xb_hbm), (xa_s, xb_s)
    wt_s, wot_s = (wta_s, wtb_s), (wota_s, wotb_s)
    k_s, vt_s, qt_s, ot_s = (ka_s, kb_s), (vta_s, vtb_s), (qta_s, qtb_s), (ota_s, otb_s)

    nsem = [0]

    def icopy(src, dst):
        nsem[0] += 1
        return pltpu.make_async_copy(src, dst, isem.at[nsem[0] - 1])

    def xcopy(b, lo, hi):
        j, o = divmod(lo, 512)
        return icopy(x_hbm[b].at[:, lo:hi], x_s[b].at[j, :, o:o + hi - lo])

    def ocopy(row, c0=0, c1=2 * D):
        return pltpu.make_async_copy(o_s.at[pl.ds(row, 128), c0:c1], o_hbm.at[pl.ds(row, 128), c0:c1], osem.at[0])

    stage_w = [[icopy(wa_hbm.at[k0:k1, c0:c1], wa_s.at[k0:k1, c0:c1]) for k0, k1, c0, c1 in ws]
               for ws, _, _ in STAGES]
    stage_x = [[icopy(xa_hbm.at[k0:k1, 0:512], xa_s.at[0, k0:k1, :]) for k0, k1 in xs] for _, xs, _ in STAGES]
    bcopies = [icopy(wb_hbm, wb_s), xcopy(1, 0, 512), icopy(woa_hbm, woa_s), icopy(wob_hbm, wob_s)]
    xrest = [xcopy(b, lo, lo + 512) for lo in (512, 1024, 1536) for b in range(2)]

    def body(kind):
        first, last = kind == "first", kind == "last"
        prm = PARAMS[kind]
        FENCE, PDELAY, DELAY, PVOFF, SSTAGE, NSB, TAILF = (
            prm[k] for k in ("FENCE", "PDELAY", "DELAY", "PVOFF", "SSTAGE", "NSB", "TAILF"))
        us = {"first": (0, 2, 1), "mid": (3, 4, 5, 6), "last": (15,)}[kind]
        r16 = _iota((16, 128), 0)
        lane16 = _iota((16, 128), 1)
        keyidx = jnp.where(r16 < 8, 2 * r16, 2 * r16 - 15)
        tri_lo = keyidx <= (lane16 & 31)
        tri_hi = keyidx + 16 <= (lane16 & 31)
        g03 = (((lane16 + 32) & 64) == 0)
        sel1 = (lane16 & 32) == 0
        sel2 = (lane16 & 64) == 0
        lo4 = _iota((8, 128), 0) < 4
        left8 = (_iota((8, 128), 1) & 64) == 0
        zero = jnp.zeros((16, 128), u32)
        xcache = {}
        scnt = [0]
        zdyn = step // 8

        def orow(q):
            if kind == "mid":
                return pl.multiple_of((step - 1) * 512 + 128 * q, 128)
            if FENCE:
                return pl.multiple_of(zdyn * 128 + 128 * q, 128)
            return 128 * q

        q0 = 2 * (us[0] // 2)
        have = {}
        if not first:
            for t in range(4):
                for q in range(q0 - 2, q0 + 2):
                    for b in range(2):
                        for kd in "qkv":
                            have[kd, b, q % 4, t] = q
                for q in range(q0 - 2, q0):
                    have["o", 1, q % 4, t] = q
                    have["o", 0, (q + 2) % 4, t] = q + 2
            for q in range(q0 - 2, q0):
                have["m", 0, q % 4, 2] = have["m", 0, q % 4, 3] = q

        def made(kd, b, q, t):
            have[kd, b, q % 4, t] = q

        def need(kd, b, q, t):
            assert have.get((kd, b, q % 4, t)) == q, (kind, kd, b, q, t)

        cur = [0]
        posts = []

        def later(th):
            posts.append((cur[0] + PDELAY, th))

        def run_posts(upto):
            while posts and posts[0][0] <= upto:
                posts.pop(0)[1]()

        def ring(q):
            return slice(128 * (q % 4), 128 * (q % 4) + 128)

        def proj(b, q, part, t):
            r0 = part * (D // 2) + 56 * t
            if (b, q) not in xcache:
                j, o = divmod(128 * q, 512)
                xcache[b, q] = x_s[b][j + step - 1 if kind == "mid" else j, :, o:o + 128]
            y = jnp.dot(_b(wt_s[b][r0:r0 + 56, :]), xcache[b, q], preferred_element_type=f32)
            proj_post(b, q, part, t, y)

        def proj_post(b, q, part, t, y):
            made("qkv"[part], b, q, t)
            if part == 0:
                y = y * QSCALE
                r1 = pltpu.roll(y[24:56], 96, 1)
                r2 = pltpu.roll(y[56:88], 64, 1)
                r3 = pltpu.roll(y[80:112], 32, 1)
                z8 = jnp.zeros((8, 128), f32)
                qr = jnp.concatenate([
                    y[0:24], jnp.where(lo4, y[24:32], r1[0:8]), r1[8:32], z8,
                    r2[0:24], jnp.where(lo4, r2[24:32], r3[0:8]), r3[8:32], z8], axis=0)
                qt_s[b][64*t:64*t + 64, ring(q)] = _w(qr.astype(bf16))
            elif part == 1:
                z8 = jnp.zeros((8, 128), f32)
                evc = (_iota((56, 128), 1) & 16) == 0
                kt = jnp.concatenate([jnp.where(evc, y[0:56], y[56:112]), z8,
                                      jnp.where(evc, y[56:112], y[0:56]), z8], axis=0)
                kw = _w(kt.astype(bf16).T)
                ev = lax.bitcast_convert_type(kw << 16, f32)
                od = lax.bitcast_convert_type(kw & jnp.uint32(HI), f32)
                kk = _w(jnp.concatenate([z[8*i:8*i + 8] for i in range(8) for z in (ev, od)], axis=0).astype(bf16))
                k_s[b][64*(q % 4):64*(q % 4) + 64, 128*t:128*t + 128] = kk
            else:
                v = jnp.concatenate([
                    y[0:24], jnp.where(lo4, y[24:32], 1.0), jnp.where(lo4, 1.0, y[24:32]), y[32:56],
                    y[56:80], jnp.where(lo4, y[80:88], 1.0), jnp.where(lo4, 1.0, y[80:88]), y[88:112]], axis=0)
                vt_s[b][64*t:64*t + 64, ring(q)] = _w(v.astype(bf16))

        def kload(b, t, off):
            return k_s[b][off % 256:off % 256 + 8, 128*t:128*t + 128]

        def fence_zero():
            return _w(o_s[pl.ds(pl.multiple_of(S + 16 * zdyn, 16), 16), 0:128])

        xch = {}

        def edge(b, q, t, c):
            q32 = qt_s[b][64*t:64*t + 64, ring(q)]
            f_lo = kload(b, t, 64 * q + 16 * c - 128)
            l_hi = kload(b, t, 64 * q + 16 * c + 8)
            za = jnp.dot(_b(jnp.where(left8, f_lo, l_hi)),
                         _b(jnp.concatenate([q32[0:32], q32[0:32]], axis=0) & mq_s[4 + c]),
                         preferred_element_type=f32)
            zb = jnp.dot(_b(jnp.where(left8, l_hi, f_lo)),
                         _b(jnp.concatenate([q32[32:64], q32[32:64]], axis=0) & mq_s[8 + c]),
                         preferred_element_type=f32)
            g = g03 if c % 2 == 0 else sel2
            if c >= 2:
                za, zb = zb, za
            xch[c, "m"] = jnp.where(g, za, zb)
            xch[(c + 2) % 4, "p"] = jnp.where(g, zb, za)

        def qk(b, q, t, c):
            imin = max(0, 8 - 4 * q - c)
            need("q", b, q, t)
            for qq in range(max(0, q - 2), q + 1):
                need("k", b, qq, t)
            q32 = qt_s[b][64*t:64*t + 64, ring(q)]
            w = q32 & mq_s[c]
            if FENCE and cur[0] % FENCE == 0:
                w = jnp.concatenate([w[0:56], w[56:64] | fence_zero()], axis=0)
            wpar = (_b(w), _b(jnp.concatenate([w[32:64], w[0:32]], axis=0)))
            off = 64 * q + 16 * c - 128
            if imin == 0:
                pu = 4 if c < 2 else 13
                ev = [u for u in range(2, 16, 2) if u != pu]
                od = [u for u in range(3, 16, 2) if u != pu]
                plan = [od[0:4], ev[0:4], od[4:] + [1], ev[4:] + [16]]
            else:
                plan = []
                for par in ((0, 1) if c % 2 == 0 else (1, 0)):
                    same = list(range(2 * imin + par, 18, 2))
                    plan += [same[:(len(same) + 1) // 2], same[(len(same) + 1) // 2:]]
            plan = sorted([chunks for chunks in plan if chunks], key=lambda chunks: -len(chunks))
            ch = {}
            for chunks in plan:
                kw = [kload(b, t, off + 8 * u) for u in chunks]
                kw = kw[0] if len(kw) == 1 else jnp.concatenate(kw, axis=0)
                z = jnp.dot(_b(kw), wpar[chunks[0] % 2], preferred_element_type=f32)
                for k, u in enumerate(chunks):
                    ch[u] = z[16*k:16*k + 16]
            if imin == 0:
                mm = xch.pop((c, "m"))
                ch[pu] = xch.pop((c, "p"))
                s_lo = jnp.where(tri_lo, ch[16], mm)
                s_hi = jnp.where(tri_hi, mm, ch[1])
            else:
                s_lo = jnp.where(tri_lo, ch[16], NEG)
                s_hi = jnp.where(tri_hi, ch[17], NEG)
            mx = [s_lo, s_hi]
            for u in range(2 * max(imin, 1), 16):
                mx[u % 2] = jnp.maximum(mx[u % 2], ch[u])
            m = jnp.max(jnp.maximum(mx[0], mx[1]), axis=0, keepdims=True)
            if imin <= SIMIN:
                sref = ss_s[scnt[0] % NSB]
                scnt[0] += 1
                early = [u for chunks in plan
                         for u in chunks[:SSTAGE if imin == 0 else min(SSTAGE, len(chunks) - 1)] if 2 <= u < 16]
                if imin == 0:
                    early = [pu] + early
                for u in early:
                    sref[0, 16*u:16*u + 16, :] = ch[u]
            else:
                early, sref = [], None
            born = scnt[0]

            def pk(p):
                return _pack(p[0:8], p[8:16])

            def finish():
                assert scnt[0] - born < NSB
                for u in early:
                    ch[u] = sref[zdyn, 16*u:16*u + 16, :]
                p_lo = jnp.exp2(s_lo - m)
                p_hi = jnp.exp2(s_hi - m)
                X = [None] * 9
                for i in range(max(imin, 1), 8):
                    X[i] = jnp.concatenate([pk(jnp.exp2(ch[2*i] - m)), pk(jnp.exp2(ch[2*i + 1] - m))], axis=0)
                if imin == 0:
                    X[0] = jnp.concatenate([pk(jnp.where(tri_lo, 0.0, p_lo)),
                                            pk(jnp.where(tri_hi, 0.0, p_hi))], axis=0)
                    p_lo = jnp.where(tri_lo, p_lo, 0.0)
                    p_hi = jnp.where(tri_hi, p_hi, 0.0)
                X[8] = jnp.concatenate([pk(p_lo), pk(p_hi)], axis=0)
                return X
            return finish if first and WBSLOT - LAZY < cur[0] <= WBSLOT else finish()

        def pv(b, q, t, X, T, acc):
            if q + T < 2:
                return acc
            need("v", b, q + T - 2, t)
            zz = zero
            if last and (b, q, t, T) == (1, NT - 1, 0, 0):
                fz = fence_zero()
                zz = jnp.concatenate([fz, fz], axis=0)

            def sel(m, a, bb):
                if a is None and bb is None:
                    return None
                return jnp.where(m, zz if a is None else a, zz if bb is None else bb)
            Y = [[] for _ in range(4)]
            for B in range(4*T, 4*T + 4):
                xs = [X[c][B - c] if 0 <= B - c <= 8 else None for c in range(4)]
                a = [sel(sel1, xs[k], xs[(k + 1) % 4]) for k in range(4)]
                for j in range(4):
                    y = sel(sel2, a[j], a[(j + 2) % 4])
                    Y[j].append(zero if y is None else y)
            res = []
            for j in range(4):
                h = 4*t + j
                p = _b(jnp.concatenate(Y[j], axis=0))
                vt = _b(vt_s[b][16*h:16*h + 16, ring(q + T - 2)])
                o = jnp.dot(vt, p, preferred_element_type=f32)
                res.append(o if acc is None else o + acc[j])
            return res

        def fin(b, q, t, acc):
            made("o", b, q, t)
            outs = []
            for j in range(4):
                o = acc[j]
                den = o[28:29] if j % 2 == 0 else o[0:1]
                o = o * (1.0 / den)
                if j:
                    o = pltpu.roll(o, 32*j, 1)
                outs.append(o)
            oc = jnp.concatenate([
                outs[0][0:24], jnp.where(lo4, outs[0][24:32], outs[1][0:8]), outs[1][8:32],
                outs[2][0:24], jnp.where(lo4, outs[2][24:32], outs[3][0:8]), outs[3][8:32]], axis=0)
            ot_s[b][56*t:56*t + 56, ring(q)] = _w(oc.astype(bf16))

        ohold = {}

        def put(q, c0, c1, val):
            row = orow(q)
            o_s[pl.ds(row, 128), c0:c1] = val.astype(bf16).T
            if q == NT - 1:
                ocopy(row, c0, c1).start()
            elif c1 == 2 * D:
                ocopy(row).start()

        def outp(b, q, n):
            for t in range(4):
                need("o", b, q, t)
            r0, r1 = ((0, 128, 256, 384, 448) if b == 0 else (0, 64, 192, 320, 448))[n:n + 2]
            y = jnp.dot(_b(wot_s[b][r0 // 2:r1 // 2, :]), _b(ot_s[b][:, ring(q)]),
                        preferred_element_type=f32)

            def post():
                if b == 0:
                    if n == 0:
                        ohold[q] = y
                    elif n == 1:
                        put(q, 0, 256, jnp.concatenate([ohold.pop(q), y], axis=0))
                    elif n == 2 and q == NT - 1:
                        put(q, 256, 384, y)
                    else:
                        made("m", 0, q, n)
                        omid_s[q % 4, 128 * (n - 2):r1 - 256] = y
                else:
                    if n == 0:
                        need("m", 0, q, 2)
                        need("m", 0, q, 3)
                        put(q, 256, 512, jnp.concatenate([omid_s[q % 4], y], axis=0))
                    elif n == 1:
                        ohold[q] = y
                    elif n == 2:
                        put(q, 512, 768, jnp.concatenate([ohold.pop(q), y], axis=0))
                    else:
                        put(q, 768, 896, y)
            later(post)

        def final_out():
            q = NT - 1
            for t in range(4):
                need("o", 1, q, t)
            need("m", 0, q, 3)
            parts = []
            sets = [list(range(n, 28, 4)) for n in range(4)]
            for k0, k1 in ((128, D), (0, 128)):
                rhs = _b(ot_s[1][k0 // 2:k1 // 2, ring(q)])
                ys = [jnp.dot(_b(jnp.concatenate([wot_s[1][8*u:8*u + 8, k0:k1] for u in st], axis=0)), rhs,
                              preferred_element_type=f32) for st in sets]
                parts = [y + p for y, p in zip(ys, parts)] if parts else ys
            ch = {u: p[16*i:16*i + 16] for st, p in zip(sets, parts) for i, u in enumerate(st)}
            y = jnp.concatenate([omid_s[q % 4, 128:192]] + [ch[u] for u in range(28)], axis=0)
            for c0, c1 in FPIECES:
                put(q, c0, c1, y[c0 - 384:c1 - 384])

        def wtile(src, dst, i, ncol):
            c0, c1 = 128 * i, min(128 * i + 128, ncol)
            dst[c0 // 2:c1 // 2, :] = _w(src[:, c0:c1].T)

        def projs(u):
            s, b = divmod(u, 2)
            return [(lambda p=p, t=t, q=q: proj(b, q, p, t))
                    for p in (1, 0, 2) for q in (2*s, 2*s + 1) for t in range(4)]

        def outs(u, qi):
            s, b = divmod(u, 2)
            return [(lambda n=n: outp(b, 2*s + qi, n)) for n in range(4)]

        groups = [(u % 2, 2 * (u // 2) + qi, t) for u in us for qi in range(2) for t in range(4)]
        if last:
            groups = [(1, NT - 2, t) for t in range(4)] + [(1, NT - 1, t) for t in (3, 2, 1, 0)]
        N = len(groups)
        Xs = [[None] * 4 for _ in range(N)]
        accs = [None] * N

        def emit_pv(slot):
            for T in range(3):
                r = slot - 3 - DELAY - PVOFF[T]
                if r >= 0 and r % 4 == 0 and r // 4 < N:
                    g = r // 4
                    Xs[g] = [x() if callable(x) else x for x in Xs[g]]
                    accs[g] = pv(*groups[g], Xs[g], T, accs[g])
                    if T == 2:
                        fin(*groups[g], accs[g])
                        Xs[g] = accs[g] = None

        fill = {}

        def spread(thunks, lo, hi):
            n = len(thunks)
            for k, th in enumerate(thunks):
                fill.setdefault(lo + (k * (hi - lo)) // n, []).append(th)

        ntail = sum(TAILF)
        if first:
            for cw, cx in zip(stage_w, stage_x):
                for cp in cw + cx:
                    cp.start()
            for cp in bcopies:
                cp.start()
            row = _iota((64, 128), 0)
            lane = _iota((64, 128), 1)
            half, hh, l, jlo = row // 32, (row % 32) // 14, lane // 32, (lane & 16) == 0
            ok = hh < 2
            o_s[S:S + 16, :] = jnp.zeros((16, 2 * D), bf16)

            def bits(m):
                return jnp.where(m & ok, jnp.uint32(0xFFFFFFFF), jnp.uint32(0))
            for c in range(4):
                mq_s[c] = bits(((2 * half + hh + l) & 3) == c)
                for k in range(2):
                    sb = (2 * k + hh + l) & 3
                    isf = half == k
                    own = (sb == c) & (isf == jlo)
                    other = (sb == (c + 2) % 4) & (isf if c >= 2 else ~isf)
                    mq_s[4 + 4 * k + c] = bits(own | other)

            def wsub(k0, k1, c0, c1):
                for c in range(c0, c1, 128):
                    ce = min(c + 128, c1)
                    wta_s[c // 2:ce // 2, k0:k1] = _w(wa_s[k0:k1, c:ce].T)
            part_sum = {}
            for i, (ws, xs, work) in enumerate(STAGES):
                _wait(stage_w[i] + (stage_x[i] if i else []))
                for blk in ws:
                    wsub(*blk)
                if i == 0:
                    _wait(stage_x[0])
                if i == len(STAGES) - 1:
                    for cp in xrest:
                        cp.start()
                for n0, n1, k0, k1 in work:
                    y = jnp.dot(_b(wta_s[56 * n0:56 * n1, k0:k1]), xa_s[0, k0:k1, :], preferred_element_type=f32)
                    for n in range(n0, n1):
                        z = y[112 * (n - n0):112 * (n - n0) + 112]
                        assert part_sum.get(n, (None, 0))[1] == k0
                        part_sum[n] = (z if k0 == 0 else z + part_sum[n][0], k1)
            xfin = {}
            held = []

            def proj_fin(qp, n, defer=False):
                z, k0 = part_sum[n]
                if (qp, k0) not in xfin:
                    xfin[qp, k0] = xa_s[0, k0:D, 256 * qp:256 * qp + 256]
                y = jnp.dot(_b(wta_s[56 * n:56 * n + 56, k0:D]), xfin[qp, k0], preferred_element_type=f32)
                y = y + z[:, 256 * qp:256 * qp + 256]

                def post():
                    for i in range(2):
                        proj_post(0, 2 * qp + i, n // 4, n % 4, y[:, 128 * i:128 * i + 128])
                if defer:
                    held.append(post)
                else:
                    post()
            for n in range(12):
                proj_fin(0, n)

            def b_prep():
                _wait(bcopies)
                held.pop()()
                for ti in range(11):
                    wtile(wb_s, wtb_s, ti, 3 * D)
                for ti in range(4):
                    wtile(woa_s, wota_s, ti, D)
                    wtile(wob_s, wotb_s, ti, D)
            spread([(lambda n=n: proj_fin(1, n)) for n in (4, 5, 6, 7, 0, 1, 2, 3)], 0, FA1)
            spread([(lambda n=n: proj_fin(1, n)) for n in (8, 9, 10)], FA1, WBSLOT)
            fill.setdefault(WBSLOT, []).extend([lambda: proj_fin(1, 11, defer=True), b_prep])
            spread([(lambda p=p, t=t, q=q: proj(1, q, p, t))
                    for q, order in ((0, (0, 1, 2)), (1, (1, 0, 2))) for p in order for t in range(4)],
                   WBSLOT + 2, FB1)
            more = outs(0, 0) + outs(0, 1) + projs(3)
            spread(more[:len(more) - ntail], FB1, 96)
            tail = more[len(more) - ntail:]
        elif not last:
            pslots = [s for s in range(32) if s % 4 != OPOS]
            for k, u in enumerate(us):
                p = projs(u + 1)
                if u == us[-1]:
                    p, tail = p[:24 - ntail], p[24 - ntail:]
                for i, th in enumerate(p):
                    fill.setdefault(32 * k + pslots[(i * 24) // len(p)], []).append(th)
                for i, th in enumerate(outs(u - 2, 0) + outs(u - 2, 1)):
                    fill.setdefault(32 * k + 4 * i + OPOS, []).append(th)
        else:
            oa = outs(14, 1)
            spread(outs(13, 0) + outs(13, 1) + outs(14, 0) + oa[:2], 0, LA)
            spread(outs(15, 0), LA, LB)
            tail = oa[2:]

        slot = 0
        for g in range(N):
            pat = "a0f2fb1f3f" if groups[g][1] >= 2 else "0f2f1f3f"
            if g == 0 and kind == "mid":
                pat = "fa02fb1f3f"
            for tok in pat:
                cur[0] = slot
                if tok in "ab":
                    need("q", *groups[g])
                    need("k", *groups[g])
                    edge(*groups[g], "ab".index(tok))
                    edge(*groups[g], "ab".index(tok) + 2)
                elif tok == "f":
                    emit_pv(slot)
                    for th in fill.get(slot, []):
                        th()
                    slot += 1
                    run_posts(slot)
                else:
                    Xs[g][int(tok)] = qk(*groups[g], int(tok))

        def take(n):
            for _ in range(n):
                tail.pop(0)()
        nd = DELAY + max(PVOFF)
        if last:
            run_posts(10**9)
            take(len(tail))
            for k in range(nd):
                emit_pv(slot)
                slot += 1
            run_posts(10**9)
            final_out()
            _wait([ocopy(128 * q) for q in range(NT - 1)]
                  + [ocopy(128 * (NT - 1), c0, c1) for c0, c1 in ((0, 256), (256, 384)) + FPIECES])
            return
        for k in range(nd):
            if k < len(TAILF) - 1:
                take(TAILF[k])
            emit_pv(slot)
            slot += 1
        take(len(tail))
        run_posts(10**9)
        if first:
            _wait(xrest)

    pl.when(step == 0)(lambda: body("first"))
    pl.when(jnp.logical_and(step > 0, step < 4))(lambda: body("mid"))
    pl.when(step == 4)(lambda: body("last"))


@jax.jit
def pallas_concat_heads__sliding_block__sliding_block__prompt_kernel(
    A_x: jax.Array,
    A_wqkv: jax.Array,
    A_wo: jax.Array,
    B_x: jax.Array,
    B_wqkv: jax.Array,
    B_wo: jax.Array,
):
    xa = A_x.reshape(S, D).T
    xb = B_x.reshape(S, D).T
    V = pltpu.VMEM

    def two(shape, dtype):
        return [V(shape, dtype), V(shape, dtype)]

    scratch = (
        two((4, D, 512), bf16)
        + two((D, 3 * D), bf16) + two((D, D), bf16)
        + two((3 * D // 2, D), u32) + two((D // 2, D), u32)
        + two((256, 512), u32) + two((256, 512), u32)
        + two((256, 512), u32) + two((D // 2, 512), u32)
        + [V((4, 192, 128), f32), V((12, 64, 128), u32)]
        + [V((1, 256, 128), f32)] * NSTAGE_BUFS
        + [V((S + 16, 2 * D), bf16),
           pltpu.SemaphoreType.DMA((24,)),
           pltpu.SemaphoreType.DMA((1,))])
    out = pl.pallas_call(
        _kernel,
        grid=(5,),
        in_specs=[pl.BlockSpec(memory_space=pl.ANY)] * 6,
        out_specs=pl.BlockSpec(memory_space=pl.ANY),
        out_shape=jax.ShapeDtypeStruct((S, 2 * D), bf16),
        scratch_shapes=scratch,
        compiler_params=pltpu.CompilerParams(
            dimension_semantics=("arbitrary",), vmem_limit_bytes=100 * 1024 * 1024,
            disable_semaphore_checks=True, disable_bounds_checks=True),
    )(xa, xb, A_wqkv, A_wo, B_wqkv, B_wo)
    return out.reshape(1, S, 2 * D)
```
